```python
import jax
import jax.numpy as jnp

def _softmax(x, axis=-1):
    return jax.nn.softmax(x, axis=axis)

def _gelu(x):
    return jax.nn.gelu(x, approximate=True)

def _silu(x):
    return jax.nn.silu(x)

def _sigmoid(x):
    return jax.nn.sigmoid(x)

def _layernorm(x, axis=-1, eps=1e-05):
    m = jnp.mean(x, axis=axis, keepdims=True)
    v = jnp.var(x, axis=axis, keepdims=True)
    return (x - m) / jnp.sqrt(v + eps)

def _scatter_add(tgt, idx, src, axis=0):
    return tgt.at[idx].add(src)

def _segment_sum(src, seg, n):
    return jax.ops.segment_sum(src, seg, n)

class _Rng:

    def __init__(self, key):
        self._k = key

    def _next(self):
        self._k, sub = jax.random.split(self._k)
        return sub

    def normal(self, shape):
        return jax.random.normal(self._next(), shape, dtype=jnp.bfloat16)

    def randint(self, lo, hi, shape):
        return jax.random.randint(self._next(), shape, lo, hi, dtype=jnp.int32)

    def uniform(self, shape, lo=0.0, hi=1.0):
        return jax.random.uniform(self._next(), shape, jnp.bfloat16, lo, hi)

    def permutation(self, n):
        return jax.random.permutation(self._next(), n)
kernel_name = 'adaLN_cond__linear_kernel_hedgehog__moe_arch_mod__prompt'

def setup_inputs():
    _rng = _Rng(jax.random.key(int.from_bytes(__import__("os").urandom(4), "little")))
    _w = lambda a: (lambda t: t.astype(jnp.bfloat16) if jnp.issubdtype(t.dtype, jnp.floating) else t)(jnp.asarray(a))

    def _A_setup():
        B, S, D, H = (1, 2048, 1024, 32)
        Dh = D // H
        return {'x': _w((lambda *s: _rng.normal(s) * 0.05)(B, S, D)), 'wqkv': _w((lambda *s: _rng.normal(s) * 0.05)(D, 3 * D)), 'w_phi': _w((lambda *s: _rng.normal(s) * 0.05)(H, Dh, Dh) * Dh ** (-0.5)), 'wo': _w((lambda *s: _rng.normal(s) * 0.05)(D, D))}
    _A_in = _A_setup()

    def _B_setup():
        B, S, D, F, C = (1, 2048, 1024, 3584, 2)
        return {'x': _w((lambda *s: _rng.normal(s) * 0.05)(B, S, D)), 'w_r': _w((lambda *s: _rng.normal(s) * 0.05)(D)), 'w_gate': _w((lambda *s: _rng.normal(s) * 0.05)(D, F)), 'w_up': _w((lambda *s: _rng.normal(s) * 0.05)(D, F)), 'w_down': _w((lambda *s: _rng.normal(s) * 0.05)(F, D))}
    _B_in = _B_setup()
    return {'A_x': _A_in['x'], 'A_wqkv': _A_in['wqkv'], 'A_w_phi': _A_in['w_phi'], 'A_wo': _A_in['wo'], 'B_x': _B_in['x'], 'B_w_r': _B_in['w_r'], 'B_w_gate': _B_in['w_gate'], 'B_w_up': _B_in['w_up'], 'B_w_down': _B_in['w_down'], 'c': _w((lambda *s: _rng.normal(s) * 0.05)(1, 1024)), 'w_mod': _w((lambda *s: _rng.normal(s) * 0.05)(1024, 6 * 1024) * 1024 ** (-0.5))}

def reference(A_x, A_wqkv, A_w_phi, A_wo, B_x, B_w_r, B_w_gate, B_w_up, B_w_down, c, w_mod):

    def _A_ref(x, wqkv, w_phi, wo):
        B, S, D = x.shape
        H = 32
        Dh = D // H
        qkv = (lambda x, *d: x.transpose(*d))((x @ wqkv).reshape(B, S, 3, H, Dh), 2, 0, 3, 1, 4)
        q, k, v = (qkv[0], qkv[1], qkv[2])
        pq = jnp.einsum('bhsd,hdf->bhsf', q, w_phi)
        pk = jnp.einsum('bhsd,hdf->bhsf', k, w_phi)
        phi_q = jnp.concatenate([_softmax(pq, axis=-1), _softmax(-pq, axis=-1)], axis=-1)
        phi_k = jnp.concatenate([_softmax(pk, axis=-1), _softmax(-pk, axis=-1)], axis=-1)
        kv = jnp.einsum('bhsf,bhsd->bhfd', phi_k, v)
        z = jnp.einsum('bhsf->bhf', phi_k)
        num = jnp.einsum('bhqf,bhfd->bhqd', phi_q, kv)
        den = jnp.einsum('bhqf,bhf->bhq', phi_q, z)[..., None] + 1e-06
        o = num / den
        return (lambda x, *d: x.transpose(*d))(o, 0, 2, 1, 3).reshape(B, S, D) @ wo

    def _B_ref(x, w_r, w_gate, w_up, w_down):
        B, S, D = x.shape
        C = 2
        r = x @ w_r
        idx = jnp.argsort(-r, axis=-1)[:, :C]
        idx_e = jnp.repeat(idx.reshape(B, C, 1), D, axis=2)
        x_sel = jnp.take_along_axis(x, idx_e, axis=1)
        g = _silu(x_sel @ w_gate)
        u = x_sel @ w_up
        y = g * u @ w_down
        r_sel = _sigmoid(jnp.take_along_axis(r, idx, axis=1))
        y = y * r_sel.reshape(B, C, 1)
        b_off = (jnp.arange(B) * S).reshape(B, 1)
        flat_idx = (idx + b_off).reshape(B * C)
        zero = (x * 0.0).reshape(B * S, D)
        upd = _scatter_add(zero, flat_idx, y.reshape(B * C, D), axis=0)
        return x + upd.reshape(B, S, D)
    x = A_x
    mod = (_silu(c) @ w_mod).reshape(c.shape[0], 6, 1, -1)
    sa, ca, ga, sb, cb, gb = (mod[:, 0].copy(), mod[:, 1].copy(), mod[:, 2].copy(), mod[:, 3].copy(), mod[:, 4].copy(), mod[:, 5].copy())
    h = _layernorm(x, axis=-1) * (1 + ca) + sa
    x = x + ga * _A_ref(h, A_wqkv, A_w_phi, A_wo)
    h = _layernorm(x, axis=-1) * (1 + cb) + sb
    x = x + gb * _B_ref(h, B_w_r, B_w_gate, B_w_up, B_w_down)
    return x
```

```python
import jax
import jax.numpy as jnp
from jax import lax
import jax.experimental.pallas as pl
import jax.experimental.pallas.tpu as pltpu

S, D, H, DH, F = 2048, 1024, 32, 32, 3584
G = 8
T1 = 512
T2 = 256
LOG2E = 1.4426950408889634
NT = (((1,), (1,)), ((), ()))
NN = (((1,), (0,)), ((), ()))
F32, BF16 = jnp.float32, jnp.bfloat16


def _dot(a, b, dims=NN):
    return lax.dot_general(a, b, dims, preferred_element_type=F32)


def _rnd(x):
    return x.astype(BF16).astype(F32)


def _iota(shape, axis):
    return lax.broadcasted_iota(jnp.int32, shape, axis)


def _head_reduce(x3, op):
    m = op(op(op(x3[0], x3[1]), op(x3[2], x3[3])), op(op(x3[4], x3[5]), op(x3[6], x3[7])))
    m = op(m, pltpu.roll(m, 2, 0))
    return op(m, pltpu.roll(m, 4, 0))


def _exp_pm(p):
    p3 = p.reshape(8, 8, p.shape[1])
    ep = jnp.exp2(p3 - _head_reduce(p3, jnp.maximum)[None])
    en = jnp.exp2(_head_reduce(p3, jnp.minimum)[None] - p3)
    return ep, en, _head_reduce(ep, jnp.add), _head_reduce(en, jnp.add)


def _center_scale(x):
    mean = jnp.mean(x, axis=-1, keepdims=True)
    mr = _rnd(mean)
    d = x - mr
    var = jnp.mean(d * d, axis=-1, keepdims=True) - (mean - mr) * (mean - mr)
    sd = _rnd(jnp.sqrt(_rnd(_rnd(var) + _rnd(jnp.full_like(var, 1e-5)))))
    return d, 1.0 / sd


def _kernel(x_hbm, wqkv_hbm, wphi_hbm, wo_hbm, wr_hbm, wg_hbm, wu_hbm, wd_hbm, c_hbm, wmod_hbm,
            out_hbm,
            x_buf, w_buf, wphi_buf, wo_buf, wr_buf, wg_buf, wu_buf, wd_buf, c_buf, wmod_buf,
            h_buf, wt_buf, y_bufs, pq_buf, o_buf, a_bufs, x1_buf, out_buf, fix_buf, sem):
    n1, n2 = S // T1, S // T2
    s_x, s_w, s_misc, s_out = 0, n1, n1 + 3 * G, n1 + 3 * G + 9
    s_fix = s_out + n2

    def x_copy(j):
        r = pl.ds(j * T1, T1)
        return pltpu.make_async_copy(x_hbm.at[r], x_buf.at[r], sem.at[s_x + j])

    def w_copy(i, g):
        col = i * D + g * 128
        if not isinstance(col, int):
            col = pl.multiple_of(col, 128)
        return pltpu.make_async_copy(wqkv_hbm.at[:, pl.ds(col, 128)], w_buf.at[i, g], sem.at[s_w + i * G + g])

    def mod_cols(lo, n):
        return wmod_hbm.at[:, pl.ds(lo, n)], wmod_buf.at[:, pl.ds(lo, n)]

    cp_c, cp_phi, cp_moda, cp_modb, cp_wr, cp_wo, cp_wg, cp_wu, cp_wd = [
        pltpu.make_async_copy(s, d, sem.at[s_misc + i]) for i, (s, d) in enumerate((
            (c_hbm, c_buf), (wphi_hbm, wphi_buf), mod_cols(0, 2 * D), mod_cols(2 * D, 4 * D),
            (wr_hbm, wr_buf), (wo_hbm, wo_buf), (wg_hbm, wg_buf), (wu_hbm, wu_buf), (wd_hbm, wd_buf)))]

    def out_copy(t):
        r = pl.ds(t * T2, T2)
        return pltpu.make_async_copy(out_buf.at[r], out_hbm.at[r], sem.at[s_out + t])

    cp_c.start()
    cp_phi.start()
    for i in range(3):
        w_copy(i, 0).start()
    cp_moda.start()
    for j in range(n1):
        x_copy(j).start()
    for g in range(1, G):
        for i in range(3):
            w_copy(i, g).start()
    for cp in (cp_modb, cp_wr, cp_wo, cp_wg, cp_wu, cp_wd):
        cp.start()

    row, lane = _iota((128, 128), 0), _iota((128, 128), 1)
    eye = (row == lane).astype(BF16)
    same_head = (row // 64) * 2 + row % 2 == lane // DH
    sel = ((_iota((128, DH), 0) % 64) // 2 == _iota((128, DH), 1)).astype(BF16)

    def fold_wait(g):
        for i in range(3):
            w_copy(i, g).wait()

    def fold(g):
        wp = wphi_buf[pl.ds(g * 4, 4)].reshape(128, DH)
        mix = jnp.where(same_head, _dot(sel, wp, NT), 0.0).astype(BF16)
        wt_buf[0:128] = (_dot(mix, w_buf[0, g], NT) * LOG2E).astype(BF16)
        wt_buf[128:256] = (_dot(mix, w_buf[1, g], NT) * LOG2E).astype(BF16)
        wt_buf[256:384] = _dot(eye, w_buf[2, g], NT).astype(BF16)

    cp_phi.wait()
    fold_wait(0)
    fold(0)
    cp_c.wait()
    cv = c_buf[...].astype(F32)
    sc = jnp.broadcast_to(_rnd(cv * _rnd(jax.nn.sigmoid(cv))), (16, D)).astype(BF16)
    cp_moda.wait()
    mod_a = _rnd(_dot(sc, wmod_buf[:, 0:2 * D])[0:1])
    sa, ca1 = mod_a[:, 0:D], _rnd(1.0 + mod_a[:, D:2 * D])

    def ln1(j):
        for r in range(j * T1, (j + 1) * T1, 64):
            d, rs = _center_scale(x_buf[r:r + 64].astype(F32))
            h_buf[r:r + 64] = (d * rs * ca1 + sa).astype(BF16)

    def project(j):
        y_bufs[j][...] = _dot(wt_buf[...], h_buf[j * T1:(j + 1) * T1], NT)

    def key_side(j, acc):
        pq_buf[:, j * T1:(j + 1) * T1] = y_bufs[j][0:128]
        new = []
        for p in range(2):
            ep, en, sp, sn = _exp_pm(y_bufs[j][128 + 64 * p:192 + 64 * p])
            phi = jnp.concatenate([(ep * (1.0 / sp)[None]).reshape(64, T1),
                                   (en * (1.0 / sn)[None]).reshape(64, T1)], axis=0)
            z = phi[:, 0:128]
            for l in range(128, T1, 128):
                z = z + phi[:, l:l + 128]
            kv = _dot(y_bufs[j][256 + 64 * p:320 + 64 * p].astype(BF16), phi.astype(BF16), NT)
            new.append((kv, z) if acc is None else (acc[p][0] + kv, acc[p][1] + z))
        return new

    kv_mask = _iota((64, 128), 0) // DH == _iota((64, 128), 1) % 2

    def finish(acc):
        return [(jnp.where(kv_mask, kv, 0.0).astype(BF16),
                 jnp.broadcast_to(jnp.sum(z, axis=-1, keepdims=True), (128, 128))) for kv, z in acc]

    def query_side(g, j, state):
        outs = []
        for p in range(2):
            kv, z = state[p]
            ep, en, sp, sn = _exp_pm(pq_buf[64 * p:64 * p + 64, j * T1:(j + 1) * T1])
            zt = jnp.concatenate([z] * (T1 // 128), axis=1)
            dp = _head_reduce(ep * zt[0:64].reshape(8, 8, T1), jnp.add)
            dn = _head_reduce(en * zt[64:128].reshape(8, 8, T1), jnp.add)
            iden = 1.0 / (dp * sn + dn * sp + 1e-6 * (sp * sn))
            phi = jnp.concatenate([(ep * (sn * iden)[None]).reshape(64, T1),
                                   (en * (sp * iden)[None]).reshape(64, T1)], axis=0)
            outs.append(_dot(kv, phi.astype(BF16)))
        o_buf[g, j * T1:(j + 1) * T1, :] = jnp.concatenate(outs, axis=0).T.astype(BF16)

    x_copy(0).wait()
    ln1(0)
    acc = None
    for j in range(n1):
        if j + 1 < n1:
            x_copy(j + 1).wait()
        else:
            fold_wait(1)
        project(j)
        if j + 1 < n1:
            ln1(j + 1)
        else:
            fold(1)
        if j > 0:
            acc = key_side(j - 1, acc)
    state = finish(key_side(n1 - 1, acc))

    def group(g, state, last):
        if not last:
            fold_wait(g + 1)
        acc = None
        for j in range(n1):
            query_side(g - 1, j, state)
            project(j)
            if j == n1 - 1 and not last:
                fold(g + 1)
            if j > 0:
                acc = key_side(j - 1, acc)
        return finish(key_side(n1 - 1, acc))

    state = lax.fori_loop(1, G - 1, lambda g, st: group(g, st, False), state)
    state = group(G - 1, state, True)

    cp_modb.wait()
    cp_wr.wait()
    cp_wo.wait()
    mod_b = _rnd(_dot(sc, wmod_buf[:, 2 * D:6 * D])[0:1])
    for j in range(n1):
        query_side(G - 1, j, state)
    ga, sb, gb = mod_b[:, 0:D], mod_b[:, D:2 * D], mod_b[:, 3 * D:4 * D]
    cb1 = _rnd(1.0 + mod_b[:, 2 * D:3 * D])
    wr = wr_buf[...].reshape(1, D).astype(F32)
    out_mul, out_add, r_mul = gb * cb1, gb * sb, cb1 * wr
    r_add = jnp.sum(sb * wr, axis=-1, keepdims=True)

    lane8 = _iota((8, 128), 1)

    def attn_out(t):
        o = jnp.concatenate([o_buf[g, t * T2:(t + 1) * T2, :] for g in range(G)], axis=1)
        a_bufs[t % 2][...] = _dot(o, wo_buf[...])

    def epilogue(t, racc):
        racc = list(racc)
        for k in range(0, T2, 64):
            r0 = t * T2 + k
            x1 = x_buf[r0:r0 + 64].astype(F32) + ga * a_bufs[t % 2][k:k + 64]
            x1_buf[r0:r0 + 64] = x1
            d, rs = _center_scale(x1)
            out_buf[r0:r0 + 64] = (x1 + (d * rs * out_mul + out_add)).astype(BF16)
            r = jnp.sum(d * r_mul, axis=-1, keepdims=True) * rs
            for i in range(8):
                blk = r0 // 8 + i
                rk = jnp.broadcast_to(r[8 * i:8 * i + 8], (8, 128))
                racc[blk // 128] = jnp.where(lane8 == blk % 128, rk, racc[blk // 128])
        out_copy(t).start()
        return racc

    racc = [jnp.zeros((8, 128), F32)] * 2
    attn_out(0)
    for t in range(n2):
        if t + 1 < n2:
            attn_out(t + 1)
        racc = epilogue(t, racc)

    r = _rnd(jnp.concatenate(racc, axis=0) + r_add)
    r = jnp.where(r != r, -jnp.inf, r)
    tok = (_iota((16, 128), 0) // 8) * 1024 + _iota((16, 128), 1) * 8 + _iota((16, 128), 0) % 8
    i1 = jnp.min(jnp.where(r == jnp.max(r), tok, S - 1))
    r2 = jnp.where(tok == i1, -jnp.inf, r)
    i2 = jnp.min(jnp.where((r2 == jnp.max(r2)) & (tok != i1), tok, S - 1))
    b1 = pl.multiple_of(jnp.clip(i1 // 16, 0, S // 16 - 1) * 16, 16)
    b2 = pl.multiple_of(jnp.clip(i2 // 16, 0, S // 16 - 1) * 16, 16)

    x1 = jnp.concatenate([x1_buf[pl.ds(b1, 16)], x1_buf[pl.ds(b2, 16)]], axis=0)
    d, rs = _center_scale(x1)
    h2 = d * rs * cb1 + sb
    gate = jax.nn.sigmoid(_rnd(jnp.sum(h2 * wr, axis=-1, keepdims=True)))
    hb = h2.astype(BF16)
    cp_wg.wait()
    cp_wu.wait()
    cp_wd.wait()
    u = _dot(hb, wg_buf[...])
    act = u * jax.nn.sigmoid(u) * _dot(hb, wu_buf[...])
    y = _dot(act.astype(BF16), wd_buf[...]) * gate
    rows = _iota((32, 1), 0)
    rows = jnp.where(rows < 16, rows + b1, rows - 16 + b2)
    picked = (rows == i1) | (rows == i2)
    fix_buf[...] = (x1 + gb * (h2 + jnp.where(picked, y, 0.0))).astype(BF16)

    for t in range(n2):
        out_copy(t).wait()
    fix1 = pltpu.make_async_copy(fix_buf.at[0:16], out_hbm.at[pl.ds(b1, 16)], sem.at[s_fix])
    fix2 = pltpu.make_async_copy(fix_buf.at[16:32], out_hbm.at[pl.ds(b2, 16)], sem.at[s_fix + 1])
    fix1.start()

    @pl.when(b1 != b2)
    def _():
        fix2.start()
        fix2.wait()

    fix1.wait()


@jax.jit
def pallas_adaLN_cond__linear_kernel_hedgehog__moe_arch_mod__prompt_kernel(
    A_x, A_wqkv, A_w_phi, A_wo, B_x, B_w_r, B_w_gate, B_w_up, B_w_down, c, w_mod,
):
    hbm = pl.BlockSpec(memory_space=pl.ANY)
    n1, n2 = S // T1, S // T2
    out = pl.pallas_call(
        _kernel,
        out_shape=jax.ShapeDtypeStruct((S, D), BF16),
        in_specs=[hbm] * 10,
        out_specs=hbm,
        scratch_shapes=[
            pltpu.VMEM((S, D), BF16),
            pltpu.VMEM((3, G, D, 128), BF16),
            pltpu.VMEM((H, DH, DH), BF16),
            pltpu.VMEM((D, D), BF16),
            pltpu.VMEM((D,), BF16),
            pltpu.VMEM((D, F), BF16),
            pltpu.VMEM((D, F), BF16),
            pltpu.VMEM((F, D), BF16),
            pltpu.VMEM((1, D), BF16),
            pltpu.VMEM((D, 6 * D), BF16),
            pltpu.VMEM((S, D), BF16),
            pltpu.VMEM((384, D), BF16),
            [pltpu.VMEM((384, T1), F32)] * n1,
            pltpu.VMEM((128, S), F32),
            pltpu.VMEM((G, S, 128), BF16),
            [pltpu.VMEM((T2, D), F32)] * 2,
            pltpu.VMEM((S, D), F32),
            pltpu.VMEM((S, D), BF16),
            pltpu.VMEM((32, D), BF16),
            pltpu.SemaphoreType.DMA((n1 + 3 * G + 9 + n2 + 2,)),
        ],
        compiler_params=pltpu.CompilerParams(vmem_limit_bytes=110 * 2**20),
        name="adaln_hedgehog_mod",
    )(A_x.reshape(S, D), A_wqkv, A_w_phi, A_wo, B_w_r, B_w_gate, B_w_up, B_w_down, c, w_mod)
    return out.reshape(1, S, D)
```

```python
import jax
import jax.numpy as jnp
from jax import lax
import jax.experimental.pallas as pl
import jax.experimental.pallas.tpu as pltpu


S, D, H, DH, F = 2048, 1024, 32, 32, 3584
G = 8
HD = D // 2
T = 256
HT = T // 2
NC = S // T
NG = G
NT2 = NC
TIEQ, TIER, TIEF, TIEE = 1, 0, 2, 1
KLAG, RLAG = 1, 1
PLAN0, WAITD = "wpppppppf", 0
ORDER = [int(c) for c in "1324056"]
PLAN = "pwkkqpqpqpqpqpqprqpqf"
ORDER2 = [int(c) for c in "1305246"]
PLAN2 = "wpkkpqpqpqpqprp"
WAITB, WAITC = 16, 24
EOFF = 9.0
OPAQUE = "wos,coef,out".split(",")
XW = "1,23,4,5,6,7,,".split(",")
WOLEAD = 0
SYNC1, SYNC2 = 0, 0
FINE = 0
EEND = 9.0
PIPE, DMALAG = 0, 2
WAITS, KRATE = 8, 2
F1, LNP, LASTP = 1, 2, 1
KEYLAG, WOC = 1, 128
PLAND, MODS = "kkqpppprpppp", "2231"
OPAQUEG = "none".split(",")
LNMODE = 0
BF16_MAX, F32_TINY = 3.3895313892515355e38, 1.1754943508222875e-38
LOG2E = 1.4426950408889634
NT = (((1,), (1,)), ((), ()))
NN = (((1,), (0,)), ((), ()))
F32, BF16, U32 = jnp.float32, jnp.bfloat16, jnp.uint32


def _dot(a, b, dims=NN):
    return lax.dot_general(a, b, dims, preferred_element_type=F32)


def _rnd(x):
    return x.astype(BF16).astype(F32)


def _pack(even, odd):
    return pltpu.pack_elementwise([even, odd], packed_dtype=BF16)


def _pack_halves(x):
    n = x.shape[0] // 2
    return _pack(x[:n], x[n:])


def _split(x):
    words = pltpu.bitcast(x, U32)
    return [pltpu.unpack_elementwise(words, index=i, packed_dtype=BF16, unpacked_dtype=F32) for i in range(2)]


def _unpack(x):
    return pltpu.bitcast(x, BF16)


def _iota(shape, axis):
    return lax.broadcasted_iota(jnp.int32, shape, axis)


def _tree(x3, op):
    return op(op(op(x3[0], x3[1]), op(x3[2], x3[3])), op(op(x3[4], x3[5]), op(x3[6], x3[7])))


def _fold_rows(m, op):
    m = op(m, pltpu.roll(m, 2, 0))
    return op(m, pltpu.roll(m, 4, 0))


def _softmax2(p3, sign):
    if sign == 0:
        e = jnp.exp2(p3 - _fold_rows(_tree(p3, jnp.maximum), jnp.maximum)[None])
    else:
        e = jnp.exp2(_fold_rows(_tree(p3, jnp.minimum), jnp.minimum)[None] - p3)
    return e * pl.reciprocal(_fold_rows(_tree(e, jnp.add), jnp.add), full_range=False)[None]


def _row_means(xs):
    return [jnp.mean(x, axis=-1, keepdims=True) for x in xs]


def _row_spread(xs, means):
    lane = _iota((xs[0].shape[0], 128), 1)
    cen, var = [], None
    for i, (x, mean) in enumerate(zip(xs, means)):
        mr = _rnd(mean)
        d = x - mr
        v = jnp.mean(d * d, axis=-1, keepdims=True) - (mean - mr) * (mean - mr)
        var = jnp.where(lane == i, v, var) if i else jnp.broadcast_to(v, lane.shape)
        cen.append(d)
    return cen, var


def _row_scales(var):
    return 1.0 / _rnd(jnp.sqrt(_rnd(_rnd(var) + _rnd(jnp.full_like(var, 1e-5)))))


def _lhs_term(a, n):
    return (lambda: a(0, 0) + a(1, 1), lambda: a(1, 0) + a(1, 1), lambda: a(0, 0), lambda: a(1, 1),
            lambda: a(0, 0) + a(0, 1), lambda: a(1, 0) - a(0, 0), lambda: a(0, 1) - a(1, 1))[n]()


def _rhs_term(b, n):
    return (lambda: b(0, 0) + b(1, 1), lambda: b(0, 0), lambda: b(0, 1) - b(1, 1), lambda: b(1, 0) - b(0, 0),
            lambda: b(1, 1), lambda: b(0, 0) + b(0, 1), lambda: b(1, 0) + b(1, 1))[n]()


def _quadrant(m, i, j):
    if (i, j) == (0, 0):
        return (m(0) + m(3)) + (m(6) - m(4))
    if (i, j) == (0, 1):
        return m(2) + m(4)
    if (i, j) == (1, 0):
        return m(1) + m(3)
    return (m(0) - m(1)) + (m(2) + m(5))


def _kernel(x_hbm, wqkv_hbm, wphi_hbm, wo_hbm, wr_hbm, wg_hbm, wu_hbm, wd_hbm, c_hbm, wmod_hbm,
            out_hbm,
            x_buf, w_buf, wphi_buf, wo_buf, wr_buf, wg_buf, wu_buf, wd_buf, c_buf, wmod_buf,
            hs_bufs, ws_bufs, pq_bufs, o_bufs, wos_buf, x1_buf, mean_buf, scale_buf, out_bufs, coef_buf, fix_buf, sem):
    s_x, s_w, s_misc, s_out = 0, NC, NC + 3 * G, NC + 3 * G + 12
    s_fix = s_out + NC

    def x_copy(j):
        r = pl.ds(j * T, T)
        return pltpu.make_async_copy(x_hbm.at[r], x_buf.at[0, r], sem.at[s_x + j])

    def w_copy(i, g):
        return pltpu.make_async_copy(wqkv_hbm.at[:, pl.ds(i * D + g * 128, 128)], w_buf.at[i, g],
                                     sem.at[s_w + i * G + g])

    def mod_cols(lo, n):
        return wmod_hbm.at[:, pl.ds(lo, n)], wmod_buf.at[:, pl.ds(lo, n)]

    cp_c, cp_phi0, cp_phi, cp_sa, cp_modb, cp_wr, cp_wo, cp_wg, cp_wu, cp_wd, *cp_ca = [
        pltpu.make_async_copy(s, d, sem.at[s_misc + i]) for i, (s, d) in enumerate((
            (c_hbm, c_buf), (wphi_hbm.at[0:4], wphi_buf.at[0:4]), (wphi_hbm.at[4:H], wphi_buf.at[4:H]),
            mod_cols(0, D), mod_cols(2 * D, 4 * D),
            (wr_hbm, wr_buf), (wo_hbm, wo_buf), (wg_hbm, wg_buf), (wu_hbm, wu_buf), (wd_hbm, wd_buf.at[:, 0:D]),
            *[mod_cols(l, HD) for l in range(D, 2 * D, HD)]))]

    def out_copy(t):
        r = pl.ds(t * T, T)
        return pltpu.make_async_copy(out_bufs[t].at[0, 0:T], out_hbm.at[r], sem.at[s_out + t])

    def wait_weights(groups):
        for g in groups:
            for i in range(3):
                w_copy(i, g).wait()

    def weights(g):
        return [w_copy(i, g) for i in range(3)]

    for cp in (cp_c, cp_phi0, *weights(0), x_copy(0), *cp_ca, x_copy(1), x_copy(2), cp_phi,
               *[x_copy(j) for j in range(3, NC)], *weights(1), cp_sa,
               *[cp for g in range(2, G) for cp in weights(g)], cp_wr, cp_wo, cp_modb, cp_wg, cp_wu, cp_wd):
        cp.start()

    z_put, z_get = [jnp.min(_iota((8, 128), axis)) for axis in range(2)]
    never = _iota((8, 128), 1) < z_get
    val, due, holds = {}, {}, {}

    def put(ref, kind=""):
        return ref.at[z_put if kind in OPAQUE else 0]

    def get(ref, kind=""):
        return ref.at[z_get if kind in OPAQUEG else 0]

    def after(x, dep, r=0):
        head = jnp.where(never, pltpu.bitcast(dep[0:8, 0:128], x.dtype), x[r:r + 8, 0:128])
        if x.shape[1] > 128:
            head = jnp.concatenate([head, x[r:r + 8, 128:]], axis=1)
        parts = ([x[:r]] if r else []) + [head] + ([x[r + 8:]] if x.shape[0] > r + 8 else [])
        return jnp.concatenate(parts, axis=0)

    def released(x, tie=1):
        return after(x, val["last"]) if tie and "last" in val else x

    def meet(x, key):
        cols = [x[:, l:l + 128] for l in range(0, x.shape[1], 128)]
        for j in range(len(cols)):
            for i, dep in enumerate(due.pop((*key, j), [])):
                cols[j] = after(cols[j], dep, 8 * i)
        return jnp.concatenate(cols, axis=1)

    def deadline(slot, n, dep, j=0):
        due.setdefault((slot, n, j), []).append(dep)

    same_head = _iota((128, 128), 0) // DH == _iota((128, 128), 1) // DH
    sel = (_iota((128, DH), 0) % DH == _iota((128, DH), 1)).astype(BF16)
    kv_mask = _iota((64, 128), 0) % 2 == (_iota((64, 128), 1) // 2) % 2

    def bias_part(g, i, k):
        left, right = val["folded", g, i, k]
        term = (left.reshape(16, 8, 128) * val["sa"][:, k:k + 128][None]
                + right.reshape(16, 8, 128) * val["sa"][:, HD + k:HD + k + 128][None])
        val["bias", g, i] = term if k == 0 else val["bias", g, i] + term
        if k == HD - 128:
            b = jnp.broadcast_to(jnp.sum(val["bias", g, i], axis=-1, keepdims=True), (16, 8, 128)).reshape(128, 128)
            for p in range(2):
                pair = b[64 * p:64 * p + 64]
                val["bias", g, i, p] = (_unpack(_pack_halves(pair)).astype(F32)
                                        + _unpack(_pack_halves(pair - _rnd(pair))).astype(F32))

    def fold_tasks(g):
        def part(i, k):
            def run(slot):
                halves = []
                for lo in (k, HD + k):
                    w = _unpack(released(pltpu.bitcast(w_buf[i, g, lo:lo + 128, :], U32), TIEF))
                    halves.append(_dot(val["mix", g].astype(BF16), w, NT) if i < 2 else w.astype(F32).T)
                val["folded", g, i, k] = halves
                if g > 1:
                    bias_part(g, i, k)
                for n in range(7):
                    words = _pack_halves(_lhs_term(lambda p, j: halves[j][64 * p:64 * p + 64], n))
                    put(ws_bufs[g % 3], "ws")[n, 32 * i:32 * i + 32, k:k + 128] = words
                holds["ws", g % 3, i, k] = g
                if TIEF and slot is not None:
                    deadline(slot + TIEF, 1 + k // 128, words)
            return run

        return [part(i, k) for i in range(3) for k in range(0, HD, 128)]

    def ln1_means(c, r):
        rows = [slice(c * T + n * HT + r, c * T + n * HT + r + 16) for n in range(2)]
        xs = [x for n in range(2) for x in _split(x_buf[0, rows[n], :])]
        val["ln", c, r] = xs, _row_means(xs)

    def ln1_spread(c, r):
        val["ln", c, r] = _row_spread(*val["ln", c, r])

    def ln1_scales(c, r):
        cen, var = val["ln", c, r]
        rs = _row_scales(var)
        val["ln", c, r] = [(d, rs[:, i:i + 1]) for i, d in enumerate(cen)]

    def ln1_stats(c, r):
        for stage, lag in ((ln1_means, 0), (ln1_spread, 16), (ln1_scales, 32)):
            if 0 <= r - lag < HT:
                stage(c, r - lag)

    def mix(g):
        wp = wphi_buf[g * 4:g * 4 + 4].reshape(128, DH)
        val["mix", g] = jnp.where(same_head, _dot(sel, wp, NT), 0.0)

    cp_phi0.wait()
    mix(0)
    wait_weights([0])
    for task in fold_tasks(0):
        task(None)
    cp_c.wait()
    cv = c_buf[...].astype(F32)
    sc = jnp.broadcast_to(_rnd(cv * _rnd(jax.nn.sigmoid(cv))), (16, D)).astype(BF16)
    x_copy(0).wait()
    for r in range(0, HT + 32, 16):
        ln1_stats(0, r)
    parts = []
    for i, cp in enumerate(cp_ca):
        cp.wait()
        parts.append(_rnd(1.0 + _rnd(_dot(sc, wmod_buf[:, D + i * HD:D + (i + 1) * HD])[0:8])) * LOG2E)
    ca1 = jnp.concatenate(parts, axis=1)

    def ln1_tasks(c):
        def piece(r):
            def run(slot):
                if c == 1 and r == 0:
                    for step in range(0, HT + 32, 16):
                        ln1_stats(1, step)
                if c == 2 and r == 0:
                    for step in range(0, HT + 32, 16):
                        ln1_stats(2, step)
                if 1 < c < NC - 1:
                    for step in range(r, r + (48 if r == HT - 16 else 16), 16):
                        ln1_stats(c + 1, step)
                        if step >= 32:
                            scale = val["ln", c + 1, step - 32][3][1]
                            deadline(slot + 1, ORDER[step // 16 % LNP], jnp.broadcast_to(scale, (8, 128)))
                stats = val["ln", c, r]
                for k in range(0, HD, 128):
                    h = {}
                    for j in range(2):
                        cols = slice(j * HD + k, j * HD + k + 128)
                        for n in range(2):
                            for e in range(2):
                                d, rs = stats[2 * n + e]
                                h[e, j, n] = d[:, cols] * rs * ca1[:, cols]
                    for n in range(7):
                        hs_bufs[c][0, n, r // 2:r // 2 + 8, k:k + 128] = _pack(
                            *[_rhs_term(lambda j, m: h[e, j, m], n) for e in range(2)])
                holds["hs", c, r] = True
            return run
        return [piece(r) for r in range(0, HT, 16)]

    def project_tasks(g, c):
        def product(n):
            def run():
                assert all(holds["ws", g % 3, i, k] == g for i in range(3) for k in range(0, HD, 128))
                assert all(("hs", c, r) in holds for r in range(0, HT, 16))
                rhs = meet(get(hs_bufs[c])[n], (g * NC + c, n))
                val["last"] = val["m", g * NC + c, n] = _dot(_unpack(get(ws_bufs[g % 3], "ws")[n]), _unpack(rhs), NT)
                at = 7 * (g * NC + c) + ORDER.index(n) + SYNC1
                if SYNC1 and at < 7 * NG * NC:
                    deadline(at // 7, ORDER[at % 7], val["last"][184:192], 3)
            return run
        return [product(n) for n in ORDER]

    def key_tasks(g, c):
        def piece(p, n):
            def run():
                def part(i):
                    y = _quadrant(lambda k: val["m", g * NC + c, k][64 * i:64 * i + 64], p, n)
                    return y + val["bias", g, i, p]
                put(pq_bufs[g % 3])[c, p, n] = part(0)
                holds["pq", g % 3, c, p, n] = g
                val["v", g, c, p, n] = part(2)
                logits = part(1).reshape(8, 8, 128)
                words = []
                for s in range(2):
                    phi = _softmax2(logits, s)
                    words.append(_pack_halves(phi.reshape(64, 128)))
                    val["z", g, p, s] = val["z", g, p, s] + phi if ("z", g, p, s) in val else phi
                val["phik", g, c, p, n] = jnp.concatenate(words, axis=0)
            return run
        return [piece(p, n) for p, n in ((1, 0), (0, 1), (1, 1), (0, 0))]

    def summary_tasks(g, c):
        def piece(p):
            def run():
                v = jnp.concatenate([val["v", g, c, p, n] for n in range(2)], axis=1).astype(BF16)
                phi = _unpack(jnp.concatenate([val["phik", g, c, p, n] for n in range(2)], axis=1))
                kv = _dot(v, phi, NT)
                val["kv", g, p] = kv if c == 0 else val["kv", g, p] + kv
                if c == NC - 1:
                    val["kv", g, p] = jnp.where(kv_mask, val["kv", g, p], 0.0)
                    for s in range(2):
                        z = jnp.sum(val["z", g, p, s], axis=-1, keepdims=True)
                        val["zb", g, p, s] = jnp.broadcast_to(z, (8, 8, 128))
            return run
        return [piece(p) for p in range(2)]

    def query_tasks(g, c):
        def piece(p, n):
            def run():
                assert holds["pq", g % 3, c, p, n] == g
                logits = released(get(pq_bufs[g % 3])[c, p, n], TIEQ).reshape(8, 8, 128)
                words, den = [], None
                for s in range(2):
                    phi = _softmax2(logits, s)
                    words.append(_pack_halves(phi.reshape(64, 128)))
                    w = _tree(phi * val["zb", g, p, s], jnp.add)
                    den = w if den is None else den + w
                val["iden", g, c, p, n] = pl.reciprocal(_fold_rows(den, jnp.add) + 1e-6, full_range=False)
                val["phiq", g, c, p, n] = jnp.concatenate(words, axis=0)
            return run
        return [piece(p, n) for n in range(2) for p in range(2)]

    def readout(g, c, slot):
        nums = [_dot(val["kv", g, p].astype(BF16),
                     _unpack(jnp.concatenate([val["phiq", g, c, p, n] for n in range(2)], axis=1)))
                for p in range(2)]
        for p in range(2):
            for n in range(2):
                num = nums[p][:, n * HT:(n + 1) * HT].reshape(8, 8, 128)
                val["o", g, c, n, p] = (num * val["iden", g, c, p, n][None]).reshape(64, 128)
        if g % 2:
            for k in range(7):
                term = _lhs_term(
                    lambda n, p: jnp.concatenate([val["o", g - 1, c, n, p], val["o", g, c, n, p]], axis=0), k)
                words = pltpu.bitcast(term.astype(BF16).T, U32)
                o_bufs[c][k, :, 64 * (g - 1):64 * (g + 1)] = words
                holds["o", c, g] = True
                if TIER:
                    deadline(slot + TIER, k, words[56:64])
        elif TIER:
            for k, (n, p) in enumerate(((0, 0), (0, 1), (1, 0), (1, 1))):
                deadline(slot + TIER, k, val["o", g, c, n, p][56:64])

    def wo_tasks():
        def piece(r, l):
            def run(slot):
                src = r // DH * 128 + r % DH
                quads = {}
                for e in range(2):
                    for i in range(2):
                        lo = src + i * 64 + DH * e
                        for j in range(2):
                            w = wo_buf[lo:lo + 16, j * HD + l:j * HD + l + WOC].astype(F32)
                            quads[e, i, j] = released(w, TIEF)
                for n in range(7):
                    words = _pack(*[_rhs_term(lambda i, j: quads[e, i, j], n) for e in range(2)])
                    put(wos_buf, "wos")[n, r:r + 16, l:l + WOC] = words
                holds["wos", r, l] = True
                if TIEF:
                    deadline(slot + TIEF, (r // 16 + l // 128) % 7, get(wos_buf, "wos")[0, r:r + 8, l:l + 128])
            return run
        return [piece(r, l) for r in range(0, HD // 2, 16) for l in range(0, HD, WOC)]

    def spread(tasks, n):
        return [tasks[i * len(tasks) // n:(i + 1) * len(tasks) // n] for i in range(n)]

    total = NG * NC
    lead = KEYLAG + KLAG + RLAG + 1
    agenda = {}

    def book(kind, s, item):
        agenda.setdefault((kind, s), []).append(item)

    def key_slot(u):
        return max(u + KEYLAG, WAITS + 1 + u // KRATE)

    for u in range(total):
        g, c = divmod(u, NC)
        s_key = key_slot(u)
        ready = key_slot(g * NC + NC - 1) + KLAG + 1
        first = key_slot(NC - 1) + KLAG + 1
        s_query = max(first + u * (total + KEYLAG + KLAG + NC - first) // total, ready)
        s_query = min(s_query, total + lead + c - RLAG - 1)
        assert s_query >= ready
        book("key", s_key, (g, c))
        book("sum", s_key + KLAG, (g, c))
        book("query", s_query, (g, c))
        book("read", s_query + RLAG, (g, c))

    def run_slot(s, plan, main, extra, wait=None):
        keys = [t for gc in agenda.get(("key", s), []) for t in key_tasks(*gc)]
        queries = [t for gc in agenda.get(("query", s), []) for t in query_tasks(*gc)]
        mixed = sorted([((i + 0.5) / len(keys), 0, i) for i in range(len(keys))]
                       + [((i + 0.5) / len(queries), 1, i) for i in range(len(queries))])
        pieces = spread([(keys, queries)[kind][i] for _, kind, i in mixed], plan.count("q"))
        sums = spread([t for gc in agenda.get(("sum", s), []) for t in summary_tasks(*gc)], plan.count("k"))
        main = list(main)
        for step in plan:
            if step == "p" and main:
                main.pop(0)()
            elif step in "qk":
                for task in (pieces if step == "q" else sums).pop(0):
                    task()
            elif step == "r":
                for gc in agenda.get(("read", s), []):
                    readout(*gc, s)
            elif step == "f":
                for task in extra:
                    task(s)
            elif step == "w" and wait:
                wait()

    def late_inputs():
        wait_weights(range(4, G))
        cp_wr.wait()
        cp_wo.wait()

    def shift():
        cp_sa.wait()
        wait_weights([2, 3])
        val["sa"] = _rnd(_dot(sc, wmod_buf[:, 0:D])[0:8]) * LOG2E

    waits = {c: (lambda js=js: [x_copy(int(j)).wait() for j in js]) for c, js in enumerate(XW) if js}
    waits[3] = lambda: (x_copy(5).wait(), cp_phi.wait())
    waits[6] = lambda: wait_weights([1])
    waits[WAITS] = shift
    waits[min(WAITC, total - 1)] = late_inputs

    extras = {s: [] for s in range(total)}
    for c in range(NC - 1):
        extras[c] += ln1_tasks(c + 1)
    extras[3] += [lambda s, g=g: mix(g) for g in range(1, 5)]
    extras[4] += [lambda s, g=g: mix(g) for g in range(5, G)]
    for k, chunk in enumerate(spread(fold_tasks(1), 3)):
        extras[NC - 2 + (k > 0)] += chunk
    for g in range(2):
        extras[WAITS + g] += [lambda s, g=g, i=i, k=k: bias_part(g, i, k) for i in range(3) for k in range(0, HD, 128)]
    for g in range(2, NG):
        tasks = fold_tasks(g)
        first = max((g - 1) * NC, WAITS + 1)
        for k, chunk in enumerate(spread(tasks[:8], g * NC - 1 - first)):
            extras[first + k] += chunk
        for k, chunk in enumerate(spread(tasks[8:], g * NC - 1 - first)):
            extras[first + k] += chunk
    late = range(min(WAITC, total - 3), total - 2)
    for s, chunk in zip(late, spread(wo_tasks(), len(late))):
        extras[s] += chunk

    for task in ln1_tasks(0):
        task(None)
    for g in range(NG):
        for s in range(g * NC, (g + 1) * NC):
            run_slot(s, PLAN if g else PLAN0, project_tasks(*divmod(s, NC)), extras[s], waits.get(s))

    def mod_part(i):
        def run():
            lhs = _unpack(released(pltpu.bitcast(sc, U32)))
            val["mod", i] = _rnd(_dot(lhs, wmod_buf[:, i * HD:(i + 1) * HD])[0:8])
        return run

    def late_mod():
        ga, sb, cb, gb = [jnp.concatenate([val["mod", 2 * i], val["mod", 2 * i + 1]], axis=1) for i in range(2, 6)]
        cb1 = _rnd(1.0 + cb)
        wr = jnp.broadcast_to(wr_buf[...].reshape(1, D).astype(F32), (8, D))
        for i, row in enumerate((ga * (1.0 / LOG2E), gb * cb1, gb * sb, cb1 * wr, cb1, sb, gb)):
            put(coef_buf, "coef")[i] = row
        val["r_add"] = jnp.sum(sb * wr, axis=-1, keepdims=True)
        deadline(NG * NC + lead, ORDER2[0], gb)

    def coef(i):
        return get(coef_buf, "coef")[i]

    lane8 = _iota((8, 128), 1)
    racc = [jnp.zeros((8, 128), F32)] * 2

    def attn_tasks(t, slot):
        def product(n):
            def run():
                assert all(("o", t, g) in holds for g in range(1, NG, 2))
                assert all(("wos", r, l) in holds for r in range(0, HD // 2, 16) for l in range(0, HD, WOC))
                rhs = meet(get(wos_buf, "wos")[n], (slot, n))
                val["last"] = val["a", t, n] = _dot(_unpack(o_bufs[t][n]), _unpack(rhs))
                if SYNC2:
                    for j in range(4):
                        at = 4 * (7 * t + ORDER2.index(n)) + j + SYNC2
                        deadline(slot - t + at // 28, ORDER2[at // 4 % 7], val["last"][HT - 8:, 128 * j:128 * j + 128], at % 4)
            return run
        return [product(n) for n in ORDER2]

    def epilogue_tasks(t, i):
        def piece(r):
            r0 = t * T + i * HT + r

            def residual():
                xs = []
                for e in (0, 8):
                    a = jnp.concatenate(
                        [_quadrant(lambda k: val["a", t, k][r + e:r + e + 8], i, j) for j in range(2)], axis=1)
                    xs.append(x_buf[0, r0 + e:r0 + e + 8, :].astype(F32) + coef(0) * a)
                    x1_buf[r0 + e:r0 + e + 8] = xs[-1]
                val["x1", r0] = xs, _row_means(xs)

            def centre():
                val["d", r0] = _row_spread(*val["x1", r0])

            def finish():
                (xs, means), (cen, var) = val["x1", r0], val["d", r0]
                scales = _row_scales(var)
                scale_buf[r0 // 2:r0 // 2 + 8] = scales
                outs = []
                for k in range(2):
                    rs = scales[:, k:k + 1]
                    mean_buf[r0 + 8 * k:r0 + 8 * k + 8] = jnp.broadcast_to(_rnd(means[k]), (8, 128))
                    outs.append(xs[k] + (cen[k] * rs * coef(1) + coef(2)))
                    score = jnp.sum(cen[k] * coef(3), axis=-1, keepdims=True) * rs
                    racc[r0 // 1024] = jnp.where(lane8 == (r0 // 8 + k) % 128, score, racc[r0 // 1024])
                put(out_bufs[t], "out")[r0 - t * T:r0 - t * T + 16, :] = jnp.concatenate(outs, axis=0).astype(BF16)
                return pltpu.bitcast(get(out_bufs[t], "out")[r0 - t * T:r0 - t * T + 16, 0:128], U32), racc[r0 // 1024]

            return residual, centre, finish
        return [piece(r) for r in range(0, HT, 16)]

    def ffn_inputs():
        cp_modb.wait()
        cp_wg.wait()
        cp_wu.wait()
        cp_wd.wait()

    ffn_inputs()
    mods = [mod_part(i) for i in range(4, 12)]
    for k, s in enumerate(range(total, total + lead)):
        run_slot(s, PLAND, [mods.pop(0) for _ in range(int(MODS[k]))], [])
    late_mod()

    stages = [piece for t in range(NT2) for i in (1, 0) for piece in epilogue_tasks(t, i)]
    steps = []
    for q in range(-2 * PIPE, len(stages)):
        t, k = divmod(q, 16)
        when = int(4 * (7 * t + EOFF + (EEND - EOFF) * (t + k / 16) / (NT2 - 1)) + k * 7 / 4)
        ahead = min(q + 2 * PIPE, len(stages) - 1)
        ready = 4 * (7 * (ahead // 16) + (5 if ahead % 16 < 8 else 7))
        steps.append((max(when, ready), q))

    def flush(upto, slot, n):
        while steps and steps[0][0] // 4 <= upto:
            when, q = steps.pop(0)
            for stage, lag in ((0, 2 * PIPE), (1, PIPE)):
                if 0 <= q + lag < len(stages):
                    stages[q + lag][stage]()
            if q < 0:
                continue
            done = stages[q][2]()
            if TIEE and n is not None:
                for dep in done:
                    deadline(slot, n, dep, when % 4 * FINE)
            if q % 16 == 15:
                t = q // 16
                out_copy(t).start()
                put(out_bufs[t], "out")[T:T + 16, 0:128] = jnp.zeros((16, 128), BF16)
                later = upto + DMALAG
                deadline(total + lead + later // 7, ORDER2[later % 7],
                         pltpu.bitcast(get(out_bufs[t], "out")[T:T + 16, 0:128], U32), 3)

    for t in range(NT2):
        slot = NG * NC + lead + t
        main = [lambda j=j, task=task: (flush(7 * t + j, slot, ORDER2[j]), task())
                for j, task in enumerate(attn_tasks(t, slot))]
        run_slot(slot, PLAN2, main, [])
    flush(8 * NT2 + 16, None, None)

    r = _rnd(jnp.concatenate(racc, axis=0) + jnp.concatenate([val["r_add"]] * 2, axis=0))
    r = jnp.clip(jnp.where(r != r, -BF16_MAX, r), -BF16_MAX, BF16_MAX)
    r = jnp.where(jnp.abs(r) < F32_TINY, F32_TINY, r)
    tok = (_iota((16, 128), 0) // 8) * 1024 + _iota((16, 128), 1) * 8 + _iota((16, 128), 0) % 8
    keys = pltpu.bitcast(pltpu.bitcast(r, jnp.int32) | jnp.where(r > 0, S - 1 - tok, tok), F32)
    picks = []
    for _ in range(2):
        top = jnp.max(jnp.max(keys, axis=0, keepdims=True), axis=1, keepdims=True)
        bits = pltpu.bitcast(jnp.broadcast_to(top, (8, 128)), jnp.int32)
        low = bits & (S - 1)
        picks.append((jnp.where(bits > 0, S - 1 - low, low), pltpu.bitcast(bits & -65536, F32)))
        keys = jnp.where(keys == top, -jnp.inf, keys)
    b1, b2 = [pl.multiple_of(jnp.clip(i[0, 0] // 16, 0, S // 16 - 1) * 16, 16) for i, _ in picks]

    def gather(ref):
        return jnp.concatenate([ref[pl.ds(b1, 16)], ref[pl.ds(b2, 16)]], axis=0)

    def wide(x):
        return jnp.concatenate([x] * (D // 128), axis=1)

    x1 = gather(x1_buf)
    scales = [scale_buf[pl.ds(pl.multiple_of(b // 2, 8), 8)] for b in (b1, b2)]
    rs = jnp.concatenate([sv[:, i:i + 1] for sv in scales for i in range(2)], axis=0)
    h2 = (x1 - wide(gather(mean_buf))) * rs * coef(4)[0:1] + coef(5)[0:1]
    hb = h2.astype(BF16)
    u = _dot(hb, wg_buf[...])
    act = u * jax.nn.sigmoid(u) * _dot(hb, wu_buf[...])
    y = _dot(act.astype(BF16), wd_buf[:, 0:D])
    rows = _iota((32, 128), 0)
    rows = jnp.where(rows < 16, rows + b1, rows - 16 + b2)
    update = jnp.zeros((32, D), F32)
    for i, score in picks:
        hit = wide(rows == jnp.concatenate([i] * 4, axis=0))
        update = jnp.where(hit, y * wide(jax.nn.sigmoid(score))[0:1], update)
    fix_buf[...] = (x1 + coef(6)[0:1] * (h2 + update)).astype(BF16)

    for t in range(NT2):
        out_copy(t).wait()
    fix1 = pltpu.make_async_copy(fix_buf.at[0:16], out_hbm.at[pl.ds(b1, 16)], sem.at[s_fix])
    fix2 = pltpu.make_async_copy(fix_buf.at[16:32], out_hbm.at[pl.ds(b2, 16)], sem.at[s_fix + 1])
    fix1.start()

    @pl.when(b1 != b2)
    def _():
        fix2.start()
        fix2.wait()

    fix1.wait()


@jax.jit
def pallas_adaLN_cond__linear_kernel_hedgehog__moe_arch_mod__prompt_kernel(
    A_x, A_wqkv, A_w_phi, A_wo, B_x, B_w_r, B_w_gate, B_w_up, B_w_down, c, w_mod,
):
    hbm = pl.BlockSpec(memory_space=pl.ANY)
    vm = pltpu.VMEM
    out = pl.pallas_call(
        _kernel,
        out_shape=jax.ShapeDtypeStruct((S, D), BF16),
        in_specs=[hbm] * 10,
        out_specs=hbm,
        scratch_shapes=[
            vm((1, S, D), BF16),
            vm((3, G, D, 128), BF16),
            vm((H, DH, DH), BF16),
            vm((D, D), BF16),
            vm((D,), BF16),
            vm((D, F), BF16),
            vm((D, F), BF16),
            vm((F, D + 128), BF16),
            vm((1, D), BF16),
            vm((D, 6 * D + 128), BF16),
            [vm((1, 7, HT // 2, HD), U32)] * NC,
            [vm((1, 7, 96, HD), U32)] * 3,
            [vm((1, NC, 2, 2, 64, 128), F32)] * 3,
            [vm((7, HT // 2, HD), U32)] * NC,
            vm((1, 7, HD // 2, HD), U32),
            vm((S, D), F32),
            vm((S, 128), F32),
            vm((S // 2, 128), F32),
            [vm((1, T + 16, D), BF16)] * NC,
            vm((1, 7, 8, D), F32),
            vm((32, D), BF16),
            pltpu.SemaphoreType.DMA((NC + 3 * G + 12 + NC + 2,)),
        ],
        compiler_params=pltpu.CompilerParams(vmem_limit_bytes=120 * 2**20),
        name="adaln_hedgehog_mod",
    )(A_x.reshape(S, D), A_wqkv, A_w_phi, A_wo, B_w_r, B_w_gate, B_w_up, B_w_down, c, w_mod)
    return out.reshape(1, S, D)
```

```python
import jax
import jax.numpy as jnp
from jax import lax
import jax.experimental.pallas as pl
import jax.experimental.pallas.tpu as pltpu


S, D, H, DH, F = 2048, 1024, 32, 32, 3584
G = 8
HD = D // 2
T = 256
HT = T // 2
NC = S // T
NG = G
NT2 = NC
TIEQ, TIER, TIEF, TIEE = 1, 3, 3, 1
KLAG, RLAG = 1, 1
PLAN0, WAITD = "wpppppppf", 0
ORDER = [int(c) for c in "3102546"]
PLAN = "pwkkqpqpqpqpqpqprqpqf"
ORDER2 = [int(c) for c in "1305246"]
PLAN2 = "wpkkpqpqpqpqprp"
WAITB, WAITC = 16, 23
EOFF = 9.0
OPAQUE = "wos,coef,out".split(",")
XW = "1,23,4,5,6,7,,".split(",")
WOLEAD = 0
SYNC1, SYNC2 = 0, 0
FINE = 0
EEND = 9.0
PIPE, DMALAG = 0, 2
AHEAD, WPHI, WW1 = "00011110", 3, 6
CHECKS = 1
PLANW = "pppkkpwpppqqqqqqrqqf"
PLANS = "pppwppppkkqqqqqqrqqf"
KOFF = 1
BFS = 0
PLAN00 = "ppppppwpf"
CAW = 256
WAITS, KRATE = 8, 2
F1, LNP, LASTP = 1, 2, 1
KEYLAG, WOC = 1, 128
PLAND, MODS = "kkqpppprpppp", "2231"
OPAQUEG = "none".split(",")
LNMODE = 0
BF16_MAX, F32_TINY = 3.3895313892515355e38, 1.1754943508222875e-38
LOG2E = 1.4426950408889634
NT = (((1,), (1,)), ((), ()))
NN = (((1,), (0,)), ((), ()))
F32, BF16, U32 = jnp.float32, jnp.bfloat16, jnp.uint32


def _dot(a, b, dims=NN):
    return lax.dot_general(a, b, dims, preferred_element_type=F32)


def _rnd(x):
    return x.astype(BF16).astype(F32)


def _pack(even, odd):
    return pltpu.pack_elementwise([even, odd], packed_dtype=BF16)


def _pack_halves(x):
    n = x.shape[0] // 2
    return _pack(x[:n], x[n:])


def _split(x):
    words = pltpu.bitcast(x, U32)
    return [pltpu.unpack_elementwise(words, index=i, packed_dtype=BF16, unpacked_dtype=F32) for i in range(2)]


def _unpack(x):
    return pltpu.bitcast(x, BF16)


def _interleave_halves(x):
    return _unpack(_pack_halves(x)).astype(F32) + _unpack(_pack_halves(x - _rnd(x))).astype(F32)


def _iota(shape, axis):
    return lax.broadcasted_iota(jnp.int32, shape, axis)


def _tree(x3, op):
    return op(op(op(x3[0], x3[1]), op(x3[2], x3[3])), op(op(x3[4], x3[5]), op(x3[6], x3[7])))


def _fold_rows(m, op):
    m = op(m, pltpu.roll(m, 2, 0))
    return op(m, pltpu.roll(m, 4, 0))


def _softmax2(p3, sign):
    if sign == 0:
        e = jnp.exp2(p3 - _fold_rows(_tree(p3, jnp.maximum), jnp.maximum)[None])
    else:
        e = jnp.exp2(_fold_rows(_tree(p3, jnp.minimum), jnp.minimum)[None] - p3)
    return e * pl.reciprocal(_fold_rows(_tree(e, jnp.add), jnp.add), full_range=False)[None]


def _row_means(xs):
    return [jnp.mean(x, axis=-1, keepdims=True) for x in xs]


def _row_spread(xs, means):
    lane = _iota((xs[0].shape[0], 128), 1)
    cen, var = [], None
    for i, (x, mean) in enumerate(zip(xs, means)):
        mr = _rnd(mean)
        d = x - mr
        v = jnp.mean(d * d, axis=-1, keepdims=True) - (mean - mr) * (mean - mr)
        var = jnp.where(lane == i, v, var) if i else jnp.broadcast_to(v, lane.shape)
        cen.append(d)
    return cen, var


def _row_scales(var):
    return 1.0 / _rnd(jnp.sqrt(_rnd(_rnd(var) + _rnd(jnp.full_like(var, 1e-5)))))


def _lhs_term(a, n):
    return (lambda: a(0, 0) + a(1, 1), lambda: a(1, 0) + a(1, 1), lambda: a(0, 0), lambda: a(1, 1),
            lambda: a(0, 0) + a(0, 1), lambda: a(1, 0) - a(0, 0), lambda: a(0, 1) - a(1, 1))[n]()


def _rhs_term(b, n):
    return (lambda: b(0, 0) + b(1, 1), lambda: b(0, 0), lambda: b(0, 1) - b(1, 1), lambda: b(1, 0) - b(0, 0),
            lambda: b(1, 1), lambda: b(0, 0) + b(0, 1), lambda: b(1, 0) + b(1, 1))[n]()


def _quadrant(m, i, j):
    if (i, j) == (0, 0):
        return (m(0) + m(3)) + (m(6) - m(4))
    if (i, j) == (0, 1):
        return m(2) + m(4)
    if (i, j) == (1, 0):
        return m(1) + m(3)
    return (m(0) - m(1)) + (m(2) + m(5))


def _kernel(x_hbm, wqkv_hbm, wphi_hbm, wo_hbm, wr_hbm, wg_hbm, wu_hbm, wd_hbm, c_hbm, wmod_hbm,
            out_hbm,
            x_buf, w_buf, wphi_buf, wo_buf, wr_buf, wg_buf, wu_buf, wd_buf, c_buf, wmod_buf,
            hs_bufs, ws_bufs, pq_bufs, o_bufs, wos_buf, x1_buf, mean_buf, scale_buf, out_bufs, coef_buf, fix_buf, sem):
    def x_rows(*chunks):
        return [(x_hbm.at[pl.ds(j * T, T)], x_buf.at[0, pl.ds(j * T, T)]) for j in chunks]

    def weights(*groups):
        return [(wqkv_hbm.at[:, pl.ds(i * D + g * 128, 128)], w_buf.at[i, g]) for g in groups for i in range(3)]

    def mod_cols(lo, n):
        return [(wmod_hbm.at[:, pl.ds(lo, n)], wmod_buf.at[:, pl.ds(lo, n)])]

    batches = {
        "start": [(c_hbm, c_buf), (wphi_hbm.at[0:4], wphi_buf.at[0:4])] + weights(0) + x_rows(0),
        **{("scale", k): mod_cols(D + k, CAW) + mod_cols(D + HD + k, CAW) for k in range(0, HD, CAW)},
        0: x_rows(1),
        1: x_rows(2),
        2: x_rows(3, 4),
        3: x_rows(5) + [(wphi_hbm.at[4:H], wphi_buf.at[4:H])],
        4: x_rows(6),
        5: x_rows(7),
        6: weights(1),
        WAITS: mod_cols(0, D) + weights(2, 3),
        min(WAITC, NG * NC - 2): weights(*range(4, G)) + [(wr_hbm, wr_buf), (wo_hbm, wo_buf)],
        NG * NC - 1: mod_cols(2 * D, 4 * D) + [(wg_hbm, wg_buf), (wu_hbm, wu_buf), (wd_hbm, wd_buf.at[:, 0:D])],
    }
    batches = {name: [pltpu.make_async_copy(src, dst, sem.at[i]) for src, dst in pairs]
               for i, (name, pairs) in enumerate(batches.items())}
    sem_out = sem.at[len(batches)]
    for copies in batches.values():
        for cp in copies:
            cp.start()

    def arrive(name):
        for cp in batches.pop(name):
            cp.wait()

    def out_copy(t):
        return pltpu.make_async_copy(out_bufs[t].at[0, 0:T], out_hbm.at[pl.ds(t * T, T)], sem_out)

    z_put, z_get = [jnp.min(_iota((8, 128), axis)) for axis in range(2)]
    never = _iota((8, 128), 1) < z_get
    val, due, holds = {}, {}, {}

    def put(ref, kind=""):
        return ref.at[z_put if kind in OPAQUE else 0]

    def get(ref, kind=""):
        return ref.at[z_get if kind in OPAQUEG else 0]

    def after(x, dep, r=0):
        head = jnp.where(never, pltpu.bitcast(dep[0:8, 0:128], x.dtype), x[r:r + 8, 0:128])
        if x.shape[1] > 128:
            head = jnp.concatenate([head, x[r:r + 8, 128:]], axis=1)
        parts = ([x[:r]] if r else []) + [head] + ([x[r + 8:]] if x.shape[0] > r + 8 else [])
        return jnp.concatenate(parts, axis=0)

    def released(x, tie=1):
        return after(x, val["last"]) if tie and "last" in val else x

    def meet(x, key):
        cols = [x[:, l:l + 128] for l in range(0, x.shape[1], 128)]
        for j in range(len(cols)):
            for i, dep in enumerate(due.pop((*key, j), [])):
                cols[j] = after(cols[j], dep, 8 * i)
        return jnp.concatenate(cols, axis=1)

    def deadline(slot, n, dep, j=0):
        due.setdefault((slot, n, j), []).append(dep)

    same_head = _iota((128, 128), 0) // DH == _iota((128, 128), 1) // DH
    sel = (_iota((128, DH), 0) % DH == _iota((128, DH), 1)).astype(BF16)
    kv_mask = _iota((64, 128), 0) % 2 == (_iota((64, 128), 1) // 2) % 2

    def bias_part(g, i, k):
        left, right = val["folded", g, i, k]
        term = (left.reshape(16, 8, 128) * val["sa"][:, k:k + 128][None]
                + right.reshape(16, 8, 128) * val["sa"][:, HD + k:HD + k + 128][None])
        val["bias", g, i] = term if k == 0 else val["bias", g, i] + term
        if k == HD - 128:
            b = jnp.broadcast_to(jnp.sum(val["bias", g, i], axis=-1, keepdims=True), (16, 8, 128)).reshape(128, 128)
            for p in range(2):
                val["bias", g, i, p] = _interleave_halves(b[64 * p:64 * p + 64])

    def fold_tasks(g):
        def part(i, k):
            def run(slot):
                halves = []
                for lo in (k, HD + k):
                    w = _unpack(released(pltpu.bitcast(w_buf[i, g, lo:lo + 128, :], U32), TIEF))
                    halves.append(_dot(val["mix", g].astype(BF16), w, NT) if i < 2 else w.astype(F32).T)
                val["folded", g, i, k] = halves
                if g > 1:
                    bias_part(g, i, k)
                for n in range(7):
                    words = _pack_halves(_lhs_term(lambda p, j: halves[j][64 * p:64 * p + 64], n))
                    put(ws_bufs[g % 3], "ws")[n, 32 * i:32 * i + 32, k:k + 128] = words
                holds["ws", g % 3, i, k] = g
                if TIEF and slot is not None:
                    deadline(slot + TIEF, 1 + k // 128, words)
            return run

        return [part(i, k) for i in range(3) for k in range(0, HD, 128)]

    def ln1_means(c, r):
        rows = [slice(c * T + n * HT + r, c * T + n * HT + r + 16) for n in range(2)]
        xs = [x for n in range(2) for x in _split(x_buf[0, rows[n], :])]
        val["ln", c, r] = xs, _row_means(xs)

    def ln1_spread(c, r):
        val["ln", c, r] = _row_spread(*val["ln", c, r])

    def ln1_scales(c, r):
        cen, var = val["ln", c, r]
        rs = _row_scales(var)
        val["ln", c, r] = [(d, rs[:, i:i + 1]) for i, d in enumerate(cen)]

    def ln1_stats(c, r):
        for stage, lag in ((ln1_means, 0), (ln1_spread, 16), (ln1_scales, 32)):
            if 0 <= r - lag < HT:
                stage(c, r - lag)

    def ln1_terms(c, r, k):
        h = {}
        for j in range(2):
            cols = slice(j * HD + k, j * HD + k + 128)
            for n in range(2):
                for e in range(2):
                    d, rs = val["ln", c, r][2 * n + e]
                    h[e, j, n] = d[:, cols] * rs * val["ca1", j * HD + k]
        for n in range(7):
            hs_bufs[c][0, n, r // 2:r // 2 + 8, k:k + 128] = _pack(
                *[_rhs_term(lambda j, m: h[e, j, m], n) for e in range(2)])
        holds["hs", c, r, k] = True

    def mix(g):
        wp = wphi_buf[g * 4:g * 4 + 4].reshape(128, DH)
        val["mix", g] = jnp.where(same_head, _dot(sel, wp, NT), 0.0)

    arrive("start")
    mix(0)
    for task in fold_tasks(0):
        task(None)
    cv = c_buf[...].astype(F32)
    sc = jnp.broadcast_to(_rnd(cv * _rnd(jax.nn.sigmoid(cv))), (16, D)).astype(BF16)
    for r in range(0, HT + 32, 16):
        ln1_stats(0, r)
    for i, k in enumerate(range(0, HD, CAW)):
        arrive(("scale", k))
        for j in range(2):
            lo = j * HD + k
            block = _rnd(1.0 + _rnd(_dot(sc, wmod_buf[:, D + lo:D + lo + CAW])[0:8])) * LOG2E
            for l in range(0, CAW, 128):
                val["ca1", lo + l] = block[:, l:l + 128]
        for r in range(0, HT, 16):
            for l in range(k, k + CAW, 128):
                ln1_terms(0, r, l)

    staged = set()

    def ln1_tasks(c):
        def piece(r):
            def run(slot):
                if r == 0 and (c, 0) not in staged:
                    staged.add((c, 0))
                    for step in range(0, HT + 32, 16):
                        ln1_stats(c, step)
                if AHEAD[c] == "1":
                    staged.add((c + 1, 0))
                    for step in range(r, r + (48 if r == HT - 16 else 16), 16):
                        ln1_stats(c + 1, step)
                        if step >= 32:
                            scale = val["ln", c + 1, step - 32][3][1]
                            deadline(slot + 1, ORDER[step // 16 % LNP], jnp.broadcast_to(scale, (8, 128)))
                for k in range(0, HD, 128):
                    ln1_terms(c, r, k)
            return run
        return [piece(r) for r in range(0, HT, 16)]

    def project_tasks(g, c):
        def product(n):
            def run():
                assert all(holds["ws", g % 3, i, k] == g for i in range(3) for k in range(0, HD, 128))
                assert all(("hs", c, r, k) in holds for r in range(0, HT, 16) for k in range(0, HD, 128))
                rhs = meet(get(hs_bufs[c])[n], (g * NC + c, n))
                val["last"] = val["m", g * NC + c, n] = _dot(_unpack(get(ws_bufs[g % 3], "ws")[n]), _unpack(rhs), NT)
                at = 7 * (g * NC + c) + ORDER.index(n) + SYNC1
                if SYNC1 and at < 7 * NG * NC:
                    deadline(at // 7, ORDER[at % 7], val["last"][184:192], 3)
            return run
        return [product(n) for n in ORDER]

    def key_tasks(g, c):
        def piece(p, n):
            def run():
                def part(i):
                    y = _quadrant(lambda k: val["m", g * NC + c, k][64 * i:64 * i + 64], p, n)
                    return y + val["bias", g, i, p] if i < 2 else y
                put(pq_bufs[g % 3])[c, p, n] = part(0)
                holds["pq", g % 3, c, p, n] = g
                val["v", g, c, p, n] = part(2)
                logits = part(1).reshape(8, 8, 128)
                words = []
                for s in range(2):
                    phi = _softmax2(logits, s)
                    words.append(_pack_halves(phi.reshape(64, 128)))
                    val["z", g, p, s] = val["z", g, p, s] + phi if ("z", g, p, s) in val else phi
                val["phik", g, c, p, n] = jnp.concatenate(words, axis=0)
            return run
        return [piece(p, n) for p, n in ((1, 0), (0, 1), (1, 1), (0, 0))]

    def summary_tasks(g, c):
        def piece(p):
            def run():
                v = jnp.concatenate([val["v", g, c, p, n] for n in range(2)], axis=1).astype(BF16)
                phi = _unpack(jnp.concatenate([val["phik", g, c, p, n] for n in range(2)], axis=1))
                kv = _dot(v, phi, NT)
                val["kv", g, p] = kv if c == 0 else val["kv", g, p] + kv
                if c == NC - 1:
                    for s in range(2):
                        z = jnp.sum(val["z", g, p, s], axis=-1, keepdims=True)
                        val["zb", g, p, s] = jnp.broadcast_to(z, (8, 8, 128))
                    z_row = jnp.concatenate(
                        [_interleave_halves(val["zb", g, p, s].reshape(64, 128)) for s in range(2)], axis=0).T[0:64]
                    val["kv", g, p] = jnp.where(kv_mask, val["kv", g, p] + val["bias", g, 2, p] * z_row, 0.0)
            return run
        return [piece(p) for p in range(2)]

    def query_tasks(g, c):
        def piece(p, n):
            def run():
                assert holds["pq", g % 3, c, p, n] == g
                logits = released(get(pq_bufs[g % 3])[c, p, n], TIEQ).reshape(8, 8, 128)
                words, den = [], None
                for s in range(2):
                    phi = _softmax2(logits, s)
                    words.append(_pack_halves(phi.reshape(64, 128)))
                    w = _tree(phi * val["zb", g, p, s], jnp.add)
                    den = w if den is None else den + w
                val["iden", g, c, p, n] = pl.reciprocal(_fold_rows(den, jnp.add) + 1e-6, full_range=False)
                val["phiq", g, c, p, n] = jnp.concatenate(words, axis=0)
            return run
        return [piece(p, n) for n in range(2) for p in range(2)]

    def readout(g, c, slot):
        nums = [_dot(val["kv", g, p].astype(BF16),
                     _unpack(jnp.concatenate([val["phiq", g, c, p, n] for n in range(2)], axis=1)))
                for p in range(2)]
        for p in range(2):
            for n in range(2):
                num = nums[p][:, n * HT:(n + 1) * HT].reshape(8, 8, 128)
                val["o", g, c, n, p] = (num * val["iden", g, c, p, n][None]).reshape(64, 128)
        if g % 2:
            for k in range(7):
                term = _lhs_term(
                    lambda n, p: jnp.concatenate([val["o", g - 1, c, n, p], val["o", g, c, n, p]], axis=0), k)
                words = pltpu.bitcast(term.astype(BF16).T, U32)
                o_bufs[c][k, :, 64 * (g - 1):64 * (g + 1)] = words
                holds["o", c, g] = True
                if TIER:
                    deadline(slot + TIER, k, words[56:64])
        elif TIER:
            for k, (n, p) in enumerate(((0, 0), (0, 1), (1, 0), (1, 1))):
                deadline(slot + TIER, k, val["o", g, c, n, p][56:64])

    def wo_tasks():
        def piece(r, l):
            def run(slot):
                src = r // DH * 128 + r % DH
                quads = {}
                for e in range(2):
                    for i in range(2):
                        lo = src + i * 64 + DH * e
                        for j in range(2):
                            w = wo_buf[lo:lo + 16, j * HD + l:j * HD + l + WOC].astype(F32)
                            quads[e, i, j] = released(w, TIEF)
                for n in range(7):
                    words = _pack(*[_rhs_term(lambda i, j: quads[e, i, j], n) for e in range(2)])
                    put(wos_buf, "wos")[n, r:r + 16, l:l + WOC] = words
                holds["wos", r, l] = True
                if TIEF:
                    deadline(slot + TIEF, (r // 16 + l // 128) % 7, get(wos_buf, "wos")[0, r:r + 8, l:l + 128])
            return run
        return [piece(r, l) for r in range(0, HD // 2, 16) for l in range(0, HD, WOC)]

    def spread(tasks, n):
        return [tasks[i * len(tasks) // n:(i + 1) * len(tasks) // n] for i in range(n)]

    total = NG * NC
    lead = KEYLAG + KLAG + RLAG + 1
    agenda = {}

    def book(kind, s, item):
        agenda.setdefault((kind, s), []).append(item)

    def key_slot(u):
        return max(u + KEYLAG, WAITS + KOFF + u // KRATE)

    for u in range(total):
        g, c = divmod(u, NC)
        s_key = key_slot(u)
        ready = key_slot(g * NC + NC - 1) + KLAG + 1
        first = key_slot(NC - 1) + KLAG + 1
        s_query = max(first + u * (total + KEYLAG + KLAG + NC - first) // total, ready)
        s_query = min(s_query, total + lead + c - RLAG - 1)
        assert s_query >= ready
        book("key", s_key, (g, c))
        book("sum", s_key + KLAG, (g, c))
        book("query", s_query, (g, c))
        book("read", s_query + RLAG, (g, c))

    def run_slot(s, plan, main, extra, wait=None):
        keys = [t for gc in agenda.get(("key", s), []) for t in key_tasks(*gc)]
        queries = [t for gc in agenda.get(("query", s), []) for t in query_tasks(*gc)]
        mixed = sorted([((i + 0.5) / len(keys), 0, i) for i in range(len(keys))]
                       + [((i + 0.5) / len(queries), 1, i) for i in range(len(queries))])
        pieces = spread([(keys, queries)[kind][i] for _, kind, i in mixed], plan.count("q"))
        sums = spread([t for gc in agenda.get(("sum", s), []) for t in summary_tasks(*gc)], plan.count("k"))
        main = list(main)
        for step in plan:
            if step == "p" and main:
                main.pop(0)()
            elif step in "qk":
                for task in (pieces if step == "q" else sums).pop(0):
                    task()
            elif step == "r":
                for gc in agenda.get(("read", s), []):
                    readout(*gc, s)
            elif step == "f":
                for task in extra:
                    task(s)
            elif step == "w" and wait:
                wait()

    def shift():
        arrive(WAITS)
        val["sa"] = _rnd(_dot(sc, wmod_buf[:, 0:D])[0:8]) * LOG2E

    waits = {s: (lambda s=s: arrive(s)) for s in batches if isinstance(s, int)}
    waits[WAITS] = shift

    extras = {s: [] for s in range(total)}
    for c in range(NC - 1):
        extras[c] += ln1_tasks(c + 1)
    extras[3] += [lambda s, g=g: mix(g) for g in range(1, 5)]
    extras[4] += [lambda s, g=g: mix(g) for g in range(5, G)]
    for k, chunk in enumerate(spread(fold_tasks(1), 3)):
        extras[NC - 2 + (k > 0)] += chunk
    for g, slots in enumerate(([WAITS], range(WAITS + 1, WAITS + 4))):
        tasks = [lambda s, g=g, i=i, k=k: bias_part(g, i, k) for i in range(3) for k in range(0, HD, 128)]
        for s, chunk in zip(slots, spread(tasks, len(slots))):
            extras[s] += chunk
    for g in range(2, NG):
        tasks = fold_tasks(g)
        first = max((g - 1) * NC, WAITS + 1)
        for k, chunk in enumerate(spread(tasks[:8], g * NC - 1 - first)):
            extras[first + k] += chunk
        for k, chunk in enumerate(spread(tasks[8:], g * NC - 1 - first)):
            extras[first + k] += chunk
    late = range(min(WAITC, total - 3), total - 2)
    for s, chunk in zip(late, spread(wo_tasks(), len(late))):
        extras[s] += chunk

    for g in range(NG):
        for s in range(g * NC, (g + 1) * NC):
            run_slot(s, (PLANS if s == WAITS else PLANW if s in waits else PLAN) if g else PLAN0 if s else PLAN00, project_tasks(*divmod(s, NC)), extras[s], waits.get(s))

    def mod_part(i):
        def run():
            lhs = _unpack(released(pltpu.bitcast(sc, U32)))
            val["mod", i] = _rnd(_dot(lhs, wmod_buf[:, i * HD:(i + 1) * HD])[0:8])
        return run

    def late_mod():
        ga, sb, cb, gb = [jnp.concatenate([val["mod", 2 * i], val["mod", 2 * i + 1]], axis=1) for i in range(2, 6)]
        cb1 = _rnd(1.0 + cb)
        wr = jnp.broadcast_to(wr_buf[...].reshape(1, D).astype(F32), (8, D))
        for i, row in enumerate((ga * (1.0 / LOG2E), gb * cb1, gb * sb, cb1 * wr, cb1, sb, gb)):
            put(coef_buf, "coef")[i] = row
        val["r_add"] = jnp.sum(sb * wr, axis=-1, keepdims=True)
        deadline(NG * NC + lead, ORDER2[0], gb)

    def coef(i):
        return get(coef_buf, "coef")[i]

    lane8 = _iota((8, 128), 1)
    racc = [jnp.zeros((8, 128), F32)] * 2

    def attn_tasks(t, slot):
        def product(n):
            def run():
                assert all(("o", t, g) in holds for g in range(1, NG, 2))
                assert all(("wos", r, l) in holds for r in range(0, HD // 2, 16) for l in range(0, HD, WOC))
                rhs = meet(get(wos_buf, "wos")[n], (slot, n))
                val["last"] = val["a", t, n] = _dot(_unpack(o_bufs[t][n]), _unpack(rhs))
                if SYNC2:
                    for j in range(4):
                        at = 4 * (7 * t + ORDER2.index(n)) + j + SYNC2
                        deadline(slot - t + at // 28, ORDER2[at // 4 % 7], val["last"][HT - 8:, 128 * j:128 * j + 128], at % 4)
            return run
        return [product(n) for n in ORDER2]

    def epilogue_tasks(t, i):
        def piece(r):
            r0 = t * T + i * HT + r

            def residual():
                xs = []
                for e in (0, 8):
                    a = jnp.concatenate(
                        [_quadrant(lambda k: val["a", t, k][r + e:r + e + 8], i, j) for j in range(2)], axis=1)
                    xs.append(x_buf[0, r0 + e:r0 + e + 8, :].astype(F32) + coef(0) * a)
                    x1_buf[r0 + e:r0 + e + 8] = xs[-1]
                val["x1", r0] = xs, _row_means(xs)

            def centre():
                val["d", r0] = _row_spread(*val["x1", r0])

            def finish():
                (xs, means), (cen, var) = val["x1", r0], val["d", r0]
                scales = _row_scales(var)
                scale_buf[r0 // 2:r0 // 2 + 8] = scales
                outs = []
                for k in range(2):
                    rs = scales[:, k:k + 1]
                    mean_buf[r0 + 8 * k:r0 + 8 * k + 8] = jnp.broadcast_to(_rnd(means[k]), (8, 128))
                    outs.append(xs[k] + (cen[k] * rs * coef(1) + coef(2)))
                    score = jnp.sum(cen[k] * coef(3), axis=-1, keepdims=True) * rs
                    racc[r0 // 1024] = jnp.where(lane8 == (r0 // 8 + k) % 128, score, racc[r0 // 1024])
                put(out_bufs[t], "out")[r0 - t * T:r0 - t * T + 16, :] = jnp.concatenate(outs, axis=0).astype(BF16)
                return pltpu.bitcast(get(out_bufs[t], "out")[r0 - t * T:r0 - t * T + 16, 0:128], U32), racc[r0 // 1024]

            return residual, centre, finish
        return [piece(r) for r in range(0, HT, 16)]

    mods = [mod_part(i) for i in range(4, 12)]
    for k, s in enumerate(range(total, total + lead)):
        run_slot(s, PLAND, [mods.pop(0) for _ in range(int(MODS[k]))], [])
    late_mod()

    stages = [piece for t in range(NT2) for i in (1, 0) for piece in epilogue_tasks(t, i)]
    steps = []
    for q in range(-2 * PIPE, len(stages)):
        t, k = divmod(q, 16)
        when = int(4 * (7 * t + EOFF + (EEND - EOFF) * (t + k / 16) / (NT2 - 1)) + k * 7 / 4)
        ahead = min(q + 2 * PIPE, len(stages) - 1)
        ready = 4 * (7 * (ahead // 16) + (5 if ahead % 16 < 8 else 7))
        steps.append((max(when, ready), q))

    def flush(upto, slot, n):
        while steps and steps[0][0] // 4 <= upto:
            when, q = steps.pop(0)
            for stage, lag in ((0, 2 * PIPE), (1, PIPE)):
                if 0 <= q + lag < len(stages):
                    stages[q + lag][stage]()
            if q < 0:
                continue
            done = stages[q][2]()
            if TIEE and n is not None:
                for dep in done:
                    deadline(slot, n, dep, when % 4 * FINE)
            if q % 16 == 15:
                t = q // 16
                out_copy(t).start()
                put(out_bufs[t], "out")[T:T + 16, 0:128] = jnp.zeros((16, 128), BF16)
                later = upto + DMALAG
                deadline(total + lead + later // 7, ORDER2[later % 7],
                         pltpu.bitcast(get(out_bufs[t], "out")[T:T + 16, 0:128], U32), 3)

    for t in range(NT2):
        slot = NG * NC + lead + t
        main = [lambda j=j, task=task: (flush(7 * t + j, slot, ORDER2[j]), task())
                for j, task in enumerate(attn_tasks(t, slot))]
        run_slot(slot, PLAN2, main, [])
    if BFS:
        rest = [q for _, q in steps]
        for lo in range(0, len(rest), BFS):
            for stage in range(3):
                for q in rest[lo:lo + BFS]:
                    stages[q][stage]()
                    if stage == 2 and q % 16 == 15:
                        out_copy(q // 16).start()
    else:
        flush(8 * NT2 + 16, None, None)

    r = _rnd(jnp.concatenate(racc, axis=0) + jnp.concatenate([val["r_add"]] * 2, axis=0))
    r = jnp.clip(jnp.where(r != r, -BF16_MAX, r), -BF16_MAX, BF16_MAX)
    r = jnp.where(jnp.abs(r) < F32_TINY, F32_TINY, r)
    tok = (_iota((16, 128), 0) // 8) * 1024 + _iota((16, 128), 1) * 8 + _iota((16, 128), 0) % 8
    keys = pltpu.bitcast(pltpu.bitcast(r, jnp.int32) | jnp.where(r > 0, S - 1 - tok, tok), F32)
    picks = []
    for _ in range(2):
        top = jnp.max(jnp.max(keys, axis=0, keepdims=True), axis=1, keepdims=True)
        bits = pltpu.bitcast(jnp.broadcast_to(top, (8, 128)), jnp.int32)
        low = bits & (S - 1)
        picks.append((jnp.where(bits > 0, S - 1 - low, low), pltpu.bitcast(bits & -65536, F32)))
        keys = jnp.where(keys == top, -jnp.inf, keys)
    b1, b2 = [pl.multiple_of(jnp.clip(i[0, 0] // 16, 0, S // 16 - 1) * 16, 16) for i, _ in picks]

    def gather(ref):
        return jnp.concatenate([ref[pl.ds(b1, 16)], ref[pl.ds(b2, 16)]], axis=0)

    def wide(x):
        return jnp.concatenate([x] * (D // 128), axis=1)

    x1 = gather(x1_buf)
    scales = [scale_buf[pl.ds(pl.multiple_of(b // 2, 8), 8)] for b in (b1, b2)]
    rs = jnp.concatenate([sv[:, i:i + 1] for sv in scales for i in range(2)], axis=0)
    h2 = (x1 - wide(gather(mean_buf))) * rs * coef(4)[0:1] + coef(5)[0:1]
    hb = h2.astype(BF16)
    u = _dot(hb, wg_buf[...])
    act = u * jax.nn.sigmoid(u) * _dot(hb, wu_buf[...])
    y = _dot(act.astype(BF16), wd_buf[:, 0:D])
    rows = _iota((32, 128), 0)
    rows = jnp.where(rows < 16, rows + b1, rows - 16 + b2)
    update = jnp.zeros((32, D), F32)
    for i, score in picks:
        hit = wide(rows == jnp.concatenate([i] * 4, axis=0))
        update = jnp.where(hit, y * wide(jax.nn.sigmoid(score))[0:1], update)
    fix_buf[...] = (x1 + coef(6)[0:1] * (h2 + update)).astype(BF16)

    assert not batches
    for t in range(NT2):
        out_copy(t).wait()
    fix1 = pltpu.make_async_copy(fix_buf.at[0:16], out_hbm.at[pl.ds(b1, 16)], sem_out)
    fix2 = pltpu.make_async_copy(fix_buf.at[16:32], out_hbm.at[pl.ds(b2, 16)], sem_out)
    fix1.start()

    @pl.when(b1 != b2)
    def _():
        fix2.start()
        fix2.wait()

    fix1.wait()


@jax.jit
def pallas_adaLN_cond__linear_kernel_hedgehog__moe_arch_mod__prompt_kernel(
    A_x, A_wqkv, A_w_phi, A_wo, B_x, B_w_r, B_w_gate, B_w_up, B_w_down, c, w_mod,
):
    hbm = pl.BlockSpec(memory_space=pl.ANY)
    vm = pltpu.VMEM
    out = pl.pallas_call(
        _kernel,
        out_shape=jax.ShapeDtypeStruct((S, D), BF16),
        in_specs=[hbm] * 10,
        out_specs=hbm,
        scratch_shapes=[
            vm((1, S, D), BF16),
            vm((3, G, D, 128), BF16),
            vm((H, DH, DH), BF16),
            vm((D, D), BF16),
            vm((D,), BF16),
            vm((D, F), BF16),
            vm((D, F), BF16),
            vm((F, D + 128), BF16),
            vm((1, D), BF16),
            vm((D, 6 * D + 128), BF16),
            [vm((1, 7, HT // 2, HD), U32)] * NC,
            [vm((1, 7, 96, HD), U32)] * 3,
            [vm((1, NC, 2, 2, 64, 128), F32)] * 3,
            [vm((7, HT // 2, HD), U32)] * NC,
            vm((1, 7, HD // 2, HD), U32),
            vm((S, D), F32),
            vm((S, 128), F32),
            vm((S // 2, 128), F32),
            [vm((1, T + 16, D), BF16)] * NC,
            vm((1, 7, 8, D), F32),
            vm((32, D), BF16),
            pltpu.SemaphoreType.DMA((12 + HD // CAW,)),
        ],
        compiler_params=pltpu.CompilerParams(vmem_limit_bytes=120 * 2**20, disable_bounds_checks=CHECKS < 1, disable_semaphore_checks=CHECKS < 0),
        name="adaln_hedgehog_mod",
    )(A_x.reshape(S, D), A_wqkv, A_w_phi, A_wo, B_w_r, B_w_gate, B_w_up, B_w_down, c, w_mod)
    return out.reshape(1, S, D)
```

```python
import numpy as np

import jax
import jax.numpy as jnp
from jax import lax
import jax.experimental.pallas as pl
import jax.experimental.pallas.tpu as pltpu

S, D, H, DH, F = 2048, 1024, 32, 32, 3584
G = 8
HD = D // 2
T = 256
HT = T // 2
NC = S // T

LOG2E = float(np.log2(np.e))
BF16_MAX = 3.3895313892515355e38
F32_TINY = float(np.finfo(np.float32).tiny)
NT = (((1,), (1,)), ((), ()))
NN = (((1,), (0,)), ((), ()))
F32, BF16, U32 = jnp.float32, jnp.bfloat16, jnp.uint32

LEAD_IN = [int(g) for g in "0000010101011111"]
SLOTS = [(g, LEAD_IN[:i].count(g)) for i, g in enumerate(LEAD_IN)] + [(g, c) for g in range(2, G) for c in range(NC)]
SLOT = {gc: s for s, gc in enumerate(SLOTS)}
PRODUCTS = (3, 1, 0, 2, 5, 4, 6)
SHIFT_SLOT, FOLD_SLOT, LATE_SLOT = 7, 10, 23
TILE_SLOT = len(SLOTS) + 4
SCALE_COLS, WO_COLS = 256, 256
SLACK = 3
EPILOGUE_LAG = 9

PLAN_FIRST, PLAN_STREAM = "ppppppwpf", "wpppppppf"
PLAN_SHIFT, PLAN_WAIT = "pppwppppkkqqqqqqrqqf", "pppkkpwpppqqqqqqrqqf"
PLAN_STEADY = "pwkkqpqpqpqpqpqprqpqf"
PLAN_DRAIN, PLAN_TILE = "kkqpppprpppp", "pkkpqpqpqpqprp"


def _dot(a, b, dims=NN):
    return lax.dot_general(a, b, dims, preferred_element_type=F32)


def _rnd(x):
    return x.astype(BF16).astype(F32)


def _iota(shape, axis):
    return lax.broadcasted_iota(jnp.int32, shape, axis)


def _pack(even, odd):
    return pltpu.pack_elementwise([even, odd], packed_dtype=BF16)


def _pack_halves(x):
    n = x.shape[0] // 2
    return _pack(x[:n], x[n:])


def _unpack(words):
    return pltpu.bitcast(words, BF16)


def _split(x):
    words = pltpu.bitcast(x, U32)
    return [pltpu.unpack_elementwise(words, index=i, packed_dtype=BF16, unpacked_dtype=F32) for i in range(2)]


def _interleave_halves(x):
    return _unpack(_pack_halves(x)).astype(F32) + _unpack(_pack_halves(x - _rnd(x))).astype(F32)


def _tree(x3, op):
    return op(op(op(x3[0], x3[1]), op(x3[2], x3[3])), op(op(x3[4], x3[5]), op(x3[6], x3[7])))


def _fold_rows(m, op):
    m = op(m, pltpu.roll(m, 2, 0))
    return op(m, pltpu.roll(m, 4, 0))


def _softmax2(p3, sign):
    if sign == 0:
        e = jnp.exp2(p3 - _fold_rows(_tree(p3, jnp.maximum), jnp.maximum)[None])
    else:
        e = jnp.exp2(_fold_rows(_tree(p3, jnp.minimum), jnp.minimum)[None] - p3)
    return e * pl.reciprocal(_fold_rows(_tree(e, jnp.add), jnp.add), full_range=False)[None]


def _row_means(xs):
    return [jnp.mean(x, axis=-1, keepdims=True) for x in xs]


def _row_spread(xs, means):
    lane = _iota((xs[0].shape[0], 128), 1)
    centred, var = [], None
    for i, (x, mean) in enumerate(zip(xs, means)):
        rounded = _rnd(mean)
        d = x - rounded
        v = jnp.mean(d * d, axis=-1, keepdims=True) - (mean - rounded) * (mean - rounded)
        var = jnp.where(lane == i, v, var) if i else jnp.broadcast_to(v, lane.shape)
        centred.append(d)
    return centred, var


def _row_scales(var):
    return 1.0 / _rnd(jnp.sqrt(_rnd(_rnd(var) + _rnd(jnp.full_like(var, 1e-5)))))


def _lhs_term(a, n):
    return (lambda: a(0, 0) + a(1, 1), lambda: a(1, 0) + a(1, 1), lambda: a(0, 0), lambda: a(1, 1),
            lambda: a(0, 0) + a(0, 1), lambda: a(1, 0) - a(0, 0), lambda: a(0, 1) - a(1, 1))[n]()


def _rhs_term(b, n):
    return (lambda: b(0, 0) + b(1, 1), lambda: b(0, 0), lambda: b(0, 1) - b(1, 1), lambda: b(1, 0) - b(0, 0),
            lambda: b(1, 1), lambda: b(0, 0) + b(0, 1), lambda: b(1, 0) + b(1, 1))[n]()


def _quadrant(m, i, j):
    if (i, j) == (0, 0):
        return (m(0) + m(3)) + (m(6) - m(4))
    if (i, j) == (0, 1):
        return m(2) + m(4)
    if (i, j) == (1, 0):
        return m(1) + m(3)
    return (m(0) - m(1)) + (m(2) + m(5))


def _spread(tasks, n):
    return [tasks[i * len(tasks) // n:(i + 1) * len(tasks) // n] for i in range(n)]


def _agenda():
    total, agenda = len(SLOTS), {}

    def key_slot(s):
        return max(s + 1, SHIFT_SLOT + 2 + s // 2)

    def ready(g):
        return key_slot(SLOT[g, NC - 1]) + 2

    for s, gc in enumerate(SLOTS):
        agenda.setdefault(("key", key_slot(s)), []).append(gc)
        agenda.setdefault(("sum", key_slot(s) + 1), []).append(gc)
    for u in range(total):
        g, c = divmod(u, NC)
        s = min(max(ready(0) + u * (total + 2 + NC - ready(0)) // total, ready(g)), TILE_SLOT + c - 2)
        assert s >= ready(g)
        agenda.setdefault(("query", s), []).append((g, c))
        agenda.setdefault(("read", s + 1), []).append((g, c))
    return agenda


def _kernel(x_hbm, wqkv_hbm, wphi_hbm, wo_hbm, wr_hbm, wg_hbm, wu_hbm, wd_hbm, c_hbm, wmod_hbm,
            out_hbm,
            x_buf, w_buf, wphi_buf, wo_buf, wr_buf, wg_buf, wu_buf, wd_buf, c_buf, wmod_buf,
            h_terms, w_terms, pq_bufs, o_terms, wo_terms, x1_buf, mean_buf, scale_buf, out_bufs, coef_buf,
            fix_buf, sem):
    def x_rows(j):
        return [(x_hbm.at[pl.ds(j * T, T)], x_buf.at[pl.ds(j * T, T)])]

    def weights(*groups):
        return [(wqkv_hbm.at[:, pl.ds(i * D + g * 128, 128)], w_buf.at[i, g]) for g in groups for i in range(3)]

    def mod_cols(lo, n):
        return [(wmod_hbm.at[:, pl.ds(lo, n)], wmod_buf.at[:, pl.ds(lo, n)])]

    early = {SLOT[0, c - 1]: x_rows(c) for c in range(1, NC)}
    early[SLOT[1, 0] - 1] = weights(1) + [(wphi_hbm.at[4:H], wphi_buf.at[4:H])] + early[SLOT[1, 0] - 1]
    early[SHIFT_SLOT] = mod_cols(0, D)
    early[FOLD_SLOT] = weights(2, 3)
    batches = {
        "start": [(c_hbm, c_buf), (wphi_hbm.at[0:4], wphi_buf.at[0:4])] + weights(0) + x_rows(0),
        **{("scale", k): mod_cols(D + k, SCALE_COLS) + mod_cols(D + HD + k, SCALE_COLS)
           for k in range(0, HD, SCALE_COLS)},
        **dict(sorted(early.items())),
        LATE_SLOT: weights(*range(4, G)) + [(wr_hbm, wr_buf), (wo_hbm, wo_buf)],
        len(SLOTS) - 1: mod_cols(2 * D, 4 * D) + [(wg_hbm, wg_buf), (wu_hbm, wu_buf), (wd_hbm, wd_buf.at[:, 0:D])],
    }
    batches = {name: [pltpu.make_async_copy(src, dst, sem.at[i]) for src, dst in pairs]
               for i, (name, pairs) in enumerate(batches.items())}
    sem_out = sem.at[len(batches)]
    for copies in batches.values():
        for copy in copies:
            copy.start()

    def arrive(name):
        for copy in batches.pop(name):
            copy.wait()

    def out_copy(t):
        return pltpu.make_async_copy(out_bufs[t].at[0, 0:T], out_hbm.at[pl.ds(t * T, T)], sem_out)

    zero, other_zero = [jnp.min(_iota((8, 128), axis)) for axis in range(2)]
    never = _iota((8, 128), 1) < other_zero
    val, due, holds = {}, {}, {}

    def stored(ref):
        return ref.at[zero]

    def after(x, dep, r=0):
        head = jnp.where(never, pltpu.bitcast(dep[0:8, 0:128], x.dtype), x[r:r + 8, 0:128])
        if x.shape[1] > 128:
            head = jnp.concatenate([head, x[r:r + 8, 128:]], axis=1)
        parts = ([x[:r]] if r else []) + [head] + ([x[r + 8:]] if x.shape[0] > r + 8 else [])
        return jnp.concatenate(parts, axis=0)

    def released(x):
        return after(x, val["last product"]) if "last product" in val else x

    def deadline(slot, n, dep, j=0):
        due.setdefault((slot, n, j), []).append(dep)

    def meet(x, slot, n):
        cols = [x[:, l:l + 128] for l in range(0, x.shape[1], 128)]
        for j in range(len(cols)):
            for i, dep in enumerate(due.pop((slot, n, j), [])):
                cols[j] = after(cols[j], dep, 8 * i)
        return jnp.concatenate(cols, axis=1)

    same_head = _iota((128, 128), 0) // DH == _iota((128, 128), 1) // DH
    pick_feature = (_iota((128, DH), 0) % DH == _iota((128, DH), 1)).astype(BF16)

    def mix(g):
        wp = wphi_buf[g * 4:g * 4 + 4].reshape(128, DH)
        val["mix", g] = jnp.where(same_head, _dot(pick_feature, wp, NT), 0.0)

    def bias_part(g, i, k):
        left, right = val["folded", g, i, k]
        term = (left.reshape(16, 8, 128) * val["sa"][:, k:k + 128][None]
                + right.reshape(16, 8, 128) * val["sa"][:, HD + k:HD + k + 128][None])
        val["bias", g, i] = term if k == 0 else val["bias", g, i] + term
        if k == HD - 128:
            b = jnp.sum(val["bias", g, i], axis=-1, keepdims=True)
            b = jnp.broadcast_to(b, (16, 8, 128)).reshape(128, 128)
            for p in range(2):
                val["bias", g, i, p] = _interleave_halves(b[64 * p:64 * p + 64])

    def fold_tasks(g):
        def part(i, k):
            def run(slot):
                halves = []
                for lo in (k, HD + k):
                    w = _unpack(released(pltpu.bitcast(w_buf[i, g, lo:lo + 128, :], U32)))
                    halves.append(_dot(val["mix", g].astype(BF16), w, NT) if i < 2 else w.astype(F32).T)
                val["folded", g, i, k] = halves
                if g > 1:
                    bias_part(g, i, k)
                for n in range(7):
                    words = _pack_halves(_lhs_term(lambda p, j: halves[j][64 * p:64 * p + 64], n))
                    w_terms[g % 3][n, 32 * i:32 * i + 32, k:k + 128] = words
                holds["w", g % 3, i, k] = g
                if slot is not None:
                    deadline(slot + SLACK, 1 + k // 128, words)
            return run
        return [part(i, k) for i in range(3) for k in range(0, HD, 128)]

    def wo_tasks():
        def piece(r, l):
            def run(slot):
                quads = {}
                for e in range(2):
                    for i in range(2):
                        lo = r // DH * 128 + r % DH + i * 64 + DH * e
                        for j in range(2):
                            w = wo_buf[lo:lo + 16, j * HD + l:j * HD + l + WO_COLS].astype(F32)
                            quads[e, i, j] = released(w)
                for n in range(7):
                    words = _pack(*[_rhs_term(lambda i, j: quads[e, i, j], n) for e in range(2)])
                    stored(wo_terms)[n, r:r + 16, l:l + WO_COLS] = words
                holds["wo", r, l] = True
                deadline(slot + SLACK, (r // 16 + l // 128) % 7, wo_terms[0, 0, r:r + 8, l:l + 128])
            return run
        return [piece(r, l) for r in range(0, HD // 2, 16) for l in range(0, HD, WO_COLS)]

    def norm_means(c, r):
        rows = [slice(c * T + n * HT + r, c * T + n * HT + r + 16) for n in range(2)]
        xs = [x for n in range(2) for x in _split(x_buf[rows[n], :])]
        val["norm", c, r] = xs, _row_means(xs)

    def norm_spread(c, r):
        val["norm", c, r] = _row_spread(*val["norm", c, r])

    def norm_scales(c, r):
        centred, var = val["norm", c, r]
        scales = _row_scales(var)
        val["norm", c, r] = [(d, scales[:, i:i + 1]) for i, d in enumerate(centred)]

    def norm_stats(c, r):
        for stage, lag in ((norm_means, 0), (norm_spread, 16), (norm_scales, 32)):
            if 0 <= r - lag < HT:
                stage(c, r - lag)

    def norm_terms(c, r, k):
        h = {}
        for j in range(2):
            for n in range(2):
                for e in range(2):
                    d, scale = val["norm", c, r][2 * n + e]
                    h[e, j, n] = d[:, j * HD + k:j * HD + k + 128] * scale * val["scale", j * HD + k]
        for n in range(7):
            words = _pack(*[_rhs_term(lambda j, m: h[e, j, m], n) for e in range(2)])
            h_terms[c][n, r // 2:r // 2 + 8, k:k + 128] = words
        holds["h", c, r, k] = True
        return words

    def norm_tasks(c):
        def step(r):
            def run(slot):
                norm_stats(c, r)
                if r >= 32:
                    for k in range(0, HD, 128):
                        words = norm_terms(c, r - 32, k)
                    if slot + 1 < SLOT[0, c]:
                        deadline(slot + 1, PRODUCTS[r // 16 % 4], words)
            return run
        return [step(r) for r in range(0, HT + 32, 16)]

    arrive("start")
    mix(0)
    for task in fold_tasks(0):
        task(None)
    cv = c_buf[...].astype(F32)
    cond = jnp.broadcast_to(_rnd(cv * _rnd(jax.nn.sigmoid(cv))), (16, D)).astype(BF16)
    for r in range(0, HT + 32, 16):
        norm_stats(0, r)
    for k in range(0, HD, SCALE_COLS):
        arrive(("scale", k))
        for lo in (k, HD + k):
            block = _rnd(1.0 + _rnd(_dot(cond, wmod_buf[:, D + lo:D + lo + SCALE_COLS])[0:8])) * LOG2E
            for l in range(0, SCALE_COLS, 128):
                val["scale", lo + l] = block[:, l:l + 128]
        for r in range(0, HT, 16):
            for l in range(k, k + SCALE_COLS, 128):
                norm_terms(0, r, l)

    kv_mask = _iota((64, 128), 0) % 2 == (_iota((64, 128), 1) // 2) % 2

    def project_tasks(g, c):
        def product(n):
            def run():
                assert all(holds["w", g % 3, i, k] == g for i in range(3) for k in range(0, HD, 128))
                assert all(("h", c, r, k) in holds for r in range(0, HT, 16) for k in range(0, HD, 128))
                rhs = meet(h_terms[c][n], SLOT[g, c], n)
                val["last product"] = val["qkv", g, c, n] = _dot(_unpack(w_terms[g % 3][n]), _unpack(rhs), NT)
            return run
        return [product(n) for n in PRODUCTS]

    def key_tasks(g, c):
        def piece(p, n):
            def run():
                def part(i):
                    y = _quadrant(lambda k: val["qkv", g, c, k][64 * i:64 * i + 64], p, n)
                    return y + val["bias", g, i, p] if i < 2 else y
                pq_bufs[g % 3][c, p, n] = part(0)
                holds["pq", g % 3, c, p, n] = g
                val["v", g, c, p, n] = part(2)
                logits = part(1).reshape(8, 8, 128)
                words = []
                for sign in range(2):
                    phi = _softmax2(logits, sign)
                    words.append(_pack_halves(phi.reshape(64, 128)))
                    val["z", g, p, sign] = val["z", g, p, sign] + phi if ("z", g, p, sign) in val else phi
                val["phi_k", g, c, p, n] = jnp.concatenate(words, axis=0)
            return run
        return [piece(p, n) for p, n in ((1, 0), (0, 1), (1, 1), (0, 0))]

    def summary_tasks(g, c):
        def piece(p):
            def run():
                v = jnp.concatenate([val["v", g, c, p, n] for n in range(2)], axis=1).astype(BF16)
                phi = _unpack(jnp.concatenate([val["phi_k", g, c, p, n] for n in range(2)], axis=1))
                kv = _dot(v, phi, NT)
                val["kv", g, p] = kv if c == 0 else val["kv", g, p] + kv
                if c == NC - 1:
                    for sign in range(2):
                        z = jnp.sum(val["z", g, p, sign], axis=-1, keepdims=True)
                        val["z total", g, p, sign] = jnp.broadcast_to(z, (8, 8, 128))
                    z_row = jnp.concatenate(
                        [_interleave_halves(val["z total", g, p, sign].reshape(64, 128)) for sign in range(2)],
                        axis=0).T[0:64]
                    val["kv", g, p] = jnp.where(kv_mask, val["kv", g, p] + val["bias", g, 2, p] * z_row, 0.0)
            return run
        return [piece(p) for p in range(2)]

    def query_tasks(g, c):
        def piece(p, n):
            def run():
                assert holds["pq", g % 3, c, p, n] == g
                logits = released(pq_bufs[g % 3][c, p, n]).reshape(8, 8, 128)
                words, den = [], None
                for sign in range(2):
                    phi = _softmax2(logits, sign)
                    words.append(_pack_halves(phi.reshape(64, 128)))
                    w = _tree(phi * val["z total", g, p, sign], jnp.add)
                    den = w if den is None else den + w
                val["1 / den", g, c, p, n] = pl.reciprocal(_fold_rows(den, jnp.add) + 1e-6, full_range=False)
                val["phi_q", g, c, p, n] = jnp.concatenate(words, axis=0)
            return run
        return [piece(p, n) for n in range(2) for p in range(2)]

    def readout(g, c, slot):
        nums = [_dot(val["kv", g, p].astype(BF16),
                     _unpack(jnp.concatenate([val["phi_q", g, c, p, n] for n in range(2)], axis=1)))
                for p in range(2)]
        for p in range(2):
            for n in range(2):
                num = nums[p][:, n * HT:(n + 1) * HT].reshape(8, 8, 128)
                val["o", g, c, n, p] = (num * val["1 / den", g, c, p, n][None]).reshape(64, 128)
        if g % 2:
            for k in range(7):
                term = _lhs_term(
                    lambda n, p: jnp.concatenate([val["o", g - 1, c, n, p], val["o", g, c, n, p]], axis=0), k)
                words = pltpu.bitcast(term.astype(BF16).T, U32)
                o_terms[c][k, :, 64 * (g - 1):64 * (g + 1)] = words
                deadline(slot + SLACK, k, words[56:64])
            holds["o", c, g] = True
        else:
            for k, (n, p) in enumerate(((0, 0), (0, 1), (1, 0), (1, 1))):
                deadline(slot + SLACK, k, val["o", g, c, n, p][56:64])

    agenda = _agenda()

    def run_slot(s, plan, products, extras=(), wait=None):
        keys = [task for gc in agenda.get(("key", s), []) for task in key_tasks(*gc)]
        queries = [task for gc in agenda.get(("query", s), []) for task in query_tasks(*gc)]
        mixed = sorted([((i + 0.5) / len(keys), 0, i) for i in range(len(keys))]
                       + [((i + 0.5) / len(queries), 1, i) for i in range(len(queries))])
        pieces = _spread([(keys, queries)[kind][i] for _, kind, i in mixed], plan.count("q"))
        sums = _spread([task for gc in agenda.get(("sum", s), []) for task in summary_tasks(*gc)], plan.count("k"))
        products = list(products)
        assert plan.count("p") >= len(products) and ("f" in plan or not extras) and ("w" in plan or not wait)
        assert all(step in plan or (kind, s) not in agenda
                   for step, kind in (("q", "key"), ("q", "query"), ("k", "sum"), ("r", "read")))
        for step in plan:
            if step == "p" and products:
                products.pop(0)()
            elif step in "qk":
                for task in (pieces if step == "q" else sums).pop(0):
                    task()
            elif step == "r":
                for gc in agenda.get(("read", s), []):
                    readout(*gc, s)
            elif step == "f":
                for task in extras:
                    task(s)
            elif step == "w" and wait:
                wait()

    def shift():
        arrive(SHIFT_SLOT)
        val["sa"] = _rnd(_dot(cond, wmod_buf[:, 0:D])[0:8]) * LOG2E

    waits = {s: (lambda s=s: arrive(s)) for s in batches if isinstance(s, int)}
    waits[SHIFT_SLOT] = shift

    extras = {s: [] for s in range(len(SLOTS))}

    def assign(tasks, slots):
        for s, chunk in zip(slots, _spread(tasks, len(slots))):
            extras[s] += chunk

    assign([lambda s, g=g: mix(g) for g in range(1, G)] + fold_tasks(1), [SLOT[1, 0] - 1])
    for c in range(1, NC):
        assign(norm_tasks(c), range(SLOT[0, c - 1], SLOT[0, c]))
    for g, slots in enumerate(([SHIFT_SLOT], range(SHIFT_SLOT + 1, SHIFT_SLOT + 4))):
        assign([lambda s, g=g, i=i, k=k: bias_part(g, i, k) for i in range(3) for k in range(0, HD, 128)], slots)
    for g in range(2, G):
        tasks, slots = fold_tasks(g), range(max((g - 1) * NC, FOLD_SLOT), g * NC - 1)
        assign(tasks[:8], slots)
        assign(tasks[8:], slots)
    assign(wo_tasks(), range(LATE_SLOT, len(SLOTS) - 2))

    for s, gc in enumerate(SLOTS):
        plan = (PLAN_FIRST if s == 0 else PLAN_STREAM if s < SHIFT_SLOT else PLAN_SHIFT if s == SHIFT_SLOT
                else PLAN_WAIT if s in waits and s > FOLD_SLOT else PLAN_STEADY)
        run_slot(s, plan, project_tasks(*gc), extras[s], waits.get(s))

    def mod_part(i):
        def run():
            lhs = _unpack(released(pltpu.bitcast(cond, U32)))
            val["mod", i] = _rnd(_dot(lhs, wmod_buf[:, i * HD:(i + 1) * HD])[0:8])
        return run

    mods = [mod_part(i) for i in range(4, 12)]
    for s, count in zip(range(len(SLOTS), TILE_SLOT), (2, 2, 3, 1)):
        run_slot(s, PLAN_DRAIN, [mods.pop(0) for _ in range(count)])
    ga, sb, cb, gb = [jnp.concatenate([val["mod", 2 * i], val["mod", 2 * i + 1]], axis=1) for i in range(2, 6)]
    cb1 = _rnd(1.0 + cb)
    wr = jnp.broadcast_to(wr_buf[...].reshape(1, D).astype(F32), (8, D))
    coefs = {"attn": ga * (1.0 / LOG2E), "out mul": gb * cb1, "out add": gb * sb, "score": cb1 * wr,
             "h mul": cb1, "h add": sb, "gate": gb}
    for i, row in enumerate(coefs.values()):
        stored(coef_buf)[i] = row
    score_add = jnp.sum(sb * wr, axis=-1, keepdims=True)
    deadline(TILE_SLOT, PRODUCTS[0], gb)

    def coef(name):
        return coef_buf[0, list(coefs).index(name)]

    lane = _iota((8, 128), 1)
    scores = [jnp.zeros((8, 128), F32)] * 2

    def finish_rows(t, i, r):
        r0 = t * T + i * HT + r
        xs = []
        for e in (0, 8):
            a = jnp.concatenate(
                [_quadrant(lambda k: val["attn", t, k][r + e:r + e + 8], i, j) for j in range(2)], axis=1)
            xs.append(x_buf[r0 + e:r0 + e + 8, :].astype(F32) + coef("attn") * a)
            x1_buf[r0 + e:r0 + e + 8] = xs[-1]
        means = _row_means(xs)
        centred, var = _row_spread(xs, means)
        scales = _row_scales(var)
        scale_buf[r0 // 2:r0 // 2 + 8] = scales
        outs = []
        for k in range(2):
            scale = scales[:, k:k + 1]
            mean_buf[r0 + 8 * k:r0 + 8 * k + 8] = jnp.broadcast_to(_rnd(means[k]), (8, 128))
            outs.append(xs[k] + (centred[k] * scale * coef("out mul") + coef("out add")))
            score = jnp.sum(centred[k] * coef("score"), axis=-1, keepdims=True) * scale
            scores[r0 // 1024] = jnp.where(lane == (r0 // 8 + k) % 128, score, scores[r0 // 1024])
        rows = slice(r0 - t * T, r0 - t * T + 16)
        stored(out_bufs[t])[rows, :] = jnp.concatenate(outs, axis=0).astype(BF16)
        return pltpu.bitcast(out_bufs[t][0, rows, 0:128], U32), scores[r0 // 1024]

    pending = [(7 * t + EPILOGUE_LAG + k * 7 // 16, t, k) for t in range(NC) for k in range(16)]

    def flush(upto, slot=None, n=None):
        while pending and pending[0][0] <= upto:
            _, t, k = pending.pop(0)
            done = finish_rows(t, 1 - k // 8, 16 * (k % 8))
            if slot is not None:
                for dep in done:
                    deadline(slot, n, dep)
            if k == 15:
                out_copy(t).start()
                stored(out_bufs[t])[T:T + 16, 0:128] = jnp.zeros((16, 128), BF16)
                deadline(TILE_SLOT + (upto + 2) // 7, PRODUCTS[(upto + 2) % 7],
                         pltpu.bitcast(out_bufs[t][0, T:T + 16, 0:128], U32), 3)

    def tile_tasks(t):
        def product(j, n):
            def run():
                flush(7 * t + j, TILE_SLOT + t, n)
                assert all(("o", t, g) in holds for g in range(1, G, 2))
                assert all(("wo", r, l) in holds for r in range(0, HD // 2, 16) for l in range(0, HD, WO_COLS))
                rhs = meet(wo_terms[0, n], TILE_SLOT + t, n)
                val["last product"] = val["attn", t, n] = _dot(_unpack(o_terms[t][n]), _unpack(rhs))
            return run
        return [product(j, n) for j, n in enumerate(PRODUCTS)]

    for t in range(NC):
        run_slot(TILE_SLOT + t, PLAN_TILE, tile_tasks(t))
    flush(pending[-1][0])
    assert not batches

    r = _rnd(jnp.concatenate(scores, axis=0) + jnp.concatenate([score_add] * 2, axis=0))
    r = jnp.clip(jnp.where(r != r, -BF16_MAX, r), -BF16_MAX, BF16_MAX)
    r = jnp.where(jnp.abs(r) < F32_TINY, F32_TINY, r)
    token = (_iota((16, 128), 0) // 8) * 1024 + _iota((16, 128), 1) * 8 + _iota((16, 128), 0) % 8
    keys = pltpu.bitcast(pltpu.bitcast(r, jnp.int32) | jnp.where(r > 0, S - 1 - token, token), F32)
    picks = []
    for _ in range(2):
        top = jnp.max(jnp.max(keys, axis=0, keepdims=True), axis=1, keepdims=True)
        bits = pltpu.bitcast(jnp.broadcast_to(top, (8, 128)), jnp.int32)
        low = bits & (S - 1)
        picks.append((jnp.where(bits > 0, S - 1 - low, low), pltpu.bitcast(bits & -65536, F32)))
        keys = jnp.where(keys == top, -jnp.inf, keys)
    b1, b2 = [pl.multiple_of(jnp.clip(i[0, 0] // 16, 0, S // 16 - 1) * 16, 16) for i, _ in picks]

    def gather(ref):
        return jnp.concatenate([ref[pl.ds(b1, 16)], ref[pl.ds(b2, 16)]], axis=0)

    def wide(x):
        return jnp.concatenate([x] * (D // 128), axis=1)

    x1 = gather(x1_buf)
    stats = [scale_buf[pl.ds(pl.multiple_of(b // 2, 8), 8)] for b in (b1, b2)]
    scale = jnp.concatenate([sv[:, i:i + 1] for sv in stats for i in range(2)], axis=0)
    h2 = (x1 - wide(gather(mean_buf))) * scale * coef("h mul")[0:1] + coef("h add")[0:1]
    hb = h2.astype(BF16)
    u = _dot(hb, wg_buf[...])
    act = u * jax.nn.sigmoid(u) * _dot(hb, wu_buf[...])
    y = _dot(act.astype(BF16), wd_buf[:, 0:D])
    rows = _iota((32, 128), 0)
    rows = jnp.where(rows < 16, rows + b1, rows - 16 + b2)
    update = jnp.zeros((32, D), F32)
    for i, score in picks:
        hit = wide(rows == jnp.concatenate([i] * 4, axis=0))
        update = jnp.where(hit, y * wide(jax.nn.sigmoid(score))[0:1], update)
    fix_buf[...] = (x1 + coef("gate")[0:1] * (h2 + update)).astype(BF16)

    for t in range(NC):
        out_copy(t).wait()
    fix1 = pltpu.make_async_copy(fix_buf.at[0:16], out_hbm.at[pl.ds(b1, 16)], sem_out)
    fix2 = pltpu.make_async_copy(fix_buf.at[16:32], out_hbm.at[pl.ds(b2, 16)], sem_out)
    fix1.start()

    @pl.when(b1 != b2)
    def _():
        fix2.start()
        fix2.wait()

    fix1.wait()


@jax.jit
def pallas_adaLN_cond__linear_kernel_hedgehog__moe_arch_mod__prompt_kernel(
    A_x: jax.Array,
    A_wqkv: jax.Array,
    A_w_phi: jax.Array,
    A_wo: jax.Array,
    B_x: jax.Array,
    B_w_r: jax.Array,
    B_w_gate: jax.Array,
    B_w_up: jax.Array,
    B_w_down: jax.Array,
    c: jax.Array,
    w_mod: jax.Array,
):
    hbm = pl.BlockSpec(memory_space=pl.ANY)
    vmem = pltpu.VMEM
    out = pl.pallas_call(
        _kernel,
        out_shape=jax.ShapeDtypeStruct((S, D), BF16),
        in_specs=[hbm] * 10,
        out_specs=hbm,
        scratch_shapes=[
            vmem((S, D), BF16),
            vmem((3, G, D, 128), BF16),
            vmem((H, DH, DH), BF16),
            vmem((D, D), BF16),
            vmem((D,), BF16),
            vmem((D, F), BF16),
            vmem((D, F), BF16),
            vmem((F, D + 128), BF16),
            vmem((1, D), BF16),
            vmem((D, 6 * D + 128), BF16),
            [vmem((7, HT // 2, HD), U32)] * NC,
            [vmem((7, 96, HD), U32)] * 3,
            [vmem((NC, 2, 2, 64, 128), F32)] * 3,
            [vmem((7, HT // 2, HD), U32)] * NC,
            vmem((1, 7, HD // 2, HD), U32),
            vmem((S, D), F32),
            vmem((S, 128), F32),
            vmem((S // 2, 128), F32),
            [vmem((1, T + 16, D), BF16)] * NC,
            vmem((1, 7, 8, D), F32),
            vmem((32, D), BF16),
            pltpu.SemaphoreType.DMA((NC + 5 + HD // SCALE_COLS,)),
        ],
        compiler_params=pltpu.CompilerParams(vmem_limit_bytes=120 * 2**20),
        name="adaln_hedgehog_mod",
    )(A_x.reshape(S, D), A_wqkv, A_w_phi, A_wo, B_w_r, B_w_gate, B_w_up, B_w_down, c, w_mod)
    return out.reshape(1, S, D)
```

```python
import numpy as np

import jax
import jax.numpy as jnp
from jax import lax
import jax.experimental.pallas as pl
import jax.experimental.pallas.tpu as pltpu

S, D, H, DH, F = 2048, 1024, 32, 32, 3584
G = 8
HD = D // 2
T = 256
HT = T // 2
NC = S // T

LOG2E = float(np.log2(np.e))
BF16_MAX = 3.3895313892515355e38
F32_TINY = float(np.finfo(np.float32).tiny)
NT = (((1,), (1,)), ((), ()))
NN = (((1,), (0,)), ((), ()))
F32, BF16, U32 = jnp.float32, jnp.bfloat16, jnp.uint32

LEAD_IN = [int(g) for g in "0000010101011111"]
SLOTS = [(g, LEAD_IN[:i].count(g)) for i, g in enumerate(LEAD_IN)] + [(g, c) for g in range(2, G) for c in range(NC)]
SLOT = {gc: s for s, gc in enumerate(SLOTS)}
PRODUCTS = (3, 1, 0, 2, 5, 4, 6)
SHIFT_SLOT, FOLD_SLOT, LATE_SLOT = 7, 10, 23
TILE_SLOT = len(SLOTS) + 4
SCALE_COLS, WO_COLS = 256, 256
SLACK = 3
EPILOGUE_LAG = 9

PLAN_FIRST, PLAN_STREAM = "ppppppwpf", "wpppppppf"
PLAN_SHIFT, PLAN_WAIT = "pppwppppkkqqqqqqrqqf", "pppkkpwpppqqqqqqrqqf"
PLAN_STEADY = "pwkkqpqpqpqpqpqprqpqf"
PLAN_DRAIN, PLAN_TILE = "kkqpppprpppp", "pkkpqpqpqpqprp"


def _dot(a, b, dims=NN):
    return lax.dot_general(a, b, dims, preferred_element_type=F32)


def _rnd(x):
    return x.astype(BF16).astype(F32)


def _iota(shape, axis):
    return lax.broadcasted_iota(jnp.int32, shape, axis)


def _pack(even, odd):
    return pltpu.pack_elementwise([even, odd], packed_dtype=BF16)


def _pack_halves(x):
    n = x.shape[0] // 2
    return _pack(x[:n], x[n:])


def _unpack(words):
    return pltpu.bitcast(words, BF16)


def _split(x):
    words = pltpu.bitcast(x, U32)
    return [pltpu.unpack_elementwise(words, index=i, packed_dtype=BF16, unpacked_dtype=F32) for i in range(2)]


def _interleave_halves(x):
    return _unpack(_pack_halves(x)).astype(F32) + _unpack(_pack_halves(x - _rnd(x))).astype(F32)


def _tree(x3, op):
    return op(op(op(x3[0], x3[1]), op(x3[2], x3[3])), op(op(x3[4], x3[5]), op(x3[6], x3[7])))


def _fold_rows(m, op):
    m = op(m, pltpu.roll(m, 2, 0))
    return op(m, pltpu.roll(m, 4, 0))


def _softmax2(p3, sign):
    if sign == 0:
        e = jnp.exp2(p3 - _fold_rows(_tree(p3, jnp.maximum), jnp.maximum)[None])
    else:
        e = jnp.exp2(_fold_rows(_tree(p3, jnp.minimum), jnp.minimum)[None] - p3)
    return e * pl.reciprocal(_fold_rows(_tree(e, jnp.add), jnp.add), full_range=False)[None]


def _row_means(xs):
    return [jnp.mean(x, axis=-1, keepdims=True) for x in xs]


def _row_spread(xs, means):
    lane = _iota((xs[0].shape[0], 128), 1)
    centred, var = [], None
    for i, (x, mean) in enumerate(zip(xs, means)):
        rounded = _rnd(mean)
        d = x - rounded
        v = jnp.mean(d * d, axis=-1, keepdims=True) - (mean - rounded) * (mean - rounded)
        var = jnp.where(lane == i, v, var) if i else jnp.broadcast_to(v, lane.shape)
        centred.append(d)
    return centred, var


def _row_scales(var):
    return 1.0 / _rnd(jnp.sqrt(_rnd(_rnd(var) + _rnd(jnp.full_like(var, 1e-5)))))


def _lhs_term(a, n):
    return (lambda: a(0, 0) + a(1, 1), lambda: a(1, 0) + a(1, 1), lambda: a(0, 0), lambda: a(1, 1),
            lambda: a(0, 0) + a(0, 1), lambda: a(1, 0) - a(0, 0), lambda: a(0, 1) - a(1, 1))[n]()


def _rhs_term(b, n):
    return (lambda: b(0, 0) + b(1, 1), lambda: b(0, 0), lambda: b(0, 1) - b(1, 1), lambda: b(1, 0) - b(0, 0),
            lambda: b(1, 1), lambda: b(0, 0) + b(0, 1), lambda: b(1, 0) + b(1, 1))[n]()


def _quadrant(m, i, j):
    if (i, j) == (0, 0):
        return (m(0) + m(3)) + (m(6) - m(4))
    if (i, j) == (0, 1):
        return m(2) + m(4)
    if (i, j) == (1, 0):
        return m(1) + m(3)
    return (m(0) - m(1)) + (m(2) + m(5))


def _spread(tasks, n):
    return [tasks[i * len(tasks) // n:(i + 1) * len(tasks) // n] for i in range(n)]


def _agenda():
    total, agenda = len(SLOTS), {}

    def key_slot(s):
        return max(s + 1, SHIFT_SLOT + 2 + s // 2)

    def ready(g):
        return key_slot(SLOT[g, NC - 1]) + 2

    for s, gc in enumerate(SLOTS):
        agenda.setdefault(("key", key_slot(s)), []).append(gc)
        agenda.setdefault(("sum", key_slot(s) + 1), []).append(gc)
    for u in range(total):
        g, c = divmod(u, NC)
        s = min(max(ready(0) + u * (total + 2 + NC - ready(0)) // total, ready(g)), TILE_SLOT + c - 2)
        assert s >= ready(g)
        agenda.setdefault(("query", s), []).append((g, c))
        agenda.setdefault(("read", s + 1), []).append((g, c))
    return agenda


def _kernel(x_hbm, wqkv_hbm, wphi_hbm, wo_hbm, wr_hbm, wg_hbm, wu_hbm, wd_hbm, c_hbm, wmod_hbm,
            out_hbm,
            x_buf, w_buf, wphi_buf, wo_buf, wr_buf, wg_buf, wu_buf, wd_buf, c_buf, wmod_buf,
            h_terms, w_terms, pq_bufs, o_terms, wo_terms, x1_buf, mean_buf, scale_buf, out_bufs, coef_buf,
            fix_buf, sem):
    def x_rows(j):
        return [(x_hbm.at[pl.ds(j * T, T)], x_buf.at[pl.ds(j * T, T)])]

    def weights(*groups):
        return [(wqkv_hbm.at[:, pl.ds(i * D + g * 128, 128)], w_buf.at[i, g]) for g in groups for i in range(3)]

    def mod_cols(lo, n):
        return [(wmod_hbm.at[:, pl.ds(lo, n)], wmod_buf.at[:, pl.ds(lo, n)])]

    early = {SLOT[0, c - 1]: x_rows(c) for c in range(1, NC)}
    early[SLOT[1, 0] - 1] = weights(1) + [(wphi_hbm.at[4:H], wphi_buf.at[4:H])] + early[SLOT[1, 0] - 1]
    early[SHIFT_SLOT] = mod_cols(0, D)
    early[FOLD_SLOT] = weights(2, 3)
    batches = {
        "start": [(c_hbm, c_buf), (wphi_hbm.at[0:4], wphi_buf.at[0:4])] + weights(0) + x_rows(0),
        **{("scale", k): mod_cols(D + k, SCALE_COLS) + mod_cols(D + HD + k, SCALE_COLS)
           for k in range(0, HD, SCALE_COLS)},
        **dict(sorted(early.items())),
        LATE_SLOT: weights(*range(4, G)) + [(wr_hbm, wr_buf), (wo_hbm, wo_buf)] + mod_cols(2 * D, 2 * D),
        len(SLOTS) - 1: mod_cols(4 * D, 2 * D) + [(wg_hbm, wg_buf), (wu_hbm, wu_buf), (wd_hbm, wd_buf.at[:, 0:D])],
    }
    batches = {name: [pltpu.make_async_copy(src, dst, sem.at[i]) for src, dst in pairs]
               for i, (name, pairs) in enumerate(batches.items())}
    sem_out = sem.at[len(batches)]
    for copies in batches.values():
        for copy in copies:
            copy.start()

    def arrive(name):
        for copy in batches.pop(name):
            copy.wait()

    def out_copy(t):
        return pltpu.make_async_copy(out_bufs[t].at[0, 0:T], out_hbm.at[pl.ds(t * T, T)], sem_out)

    zero, other_zero = [jnp.min(_iota((8, 128), axis)) for axis in range(2)]
    never = _iota((8, 128), 1) < other_zero
    val, due, holds = {}, {}, {}

    def stored(ref):
        return ref.at[zero]

    def after(x, dep, r=0):
        head = jnp.where(never, pltpu.bitcast(dep[0:8, 0:128], x.dtype), x[r:r + 8, 0:128])
        if x.shape[1] > 128:
            head = jnp.concatenate([head, x[r:r + 8, 128:]], axis=1)
        parts = ([x[:r]] if r else []) + [head] + ([x[r + 8:]] if x.shape[0] > r + 8 else [])
        return jnp.concatenate(parts, axis=0)

    def released(x):
        return after(x, val["last product"]) if "last product" in val else x

    def deadline(slot, n, dep, j=0):
        due.setdefault((slot, n, j), []).append(dep)

    def meet(x, slot, n):
        cols = [x[:, l:l + 128] for l in range(0, x.shape[1], 128)]
        for j in range(len(cols)):
            for i, dep in enumerate(due.pop((slot, n, j), [])):
                cols[j] = after(cols[j], dep, 8 * i)
        return jnp.concatenate(cols, axis=1)

    same_head = _iota((128, 128), 0) // DH == _iota((128, 128), 1) // DH
    pick_feature = (_iota((128, DH), 0) % DH == _iota((128, DH), 1)).astype(BF16)

    def mix(g):
        wp = wphi_buf[g * 4:g * 4 + 4].reshape(128, DH)
        val["mix", g] = jnp.where(same_head, _dot(pick_feature, wp, NT), 0.0)

    def bias_part(g, i, k):
        left, right = val["folded", g, i, k]
        term = (left.reshape(16, 8, 128) * val["sa"][:, k:k + 128][None]
                + right.reshape(16, 8, 128) * val["sa"][:, HD + k:HD + k + 128][None])
        val["bias", g, i] = term if k == 0 else val["bias", g, i] + term
        if k == HD - 128:
            b = jnp.sum(val["bias", g, i], axis=-1, keepdims=True)
            b = jnp.broadcast_to(b, (16, 8, 128)).reshape(128, 128)
            for p in range(2):
                val["bias", g, i, p] = _interleave_halves(b[64 * p:64 * p + 64])

    def fold_tasks(g):
        def part(i, k):
            def run(slot):
                halves = []
                for lo in (k, HD + k):
                    w = _unpack(released(pltpu.bitcast(w_buf[i, g, lo:lo + 128, :], U32)))
                    halves.append(_dot(val["mix", g].astype(BF16), w, NT) if i < 2 else w.astype(F32).T)
                val["folded", g, i, k] = halves
                if g > 1:
                    bias_part(g, i, k)
                for n in range(7):
                    words = _pack_halves(_lhs_term(lambda p, j: halves[j][64 * p:64 * p + 64], n))
                    w_terms[g % 3][n, 32 * i:32 * i + 32, k:k + 128] = words
                holds["w", g % 3, i, k] = g
                if slot is not None:
                    deadline(slot + SLACK, 1 + k // 128, words)
            return run
        return [part(i, k) for i in range(3) for k in range(0, HD, 128)]

    def wo_tasks():
        def piece(r, l):
            def run(slot):
                quads = {}
                for e in range(2):
                    for i in range(2):
                        lo = r // DH * 128 + r % DH + i * 64 + DH * e
                        for j in range(2):
                            w = wo_buf[lo:lo + 16, j * HD + l:j * HD + l + WO_COLS].astype(F32)
                            quads[e, i, j] = released(w)
                for n in range(7):
                    words = _pack(*[_rhs_term(lambda i, j: quads[e, i, j], n) for e in range(2)])
                    stored(wo_terms)[n, r:r + 16, l:l + WO_COLS] = words
                holds["wo", r, l] = True
                deadline(slot + SLACK, (r // 16 + l // 128) % 7, wo_terms[0, 0, r:r + 8, l:l + 128])
            return run
        return [piece(r, l) for r in range(0, HD // 2, 16) for l in range(0, HD, WO_COLS)]

    def norm_means(c, r):
        rows = [slice(c * T + n * HT + r, c * T + n * HT + r + 16) for n in range(2)]
        xs = [x for n in range(2) for x in _split(x_buf[rows[n], :])]
        val["norm", c, r] = xs, _row_means(xs)

    def norm_spread(c, r):
        val["norm", c, r] = _row_spread(*val["norm", c, r])

    def norm_scales(c, r):
        centred, var = val["norm", c, r]
        scales = _row_scales(var)
        val["norm", c, r] = [(d, scales[:, i:i + 1]) for i, d in enumerate(centred)]

    def norm_stats(c, r):
        for stage, lag in ((norm_means, 0), (norm_spread, 16), (norm_scales, 32)):
            if 0 <= r - lag < HT:
                stage(c, r - lag)

    def norm_terms(c, r, k):
        h = {}
        for j in range(2):
            for n in range(2):
                for e in range(2):
                    d, scale = val["norm", c, r][2 * n + e]
                    h[e, j, n] = d[:, j * HD + k:j * HD + k + 128] * scale * val["scale", j * HD + k]
        for n in range(7):
            words = _pack(*[_rhs_term(lambda j, m: h[e, j, m], n) for e in range(2)])
            h_terms[c][n, r // 2:r // 2 + 8, k:k + 128] = words
        holds["h", c, r, k] = True
        return words

    def norm_tasks(c):
        def step(r):
            def run(slot):
                norm_stats(c, r)
                if r >= 32:
                    for k in range(0, HD, 128):
                        words = norm_terms(c, r - 32, k)
                    if slot + 1 < SLOT[0, c]:
                        deadline(slot + 1, PRODUCTS[r // 16 % 4], words)
            return run
        return [step(r) for r in range(0, HT + 32, 16)]

    arrive("start")
    mix(0)
    for task in fold_tasks(0):
        task(None)
    cv = c_buf[...].astype(F32)
    cond = jnp.broadcast_to(_rnd(cv * _rnd(jax.nn.sigmoid(cv))), (16, D)).astype(BF16)
    for r in range(0, HT + 32, 16):
        norm_stats(0, r)
    cond_rows = jnp.broadcast_to(cond[0:1].astype(F32), (128, D))
    cond_cols = [cond_rows[:, k:k + 128].T for k in range(0, D, 128)]
    for k in range(0, HD, SCALE_COLS):
        arrive(("scale", k))
        for lo in (k, HD + k):
            block = _rnd(1.0 + _rnd(_dot(cond, wmod_buf[:, D + lo:D + lo + SCALE_COLS])[0:8])) * LOG2E
            for l in range(0, SCALE_COLS, 128):
                val["scale", lo + l] = block[:, l:l + 128]
        for r in range(0, HT, 16):
            for l in range(k, k + SCALE_COLS, 128):
                norm_terms(0, r, l)

    kv_mask = _iota((64, 128), 0) % 2 == (_iota((64, 128), 1) // 2) % 2

    def project_tasks(g, c):
        def product(n):
            def run():
                assert all(holds["w", g % 3, i, k] == g for i in range(3) for k in range(0, HD, 128))
                assert all(("h", c, r, k) in holds for r in range(0, HT, 16) for k in range(0, HD, 128))
                rhs = meet(h_terms[c][n], SLOT[g, c], n)
                val["last product"] = val["qkv", g, c, n] = _dot(_unpack(w_terms[g % 3][n]), _unpack(rhs), NT)
            return run
        return [product(n) for n in PRODUCTS]

    def key_tasks(g, c):
        def piece(p, n):
            def run():
                def part(i):
                    y = _quadrant(lambda k: val["qkv", g, c, k][64 * i:64 * i + 64], p, n)
                    return y + val["bias", g, i, p] if i < 2 else y
                pq_bufs[g % 3][c, p, n] = part(0)
                holds["pq", g % 3, c, p, n] = g
                val["v", g, c, p, n] = part(2)
                logits = part(1).reshape(8, 8, 128)
                words = []
                for sign in range(2):
                    phi = _softmax2(logits, sign)
                    words.append(_pack_halves(phi.reshape(64, 128)))
                    val["z", g, p, sign] = val["z", g, p, sign] + phi if ("z", g, p, sign) in val else phi
                val["phi_k", g, c, p, n] = jnp.concatenate(words, axis=0)
            return run
        return [piece(p, n) for p, n in ((1, 0), (0, 1), (1, 1), (0, 0))]

    def summary_tasks(g, c):
        def piece(p):
            def run():
                v = jnp.concatenate([val["v", g, c, p, n] for n in range(2)], axis=1).astype(BF16)
                phi = _unpack(jnp.concatenate([val["phi_k", g, c, p, n] for n in range(2)], axis=1))
                kv = _dot(v, phi, NT)
                val["kv", g, p] = kv if c == 0 else val["kv", g, p] + kv
                if c == NC - 1:
                    for sign in range(2):
                        z = jnp.sum(val["z", g, p, sign], axis=-1, keepdims=True)
                        val["z total", g, p, sign] = jnp.broadcast_to(z, (8, 8, 128))
                    z_row = jnp.concatenate(
                        [_interleave_halves(val["z total", g, p, sign].reshape(64, 128)) for sign in range(2)],
                        axis=0).T[0:64]
                    val["kv", g, p] = jnp.where(kv_mask, val["kv", g, p] + val["bias", g, 2, p] * z_row, 0.0)
            return run
        return [piece(p) for p in range(2)]

    def query_tasks(g, c):
        def piece(p, n):
            def run():
                assert holds["pq", g % 3, c, p, n] == g
                logits = released(pq_bufs[g % 3][c, p, n]).reshape(8, 8, 128)
                words, den = [], None
                for sign in range(2):
                    phi = _softmax2(logits, sign)
                    words.append(_pack_halves(phi.reshape(64, 128)))
                    w = _tree(phi * val["z total", g, p, sign], jnp.add)
                    den = w if den is None else den + w
                val["1 / den", g, c, p, n] = pl.reciprocal(_fold_rows(den, jnp.add) + 1e-6, full_range=False)
                val["phi_q", g, c, p, n] = jnp.concatenate(words, axis=0)
            return run
        return [piece(p, n) for n in range(2) for p in range(2)]

    def readout(g, c, slot):
        nums = [_dot(val["kv", g, p].astype(BF16),
                     _unpack(jnp.concatenate([val["phi_q", g, c, p, n] for n in range(2)], axis=1)))
                for p in range(2)]
        for p in range(2):
            for n in range(2):
                num = nums[p][:, n * HT:(n + 1) * HT].reshape(8, 8, 128)
                val["o", g, c, n, p] = (num * val["1 / den", g, c, p, n][None]).reshape(64, 128)
        if g % 2:
            for k in range(7):
                term = _lhs_term(
                    lambda n, p: jnp.concatenate([val["o", g - 1, c, n, p], val["o", g, c, n, p]], axis=0), k)
                words = pltpu.bitcast(term.astype(BF16).T, U32)
                o_terms[c][k, :, 64 * (g - 1):64 * (g + 1)] = words
                deadline(slot + SLACK, k, words[56:64])
            holds["o", c, g] = True
        else:
            for k, (n, p) in enumerate(((0, 0), (0, 1), (1, 0), (1, 1))):
                deadline(slot + SLACK, k, val["o", g, c, n, p][56:64])

    agenda = _agenda()

    def run_slot(s, plan, products, extras=(), wait=None):
        keys = [task for gc in agenda.get(("key", s), []) for task in key_tasks(*gc)]
        queries = [task for gc in agenda.get(("query", s), []) for task in query_tasks(*gc)]
        mixed = sorted([((i + 0.5) / len(keys), 0, i) for i in range(len(keys))]
                       + [((i + 0.5) / len(queries), 1, i) for i in range(len(queries))])
        pieces = _spread([(keys, queries)[kind][i] for _, kind, i in mixed], plan.count("q"))
        sums = _spread([task for gc in agenda.get(("sum", s), []) for task in summary_tasks(*gc)], plan.count("k"))
        products = list(products)
        assert plan.count("p") >= len(products) and ("f" in plan or not extras) and ("w" in plan or not wait)
        assert all(step in plan or (kind, s) not in agenda
                   for step, kind in (("q", "key"), ("q", "query"), ("k", "sum"), ("r", "read")))
        for step in plan:
            if step == "p" and products:
                products.pop(0)()
            elif step in "qk":
                for task in (pieces if step == "q" else sums).pop(0):
                    task()
            elif step == "r":
                for gc in agenda.get(("read", s), []):
                    readout(*gc, s)
            elif step == "f":
                for task in extras:
                    task(s)
            elif step == "w" and wait:
                wait()

    def shift():
        arrive(SHIFT_SLOT)
        val["sa"] = _rnd(_dot(cond, wmod_buf[:, 0:D])[0:8]) * LOG2E

    waits = {s: (lambda s=s: arrive(s)) for s in batches if isinstance(s, int)}
    waits[SHIFT_SLOT] = shift

    def mod_tasks():
        def piece(i, k):
            def run(slot):
                cols = released(cond_cols[k // 128])
                acc = val.get(("mod sum", i))
                for r in range(0, 128, 8):
                    term = (wmod_buf[k + r:k + r + 8, i * HD:(i + 1) * HD].astype(F32)
                            * jnp.concatenate([cols[r:r + 8]] * 4, axis=1))
                    acc = term if acc is None else acc + term
                val["mod sum", i] = acc
                for j in range(4):
                    deadline(slot + SLACK, 0, acc[:, 128 * j:128 * j + 128])
                if k == D - 128:
                    val["mod", i] = jnp.broadcast_to(_rnd(jnp.sum(acc, axis=0, keepdims=True)), (8, HD))
            return run
        return [piece(i, k) for i in range(4, 8) for k in range(0, D, 128)]

    extras = {s: [] for s in range(len(SLOTS))}

    def assign(tasks, slots):
        for s, chunk in zip(slots, _spread(tasks, len(slots))):
            extras[s] += chunk

    assign([lambda s, g=g: mix(g) for g in range(1, G)] + fold_tasks(1), [SLOT[1, 0] - 1])
    for c in range(1, NC):
        assign(norm_tasks(c), range(SLOT[0, c - 1], SLOT[0, c]))
    for g, slots in enumerate(([SHIFT_SLOT], range(SHIFT_SLOT + 1, SHIFT_SLOT + 4))):
        assign([lambda s, g=g, i=i, k=k: bias_part(g, i, k) for i in range(3) for k in range(0, HD, 128)], slots)
    for g in range(2, G):
        tasks, slots = fold_tasks(g), range(max((g - 1) * NC, FOLD_SLOT), g * NC - 1)
        assign(tasks[:8], slots)
        assign(tasks[8:], slots)
    assign(wo_tasks(), range(LATE_SLOT, len(SLOTS) - 2))
    assign(mod_tasks(), range(LATE_SLOT, len(SLOTS) - 4))

    for s, gc in enumerate(SLOTS):
        plan = (PLAN_FIRST if s == 0 else PLAN_STREAM if s < SHIFT_SLOT else PLAN_SHIFT if s == SHIFT_SLOT
                else PLAN_WAIT if s in waits and s > FOLD_SLOT else PLAN_STEADY)
        run_slot(s, plan, project_tasks(*gc), extras[s], waits.get(s))

    def mod_part(i):
        def run():
            lhs = _unpack(released(pltpu.bitcast(cond, U32)))
            val["mod", i] = _rnd(_dot(lhs, wmod_buf[:, i * HD:(i + 1) * HD])[0:8])
        return run

    mods = [mod_part(i) for i in range(8, 12)]
    for s, count in zip(range(len(SLOTS), TILE_SLOT), (1, 1, 2, 0)):
        run_slot(s, PLAN_DRAIN, [mods.pop(0) for _ in range(count)])
    assert not mods
    ga, sb, cb, gb = [jnp.concatenate([val["mod", 2 * i], val["mod", 2 * i + 1]], axis=1) for i in range(2, 6)]
    cb1 = _rnd(1.0 + cb)
    wr = jnp.broadcast_to(wr_buf[...].reshape(1, D).astype(F32), (8, D))
    coefs = {"attn": ga * (1.0 / LOG2E), "out mul": gb * cb1, "out add": gb * sb, "score": cb1 * wr,
             "h mul": cb1, "h add": sb, "gate": gb}
    for i, row in enumerate(coefs.values()):
        stored(coef_buf)[i] = row
    score_add = jnp.sum(sb * wr, axis=-1, keepdims=True)
    deadline(TILE_SLOT, PRODUCTS[0], gb)

    def coef(name):
        return coef_buf[0, list(coefs).index(name)]

    lane = _iota((8, 128), 1)
    scores = [jnp.zeros((8, 128), F32)] * 2

    def finish_rows(t, i, r):
        r0 = t * T + i * HT + r
        xs = []
        for e in (0, 8):
            a = jnp.concatenate(
                [_quadrant(lambda k: val["attn", t, k][r + e:r + e + 8], i, j) for j in range(2)], axis=1)
            xs.append(x_buf[r0 + e:r0 + e + 8, :].astype(F32) + coef("attn") * a)
            x1_buf[r0 + e:r0 + e + 8] = xs[-1]
        means = _row_means(xs)
        centred, var = _row_spread(xs, means)
        scales = _row_scales(var)
        scale_buf[r0 // 2:r0 // 2 + 8] = scales
        outs = []
        for k in range(2):
            scale = scales[:, k:k + 1]
            mean_buf[r0 + 8 * k:r0 + 8 * k + 8] = jnp.broadcast_to(_rnd(means[k]), (8, 128))
            outs.append(xs[k] + (centred[k] * scale * coef("out mul") + coef("out add")))
            score = jnp.sum(centred[k] * coef("score"), axis=-1, keepdims=True) * scale
            scores[r0 // 1024] = jnp.where(lane == (r0 // 8 + k) % 128, score, scores[r0 // 1024])
        rows = slice(r0 - t * T, r0 - t * T + 16)
        stored(out_bufs[t])[rows, :] = jnp.concatenate(outs, axis=0).astype(BF16)
        return pltpu.bitcast(out_bufs[t][0, rows, 0:128], U32), scores[r0 // 1024]

    pending = [(7 * t + EPILOGUE_LAG + k * 7 // 16, t, k) for t in range(NC) for k in range(16)]

    def flush(upto, slot=None, n=None):
        while pending and pending[0][0] <= upto:
            _, t, k = pending.pop(0)
            done = finish_rows(t, 1 - k // 8, 16 * (k % 8))
            if slot is not None:
                for dep in done:
                    deadline(slot, n, dep)
            if k == 15:
                out_copy(t).start()
                stored(out_bufs[t])[T:T + 16, 0:128] = jnp.zeros((16, 128), BF16)
                deadline(TILE_SLOT + (upto + 2) // 7, PRODUCTS[(upto + 2) % 7],
                         pltpu.bitcast(out_bufs[t][0, T:T + 16, 0:128], U32), 3)

    def tile_tasks(t):
        def product(j, n):
            def run():
                flush(7 * t + j, TILE_SLOT + t, n)
                assert all(("o", t, g) in holds for g in range(1, G, 2))
                assert all(("wo", r, l) in holds for r in range(0, HD // 2, 16) for l in range(0, HD, WO_COLS))
                rhs = meet(wo_terms[0, n], TILE_SLOT + t, n)
                val["last product"] = val["attn", t, n] = _dot(_unpack(o_terms[t][n]), _unpack(rhs))
            return run
        return [product(j, n) for j, n in enumerate(PRODUCTS)]

    for t in range(NC):
        run_slot(TILE_SLOT + t, PLAN_TILE, tile_tasks(t))
    flush(pending[-1][0])
    assert not batches

    r = _rnd(jnp.concatenate(scores, axis=0) + jnp.concatenate([score_add] * 2, axis=0))
    r = jnp.clip(jnp.where(r != r, -BF16_MAX, r), -BF16_MAX, BF16_MAX)
    r = jnp.where(jnp.abs(r) < F32_TINY, F32_TINY, r)
    token = (_iota((16, 128), 0) // 8) * 1024 + _iota((16, 128), 1) * 8 + _iota((16, 128), 0) % 8
    keys = pltpu.bitcast(pltpu.bitcast(r, jnp.int32) | jnp.where(r > 0, S - 1 - token, token), F32)
    picks = []
    for _ in range(2):
        top = jnp.max(jnp.max(keys, axis=0, keepdims=True), axis=1, keepdims=True)
        bits = pltpu.bitcast(jnp.broadcast_to(top, (8, 128)), jnp.int32)
        low = bits & (S - 1)
        picks.append((jnp.where(bits > 0, S - 1 - low, low), pltpu.bitcast(bits & -65536, F32)))
        keys = jnp.where(keys == top, -jnp.inf, keys)
    b1, b2 = [pl.multiple_of(jnp.clip(i[0, 0] // 16, 0, S // 16 - 1) * 16, 16) for i, _ in picks]

    def gather(ref):
        return jnp.concatenate([ref[pl.ds(b1, 16)], ref[pl.ds(b2, 16)]], axis=0)

    def wide(x):
        return jnp.concatenate([x] * (D // 128), axis=1)

    x1 = gather(x1_buf)
    stats = [scale_buf[pl.ds(pl.multiple_of(b // 2, 8), 8)] for b in (b1, b2)]
    scale = jnp.concatenate([sv[:, i:i + 1] for sv in stats for i in range(2)], axis=0)
    h2 = (x1 - wide(gather(mean_buf))) * scale * coef("h mul")[0:1] + coef("h add")[0:1]
    hb = h2.astype(BF16)
    u = _dot(hb, wg_buf[...])
    act = u * jax.nn.sigmoid(u) * _dot(hb, wu_buf[...])
    y = _dot(act.astype(BF16), wd_buf[:, 0:D])
    rows = _iota((32, 128), 0)
    rows = jnp.where(rows < 16, rows + b1, rows - 16 + b2)
    update = jnp.zeros((32, D), F32)
    for i, score in picks:
        hit = wide(rows == jnp.concatenate([i] * 4, axis=0))
        update = jnp.where(hit, y * wide(jax.nn.sigmoid(score))[0:1], update)
    fix_buf[...] = (x1 + coef("gate")[0:1] * (h2 + update)).astype(BF16)

    for t in range(NC):
        out_copy(t).wait()
    fix1 = pltpu.make_async_copy(fix_buf.at[0:16], out_hbm.at[pl.ds(b1, 16)], sem_out)
    fix2 = pltpu.make_async_copy(fix_buf.at[16:32], out_hbm.at[pl.ds(b2, 16)], sem_out)
    fix1.start()

    @pl.when(b1 != b2)
    def _():
        fix2.start()
        fix2.wait()

    fix1.wait()


@jax.jit
def pallas_adaLN_cond__linear_kernel_hedgehog__moe_arch_mod__prompt_kernel(
    A_x: jax.Array,
    A_wqkv: jax.Array,
    A_w_phi: jax.Array,
    A_wo: jax.Array,
    B_x: jax.Array,
    B_w_r: jax.Array,
    B_w_gate: jax.Array,
    B_w_up: jax.Array,
    B_w_down: jax.Array,
    c: jax.Array,
    w_mod: jax.Array,
):
    hbm = pl.BlockSpec(memory_space=pl.ANY)
    vmem = pltpu.VMEM
    out = pl.pallas_call(
        _kernel,
        out_shape=jax.ShapeDtypeStruct((S, D), BF16),
        in_specs=[hbm] * 10,
        out_specs=hbm,
        scratch_shapes=[
            vmem((S, D), BF16),
            vmem((3, G, D, 128), BF16),
            vmem((H, DH, DH), BF16),
            vmem((D, D), BF16),
            vmem((D,), BF16),
            vmem((D, F), BF16),
            vmem((D, F), BF16),
            vmem((F, D + 128), BF16),
            vmem((1, D), BF16),
            vmem((D, 6 * D + 128), BF16),
            [vmem((7, HT // 2, HD), U32)] * NC,
            [vmem((7, 96, HD), U32)] * 3,
            [vmem((NC, 2, 2, 64, 128), F32)] * 3,
            [vmem((7, HT // 2, HD), U32)] * NC,
            vmem((1, 7, HD // 2, HD), U32),
            vmem((S, D), F32),
            vmem((S, 128), F32),
            vmem((S // 2, 128), F32),
            [vmem((1, T + 16, D), BF16)] * NC,
            vmem((1, 7, 8, D), F32),
            vmem((32, D), BF16),
            pltpu.SemaphoreType.DMA((NC + 5 + HD // SCALE_COLS,)),
        ],
        compiler_params=pltpu.CompilerParams(vmem_limit_bytes=120 * 2**20),
        name="adaln_hedgehog_mod",
    )(A_x.reshape(S, D), A_wqkv, A_w_phi, A_wo, B_w_r, B_w_gate, B_w_up, B_w_down, c, w_mod)
    return out.reshape(1, S, D)
```

```python
import numpy as np

import jax
import jax.numpy as jnp
from jax import lax
import jax.experimental.pallas as pl
import jax.experimental.pallas.tpu as pltpu

S, D, H, DH, F = 2048, 1024, 32, 32, 3584
G = 8
HD, QD = D // 2, D // 4
T = 256
HT = T // 2
NC = S // T

LOG2E = float(np.log2(np.e))
BF16_MAX = 3.3895313892515355e38
F32_TINY = float(np.finfo(np.float32).tiny)
NT = (((1,), (1,)), ((), ()))
NN = (((1,), (0,)), ((), ()))
F32, BF16, U32 = jnp.float32, jnp.bfloat16, jnp.uint32

LEAD_IN = [int(g) for g in "0000010101011111"]
SLOTS = [(g, LEAD_IN[:i].count(g)) for i, g in enumerate(LEAD_IN)] + [(g, c) for g in range(2, G) for c in range(NC)]
SLOT = {gc: s for s, gc in enumerate(SLOTS)}
PRODUCTS = (3, 1, 0, 2, 5, 4, 6)
SHIFT_SLOT, FOLD_SLOT, LATE_SLOT = 7, 10, 23
TILE_SLOT = len(SLOTS) + 4
DEEP = 2
DEEP_SLOTS = range(10, DEEP * NC + 5)
SUMMED = (0, 2, 3, 5, 6)
SCALE_COLS, WO_COLS = 256, 256
SLACK = 3
EPILOGUE_LAG = 9

PLAN_FIRST, PLAN_STREAM = "ppppppwpf", "wpppppppf"
PLAN_SHIFT, PLAN_WAIT = "pppwppppkkqqqqqqrqqf", "pppkkpwpppqqqqqqrqqf"
PLAN_STEADY = "pwkkqpqfpqpqfpqpqfprqpq"
PLAN_DRAIN, PLAN_TILE = "kkqpppprpppp", "pkkpqpqpqpqprp"


def _dot(a, b, dims=NN):
    return lax.dot_general(a, b, dims, preferred_element_type=F32)


def _rnd(x):
    return x.astype(BF16).astype(F32)


def _iota(shape, axis):
    return lax.broadcasted_iota(jnp.int32, shape, axis)


def _pack(even, odd):
    return pltpu.pack_elementwise([even, odd], packed_dtype=BF16)


def _pack_halves(x):
    n = x.shape[0] // 2
    return _pack(x[:n], x[n:])


def _unpack(words):
    return pltpu.bitcast(words, BF16)


def _split(x):
    words = pltpu.bitcast(x, U32)
    return [pltpu.unpack_elementwise(words, index=i, packed_dtype=BF16, unpacked_dtype=F32) for i in range(2)]


def _interleave_halves(x):
    return _unpack(_pack_halves(x)).astype(F32) + _unpack(_pack_halves(x - _rnd(x))).astype(F32)


def _tree(x3, op):
    return op(op(op(x3[0], x3[1]), op(x3[2], x3[3])), op(op(x3[4], x3[5]), op(x3[6], x3[7])))


def _fold_rows(m, op):
    m = op(m, pltpu.roll(m, 2, 0))
    return op(m, pltpu.roll(m, 4, 0))


def _softmax2(p3, sign):
    if sign == 0:
        e = jnp.exp2(p3 - _fold_rows(_tree(p3, jnp.maximum), jnp.maximum)[None])
    else:
        e = jnp.exp2(_fold_rows(_tree(p3, jnp.minimum), jnp.minimum)[None] - p3)
    return e * pl.reciprocal(_fold_rows(_tree(e, jnp.add), jnp.add), full_range=False)[None]


def _row_means(xs):
    return [jnp.mean(x, axis=-1, keepdims=True) for x in xs]


def _row_spread(xs, means):
    lane = _iota((xs[0].shape[0], 128), 1)
    centred, var = [], None
    for i, (x, mean) in enumerate(zip(xs, means)):
        rounded = _rnd(mean)
        d = x - rounded
        v = jnp.mean(d * d, axis=-1, keepdims=True) - (mean - rounded) * (mean - rounded)
        var = jnp.where(lane == i, v, var) if i else jnp.broadcast_to(v, lane.shape)
        centred.append(d)
    return centred, var


def _row_scales(var):
    return 1.0 / _rnd(jnp.sqrt(_rnd(_rnd(var) + _rnd(jnp.full_like(var, 1e-5)))))


def _lhs_term(a, n):
    return (lambda: a(0, 0) + a(1, 1), lambda: a(1, 0) + a(1, 1), lambda: a(0, 0), lambda: a(1, 1),
            lambda: a(0, 0) + a(0, 1), lambda: a(1, 0) - a(0, 0), lambda: a(0, 1) - a(1, 1))[n]()


def _rhs_term(b, n):
    return (lambda: b(0, 0) + b(1, 1), lambda: b(0, 0), lambda: b(0, 1) - b(1, 1), lambda: b(1, 0) - b(0, 0),
            lambda: b(1, 1), lambda: b(0, 0) + b(0, 1), lambda: b(1, 0) + b(1, 1))[n]()


def _quadrant(m, i, j):
    if (i, j) == (0, 0):
        return (m(0) + m(3)) + (m(6) - m(4))
    if (i, j) == (0, 1):
        return m(2) + m(4)
    if (i, j) == (1, 0):
        return m(1) + m(3)
    return (m(0) - m(1)) + (m(2) + m(5))


def _spread(tasks, n):
    return [tasks[i * len(tasks) // n:(i + 1) * len(tasks) // n] for i in range(n)]


def _agenda():
    total, agenda = len(SLOTS), {}

    def key_slot(s):
        lag = 1 if SLOTS[s][0] < DEEP or s == total - 1 else 2
        return max(s + lag, SHIFT_SLOT + 2 + s // 2)

    def ready(g):
        return key_slot(SLOT[g, NC - 1]) + 2

    for s, gc in enumerate(SLOTS):
        agenda.setdefault(("key", key_slot(s)), []).append(gc)
        agenda.setdefault(("sum", key_slot(s) + 1), []).append(gc)
    for u in range(total):
        g, c = divmod(u, NC)
        s = min(max(ready(0) + u * (total + 2 + NC - ready(0)) // total, ready(g)), TILE_SLOT + c - 2)
        assert s >= ready(g)
        agenda.setdefault(("query", s), []).append((g, c))
        agenda.setdefault(("read", s + 1), []).append((g, c))
    return agenda


def _kernel(x_hbm, wqkv_hbm, wphi_hbm, wo_hbm, wr_hbm, wg_hbm, wu_hbm, wd_hbm, c_hbm, wmod_hbm,
            out_hbm,
            x_buf, w_buf, wphi_buf, wo_buf, wr_buf, wg_buf, wu_buf, wd_buf, c_buf, wmod_buf,
            h_terms, h_deep, w_terms, w_deep, pq_bufs, o_terms, wo_terms, x1_buf, mean_buf, scale_buf, out_bufs, coef_buf,
            fix_buf, sem):
    def x_rows(j):
        return [(x_hbm.at[pl.ds(j * T, T)], x_buf.at[pl.ds(j * T, T)])]

    def weights(*groups):
        return [(wqkv_hbm.at[:, pl.ds(i * D + g * 128, 128)], w_buf.at[i, g]) for g in groups for i in range(3)]

    def mod_cols(lo, n):
        return [(wmod_hbm.at[:, pl.ds(lo, n)], wmod_buf.at[:, pl.ds(lo, n)])]

    early = {SLOT[0, c - 1]: x_rows(c) for c in range(1, NC)}
    early[SLOT[1, 0] - 1] = weights(1) + [(wphi_hbm.at[4:H], wphi_buf.at[4:H])] + early[SLOT[1, 0] - 1]
    early[SHIFT_SLOT] = mod_cols(0, D)
    early[FOLD_SLOT] = weights(2, 3)
    batches = {
        "start": [(c_hbm, c_buf), (wphi_hbm.at[0:4], wphi_buf.at[0:4])] + weights(0) + x_rows(0),
        **{("scale", k): mod_cols(D + k, SCALE_COLS) + mod_cols(D + HD + k, SCALE_COLS)
           for k in range(0, HD, SCALE_COLS)},
        **dict(sorted(early.items())),
        LATE_SLOT: weights(*range(4, G)) + [(wr_hbm, wr_buf), (wo_hbm, wo_buf)] + mod_cols(2 * D, 2 * D),
        len(SLOTS) - 1: mod_cols(4 * D, 2 * D) + [(wg_hbm, wg_buf), (wu_hbm, wu_buf), (wd_hbm, wd_buf.at[:, 0:D])],
    }
    batches = {name: [pltpu.make_async_copy(src, dst, sem.at[i]) for src, dst in pairs]
               for i, (name, pairs) in enumerate(batches.items())}
    sem_out = sem.at[len(batches)]
    for copies in batches.values():
        for copy in copies:
            copy.start()

    def arrive(name):
        for copy in batches.pop(name):
            copy.wait()

    def out_copy(t):
        return pltpu.make_async_copy(out_bufs[t].at[0, 0:T], out_hbm.at[pl.ds(t * T, T)], sem_out)

    zero, other_zero = [jnp.min(_iota((8, 128), axis)) for axis in range(2)]
    never = _iota((8, 128), 1) < other_zero
    val, due, holds, recent = {}, {}, {}, []

    def stored(ref):
        return ref.at[zero]

    def after(x, dep, r=0):
        head = jnp.where(never, pltpu.bitcast(dep[0:8, 0:128], x.dtype), x[r:r + 8, 0:128])
        if x.shape[1] > 128:
            head = jnp.concatenate([head, x[r:r + 8, 128:]], axis=1)
        parts = ([x[:r]] if r else []) + [head] + ([x[r + 8:]] if x.shape[0] > r + 8 else [])
        return jnp.concatenate(parts, axis=0)

    def released(x):
        return after(x, val["last product"]) if "last product" in val else x

    def deadline(slot, n, dep, j=0):
        due.setdefault((slot, n, j), []).append(dep)

    def soon(lag, dep, j):
        at = val["position"] + lag
        if at < 7 * len(SLOTS):
            deadline(at // 7, PRODUCTS[at % 7], dep, j)

    def meet(x, slot, n, keys=range(4)):
        cols = [x[:, l:l + 128] for l in range(0, x.shape[1], 128)]
        for l, j in zip(range(len(cols)), keys):
            for i, dep in enumerate(due.pop((slot, n, j), [])):
                cols[l] = after(cols[l], dep, 8 * i % x.shape[0])
        return jnp.concatenate(cols, axis=1)

    same_head = _iota((128, 128), 0) // DH == _iota((128, 128), 1) // DH
    pick_feature = (_iota((128, DH), 0) % DH == _iota((128, DH), 1)).astype(BF16)

    def mix(g):
        wp = wphi_buf[g * 4:g * 4 + 4].reshape(128, DH)
        val["mix", g] = jnp.where(same_head, _dot(pick_feature, wp, NT), 0.0)

    def bias_part(g, i, k):
        left, right = val["folded", g, i, k]
        term = (left.reshape(16, 8, 128) * val["sa"][:, k:k + 128][None]
                + right.reshape(16, 8, 128) * val["sa"][:, HD + k:HD + k + 128][None])
        val["bias", g, i] = term if k == 0 else val["bias", g, i] + term
        if k == HD - 128:
            b = jnp.sum(val["bias", g, i], axis=-1, keepdims=True)
            b = jnp.broadcast_to(b, (16, 8, 128)).reshape(128, 128)
            for p in range(2):
                val["bias", g, i, p] = _interleave_halves(b[64 * p:64 * p + 64])

    def fold_tasks(g):
        def part(i, k):
            def run(slot):
                halves = []
                for lo in (k, HD + k):
                    w = _unpack(released(pltpu.bitcast(w_buf[i, g, lo:lo + 128, :], U32)))
                    halves.append(_dot(val["mix", g].astype(BF16), w, NT) if i < 2 else w.astype(F32).T)
                val["folded", g, i, k] = halves
                if g > 1:
                    bias_part(g, i, k)
                if g >= DEEP:
                    return
                for n in range(7):
                    words = _pack_halves(_lhs_term(lambda p, j: halves[j][64 * p:64 * p + 64], n))
                    w_terms[g][n, 32 * i:32 * i + 32, k:k + 128] = words
                holds["w", g, i, k] = True
                if slot is not None:
                    deadline(slot + SLACK, 1 + k // 128, words)
            return run

        def deep_terms(i, k, r):
            def run(slot):
                folded = [val["folded", g, i, k + j * QD] for j in range(2)]
                for n in PRODUCTS:
                    terms = {(j, q): _lhs_term(lambda p, l: folded[j][l][64 * p + q:64 * p + q + 8], n)
                             for j in range(2) for q in range(r, 64, 16)}
                    for m in range(7):
                        words = _pack(*[_lhs_term(lambda a, j: terms[j, e + 16 * a + r], m) for e in (0, DH)])
                        w_deep[g % 3][n, m, 16 * i + r:16 * i + r + 8, k:k + 128] = words
                    holds["w deep", g % 3, i, k, r, n] = g
                    deadline(slot + SLACK, n, words, 1 + i)
                    if n in (PRODUCTS[3], PRODUCTS[6]):
                        soon(3, words, 1)
            return run

        if g < DEEP:
            return [part(i, k) for i in range(3) for k in range(0, HD, 128)]
        return [task for i in range(3) for k in range(0, QD, 128)
                for task in (part(i, k), part(i, k + QD), deep_terms(i, k, 0), deep_terms(i, k, 8))]

    def wo_tasks():
        def piece(r, l):
            def run(slot):
                quads = {}
                for e in range(2):
                    for i in range(2):
                        lo = r // DH * 128 + r % DH + i * 64 + DH * e
                        for j in range(2):
                            w = wo_buf[lo:lo + 16, j * HD + l:j * HD + l + WO_COLS].astype(F32)
                            quads[e, i, j] = released(w)
                for n in range(7):
                    words = _pack(*[_rhs_term(lambda i, j: quads[e, i, j], n) for e in range(2)])
                    stored(wo_terms)[n, r:r + 16, l:l + WO_COLS] = words
                holds["wo", r, l] = True
                soon(3, wo_terms[0, 6, r:r + 8, l:l + 128], 3)
                deadline(slot + SLACK, (r // 16 + l // 128) % 7, wo_terms[0, 0, r:r + 8, l:l + 128])
            return run
        return [piece(r, l) for r in range(0, HD // 2, 16) for l in range(0, HD, WO_COLS)]

    def norm_means(c, r):
        rows = [slice(c * T + n * HT + r, c * T + n * HT + r + 16) for n in range(2)]
        xs = [x for n in range(2) for x in _split(x_buf[rows[n], :])]
        val["norm", c, r] = xs, _row_means(xs)

    def norm_spread(c, r):
        val["norm", c, r] = _row_spread(*val["norm", c, r])

    def norm_scales(c, r):
        centred, var = val["norm", c, r]
        scales = _row_scales(var)
        val["norm", c, r] = [(d, scales[:, i:i + 1]) for i, d in enumerate(centred)]

    def norm_stats(c, r):
        for stage, lag in ((norm_means, 0), (norm_spread, 16), (norm_scales, 32)):
            if 0 <= r - lag < HT:
                stage(c, r - lag)

    def norm_terms(c, r, k):
        h = {}
        for j in range(2):
            for n in range(2):
                for e in range(2):
                    d, scale = val["norm", c, r][2 * n + e]
                    h[e, j, n] = d[:, j * HD + k:j * HD + k + 128] * scale * val["scale", j * HD + k]
        for n in range(7):
            words = _pack(*[_rhs_term(lambda j, m: h[e, j, m], n) for e in range(2)])
            h_terms[c][n, r // 2:r // 2 + 8, k:k + 128] = words
        holds["h", c, r, k] = True
        return words

    def norm_tasks(c):
        def step(r):
            def run(slot):
                norm_stats(c, r)
                if r >= 32:
                    for k in range(0, HD, 128):
                        words = norm_terms(c, r - 32, k)
                    if slot + 1 < SLOT[0, c]:
                        deadline(slot + 1, PRODUCTS[r // 16 % 4], words)
            return run
        return [step(r) for r in range(0, HT + 32, 16)]

    def deep_tasks(pair):
        def piece(n, k):
            def run(slot):
                assert all(("h", 2 * pair + 1, r, l) in holds for r in range(0, HT, 16) for l in range(0, HD, 128))
                parts = {(j, l): _split(_unpack(released(h_terms[2 * pair + l][n, :, j * QD + k:j * QD + k + 128])))
                         for j in range(2) for l in range(2)}
                for i, m in enumerate(SUMMED):
                    words = _pack(*[_rhs_term(lambda j, l: parts[j, l][e], m) for e in range(2)])
                    h_deep[pair][n, i, :, k:k + 128] = words
                    deadline(slot + SLACK - 1, (n + i) % 7, words[56:64], 2)
                    if i in (1, 4):
                        soon(3, words[56:64], 1)
                holds["h deep", pair, n, k] = True
            return run
        return [piece(n, k) for n in PRODUCTS for k in range(0, QD, 128)]

    arrive("start")
    mix(0)
    for task in fold_tasks(0):
        task(None)
    cv = c_buf[...].astype(F32)
    cond = jnp.broadcast_to(_rnd(cv * _rnd(jax.nn.sigmoid(cv))), (16, D)).astype(BF16)
    for r in range(0, HT + 32, 16):
        norm_stats(0, r)
    cond_rows = jnp.broadcast_to(cond[0:1].astype(F32), (128, D))
    cond_cols = [cond_rows[:, k:k + 128].T for k in range(0, D, 128)]
    for k in range(0, HD, SCALE_COLS):
        arrive(("scale", k))
        for lo in (k, HD + k):
            block = _rnd(1.0 + _rnd(_dot(cond, wmod_buf[:, D + lo:D + lo + SCALE_COLS])[0:8])) * LOG2E
            for l in range(0, SCALE_COLS, 128):
                val["scale", lo + l] = block[:, l:l + 128]
        for r in range(0, HT, 16):
            for l in range(k, k + SCALE_COLS, 128):
                norm_terms(0, r, l)

    kv_mask = _iota((64, 128), 0) % 2 == (_iota((64, 128), 1) // 2) % 2

    def project_tasks(g, c):
        def product(n):
            def run():
                assert all(("w", g, i, k) in holds for i in range(3) for k in range(0, HD, 128))
                assert all(("h", c, r, k) in holds for r in range(0, HT, 16) for k in range(0, HD, 128))
                rhs = meet(h_terms[c][n], SLOT[g, c], n)
                val["last product"] = val["qkv", g, c, n] = _dot(_unpack(w_terms[g][n]), _unpack(rhs), NT)
            return run

        def deep_products(step, inner):
            def run():
                for q, (n, m) in enumerate(inner):
                    assert all(holds["w deep", g % 3, i, k, r, n] == g
                               for i in range(3) for k in range(0, QD, 128) for r in (0, 8))
                    assert all(("h deep", c // 2, n, k) in holds for k in range(0, QD, 128))
                    if m in SUMMED:
                        rhs = h_deep[c // 2][n, SUMMED.index(m)]
                    else:
                        rhs = h_terms[c - c % 2 + m // 4][n, :, m // 4 * QD:m // 4 * QD + QD]
                    rhs = meet(rhs, SLOT[g, c], step, (q, 3 if q == len(inner) - 1 else None))
                    val["inner", m] = _dot(_unpack(w_deep[g % 3][n, m]), _unpack(rhs), NT)
                    recent.append(val["inner", m])
                    val["last product"] = recent[-6:][0]
                    if m == PRODUCTS[-1]:
                        for l in range(2):
                            halves = [_quadrant(lambda k: val["inner", k], a, l) for a in range(2)]
                            val["qkv", g, c - c % 2 + l, n] = jnp.concatenate(
                                [x[32 * i:32 * i + 32] for i in range(3) for x in halves], axis=0)
            return run

        if g < DEEP:
            return [product(n) for n in PRODUCTS]
        steps = _spread([(n, m) for n in PRODUCTS for m in PRODUCTS], 14)[c % 2 * 7:c % 2 * 7 + 7]
        return [deep_products(step, inner) for step, inner in zip(PRODUCTS, steps)]

    def key_tasks(g, c):
        def piece(p, n):
            def run():
                def part(i):
                    y = _quadrant(lambda k: val["qkv", g, c, k][64 * i:64 * i + 64], p, n)
                    return y + val["bias", g, i, p] if i < 2 else y
                pq_bufs[g % 3][c, p, n] = part(0)
                holds["pq", g % 3, c, p, n] = g
                val["v", g, c, p, n] = part(2)
                logits = part(1).reshape(8, 8, 128)
                words = []
                for sign in range(2):
                    phi = _softmax2(logits, sign)
                    words.append(_pack_halves(phi.reshape(64, 128)))
                    val["z", g, p, sign] = val["z", g, p, sign] + phi if ("z", g, p, sign) in val else phi
                val["phi_k", g, c, p, n] = jnp.concatenate(words, axis=0)
                for sign in range(2):
                    soon(1, words[sign][24:32], 2 * sign)
            return run
        return [piece(p, n) for p, n in ((1, 0), (0, 1), (1, 1), (0, 0))]

    def summary_tasks(g, c):
        def piece(p):
            def run():
                v = jnp.concatenate([val["v", g, c, p, n] for n in range(2)], axis=1).astype(BF16)
                phi = _unpack(jnp.concatenate([val["phi_k", g, c, p, n] for n in range(2)], axis=1))
                kv = _dot(v, phi, NT)
                val["kv", g, p] = kv if c == 0 else val["kv", g, p] + kv
                if c == NC - 1:
                    for sign in range(2):
                        z = jnp.sum(val["z", g, p, sign], axis=-1, keepdims=True)
                        val["z total", g, p, sign] = jnp.broadcast_to(z, (8, 8, 128))
                    z_row = jnp.concatenate(
                        [_interleave_halves(val["z total", g, p, sign].reshape(64, 128)) for sign in range(2)],
                        axis=0).T[0:64]
                    val["kv", g, p] = jnp.where(kv_mask, val["kv", g, p] + val["bias", g, 2, p] * z_row, 0.0)
            return run
        return [piece(p) for p in range(2)]

    def query_tasks(g, c):
        def piece(p, n):
            def run():
                assert holds["pq", g % 3, c, p, n] == g
                logits = released(pq_bufs[g % 3][c, p, n]).reshape(8, 8, 128)
                words, den = [], None
                for sign in range(2):
                    phi = _softmax2(logits, sign)
                    words.append(_pack_halves(phi.reshape(64, 128)))
                    w = _tree(phi * val["z total", g, p, sign], jnp.add)
                    den = w if den is None else den + w
                val["1 / den", g, c, p, n] = pl.reciprocal(_fold_rows(den, jnp.add) + 1e-6, full_range=False)
                val["phi_q", g, c, p, n] = jnp.concatenate(words, axis=0)
                for sign in range(2):
                    soon(1, words[sign][24:32], 2 * sign)
            return run
        return [piece(p, n) for n in range(2) for p in range(2)]

    def readout(g, c, slot):
        nums = [_dot(val["kv", g, p].astype(BF16),
                     _unpack(jnp.concatenate([val["phi_q", g, c, p, n] for n in range(2)], axis=1)))
                for p in range(2)]
        for p in range(2):
            for n in range(2):
                num = nums[p][:, n * HT:(n + 1) * HT].reshape(8, 8, 128)
                val["o", g, c, n, p] = (num * val["1 / den", g, c, p, n][None]).reshape(64, 128)
        if g % 2:
            for k in range(7):
                term = _lhs_term(
                    lambda n, p: jnp.concatenate([val["o", g - 1, c, n, p], val["o", g, c, n, p]], axis=0), k)
                words = pltpu.bitcast(term.astype(BF16).T, U32)
                o_terms[c][k, :, 64 * (g - 1):64 * (g + 1)] = words
                deadline(slot + SLACK, k, words[56:64])
            holds["o", c, g] = True
        else:
            for k, (n, p) in enumerate(((0, 0), (0, 1), (1, 0), (1, 1))):
                deadline(slot + SLACK, k, val["o", g, c, n, p][56:64])

    agenda = _agenda()

    def run_slot(s, plan, products, extras=(), wait=None):
        keys = [task for gc in agenda.get(("key", s), []) for task in key_tasks(*gc)]
        queries = [task for gc in agenda.get(("query", s), []) for task in query_tasks(*gc)]
        mixed = sorted([((i + 0.5) / len(keys), 0, i) for i in range(len(keys))]
                       + [((i + 0.5) / len(queries), 1, i) for i in range(len(queries))])
        pieces = _spread([(keys, queries)[kind][i] for _, kind, i in mixed], plan.count("q"))
        sums = _spread([task for gc in agenda.get(("sum", s), []) for task in summary_tasks(*gc)], plan.count("k"))
        products, sides = list(products), _spread(list(extras), plan.count("f"))
        assert plan.count("p") >= len(products) and ("f" in plan or not extras) and ("w" in plan or not wait)
        assert all(step in plan or (kind, s) not in agenda
                   for step, kind in (("q", "key"), ("q", "query"), ("k", "sum"), ("r", "read")))
        val["position"] = 7 * s
        for step in plan:
            val["position"] += step == "p"
            if step == "p" and products:
                products.pop(0)()
            elif step in "qk":
                for task in (pieces if step == "q" else sums).pop(0):
                    task()
            elif step == "r":
                for gc in agenda.get(("read", s), []):
                    readout(*gc, s)
            elif step == "f":
                for task in sides.pop(0):
                    task(s)
            elif step == "w" and wait:
                wait()

    def shift():
        arrive(SHIFT_SLOT)
        val["sa"] = _rnd(_dot(cond, wmod_buf[:, 0:D])[0:8]) * LOG2E

    waits = {s: (lambda s=s: arrive(s)) for s in batches if isinstance(s, int)}
    waits[SHIFT_SLOT] = shift

    def mod_tasks():
        def piece(i, k):
            def run(slot):
                cols = released(cond_cols[k // 128])
                acc = val.get(("mod sum", i))
                for r in range(0, 128, 8):
                    term = (wmod_buf[k + r:k + r + 8, i * HD:(i + 1) * HD].astype(F32)
                            * jnp.concatenate([cols[r:r + 8]] * 4, axis=1))
                    acc = term if acc is None else acc + term
                val["mod sum", i] = acc
                for j in range(4):
                    deadline(slot + SLACK, 0, acc[:, 128 * j:128 * j + 128])
                if k == D - 128:
                    val["mod", i] = jnp.broadcast_to(_rnd(jnp.sum(acc, axis=0, keepdims=True)), (8, HD))
            return run
        return [piece(i, k) for i in range(4, 8) for k in range(0, D, 128)]

    extras = {s: [] for s in range(len(SLOTS))}

    def assign(tasks, slots):
        for s, chunk in zip(slots, _spread(tasks, len(slots))):
            extras[s] += chunk

    assign([lambda s, g=g: mix(g) for g in range(1, G)] + fold_tasks(1), [SLOT[1, 0] - 1])
    for c in range(1, NC):
        assign(norm_tasks(c), range(SLOT[0, c - 1], SLOT[0, c]))
    for g, slots in enumerate(([SHIFT_SLOT], range(SHIFT_SLOT + 1, SHIFT_SLOT + 4))):
        assign([lambda s, g=g, i=i, k=k: bias_part(g, i, k) for i in range(3) for k in range(0, HD, 128)], slots)
    for g in range(2, G):
        tasks, slots = fold_tasks(g), range(max((g - 1) * NC, FOLD_SLOT), g * NC - 1)
        assign(tasks[:len(tasks) * 2 // 3], slots)
        assign(tasks[len(tasks) * 2 // 3:], slots)
    assign([task for pair in range(NC // 2) for task in deep_tasks(pair)], DEEP_SLOTS)
    assign(wo_tasks(), range(LATE_SLOT, len(SLOTS) - 2))
    assign(mod_tasks(), range(LATE_SLOT, len(SLOTS) - 4))

    for s, gc in enumerate(SLOTS):
        plan = (PLAN_FIRST if s == 0 else PLAN_STREAM if s < SHIFT_SLOT else PLAN_SHIFT if s == SHIFT_SLOT
                else PLAN_WAIT if s in waits and s > FOLD_SLOT else PLAN_STEADY)
        run_slot(s, plan, project_tasks(*gc), extras[s], waits.get(s))

    def mod_part(i):
        def run():
            lhs = _unpack(released(pltpu.bitcast(cond, U32)))
            val["mod", i] = _rnd(_dot(lhs, wmod_buf[:, i * HD:(i + 1) * HD])[0:8])
        return run

    mods = [mod_part(i) for i in range(8, 12)]
    for s, count in zip(range(len(SLOTS), TILE_SLOT), (1, 1, 2, 0)):
        run_slot(s, PLAN_DRAIN, [mods.pop(0) for _ in range(count)])
    assert not mods
    ga, sb, cb, gb = [jnp.concatenate([val["mod", 2 * i], val["mod", 2 * i + 1]], axis=1) for i in range(2, 6)]
    cb1 = _rnd(1.0 + cb)
    wr = jnp.broadcast_to(wr_buf[...].reshape(1, D).astype(F32), (8, D))
    coefs = {"attn": ga * (1.0 / LOG2E), "out mul": gb * cb1, "out add": gb * sb, "score": cb1 * wr,
             "h mul": cb1, "h add": sb, "gate": gb}
    for i, row in enumerate(coefs.values()):
        stored(coef_buf)[i] = row
    score_add = jnp.sum(sb * wr, axis=-1, keepdims=True)
    deadline(TILE_SLOT, PRODUCTS[0], gb)

    def coef(name):
        return coef_buf[0, list(coefs).index(name)]

    lane = _iota((8, 128), 1)
    scores = [jnp.zeros((8, 128), F32)] * 2

    def finish_rows(t, i, r):
        r0 = t * T + i * HT + r
        xs = []
        for e in (0, 8):
            a = jnp.concatenate(
                [_quadrant(lambda k: val["attn", t, k][r + e:r + e + 8], i, j) for j in range(2)], axis=1)
            xs.append(x_buf[r0 + e:r0 + e + 8, :].astype(F32) + coef("attn") * a)
            x1_buf[r0 + e:r0 + e + 8] = xs[-1]
        means = _row_means(xs)
        centred, var = _row_spread(xs, means)
        scales = _row_scales(var)
        scale_buf[r0 // 2:r0 // 2 + 8] = scales
        outs = []
        for k in range(2):
            scale = scales[:, k:k + 1]
            mean_buf[r0 + 8 * k:r0 + 8 * k + 8] = jnp.broadcast_to(_rnd(means[k]), (8, 128))
            outs.append(xs[k] + (centred[k] * scale * coef("out mul") + coef("out add")))
            score = jnp.sum(centred[k] * coef("score"), axis=-1, keepdims=True) * scale
            scores[r0 // 1024] = jnp.where(lane == (r0 // 8 + k) % 128, score, scores[r0 // 1024])
        rows = slice(r0 - t * T, r0 - t * T + 16)
        stored(out_bufs[t])[rows, :] = jnp.concatenate(outs, axis=0).astype(BF16)
        return pltpu.bitcast(out_bufs[t][0, rows, 0:128], U32), scores[r0 // 1024]

    pending = [(7 * t + EPILOGUE_LAG + k * 7 // 16, t, k) for t in range(NC) for k in range(16)]

    def flush(upto, slot=None, n=None):
        while pending and pending[0][0] <= upto:
            _, t, k = pending.pop(0)
            done = finish_rows(t, 1 - k // 8, 16 * (k % 8))
            if slot is not None:
                for dep in done:
                    deadline(slot, n, dep)
            if k == 15:
                out_copy(t).start()
                stored(out_bufs[t])[T:T + 16, 0:128] = jnp.zeros((16, 128), BF16)
                deadline(TILE_SLOT + (upto + 2) // 7, PRODUCTS[(upto + 2) % 7],
                         pltpu.bitcast(out_bufs[t][0, T:T + 16, 0:128], U32), 3)

    def tile_tasks(t):
        def product(j, n):
            def run():
                flush(7 * t + j, TILE_SLOT + t, n)
                assert all(("o", t, g) in holds for g in range(1, G, 2))
                assert all(("wo", r, l) in holds for r in range(0, HD // 2, 16) for l in range(0, HD, WO_COLS))
                rhs = meet(wo_terms[0, n], TILE_SLOT + t, n)
                val["last product"] = val["attn", t, n] = _dot(_unpack(o_terms[t][n]), _unpack(rhs))
            return run
        return [product(j, n) for j, n in enumerate(PRODUCTS)]

    for t in range(NC):
        run_slot(TILE_SLOT + t, PLAN_TILE, tile_tasks(t))
    flush(pending[-1][0])
    assert not batches

    r = _rnd(jnp.concatenate(scores, axis=0) + jnp.concatenate([score_add] * 2, axis=0))
    r = jnp.clip(jnp.where(r != r, -BF16_MAX, r), -BF16_MAX, BF16_MAX)
    r = jnp.where(jnp.abs(r) < F32_TINY, F32_TINY, r)
    token = (_iota((16, 128), 0) // 8) * 1024 + _iota((16, 128), 1) * 8 + _iota((16, 128), 0) % 8
    keys = pltpu.bitcast(pltpu.bitcast(r, jnp.int32) | jnp.where(r > 0, S - 1 - token, token), F32)
    picks = []
    for _ in range(2):
        top = jnp.max(jnp.max(keys, axis=0, keepdims=True), axis=1, keepdims=True)
        bits = pltpu.bitcast(jnp.broadcast_to(top, (8, 128)), jnp.int32)
        low = bits & (S - 1)
        picks.append((jnp.where(bits > 0, S - 1 - low, low), pltpu.bitcast(bits & -65536, F32)))
        keys = jnp.where(keys == top, -jnp.inf, keys)
    b1, b2 = [pl.multiple_of(jnp.clip(i[0, 0] // 16, 0, S // 16 - 1) * 16, 16) for i, _ in picks]

    def gather(ref):
        return jnp.concatenate([ref[pl.ds(b1, 16)], ref[pl.ds(b2, 16)]], axis=0)

    def wide(x):
        return jnp.concatenate([x] * (D // 128), axis=1)

    x1 = gather(x1_buf)
    stats = [scale_buf[pl.ds(pl.multiple_of(b // 2, 8), 8)] for b in (b1, b2)]
    scale = jnp.concatenate([sv[:, i:i + 1] for sv in stats for i in range(2)], axis=0)
    h2 = (x1 - wide(gather(mean_buf))) * scale * coef("h mul")[0:1] + coef("h add")[0:1]
    hb = h2.astype(BF16)
    u = _dot(hb, wg_buf[...])
    act = u * jax.nn.sigmoid(u) * _dot(hb, wu_buf[...])
    y = _dot(act.astype(BF16), wd_buf[:, 0:D])
    rows = _iota((32, 128), 0)
    rows = jnp.where(rows < 16, rows + b1, rows - 16 + b2)
    update = jnp.zeros((32, D), F32)
    for i, score in picks:
        hit = wide(rows == jnp.concatenate([i] * 4, axis=0))
        update = jnp.where(hit, y * wide(jax.nn.sigmoid(score))[0:1], update)
    fix_buf[...] = (x1 + coef("gate")[0:1] * (h2 + update)).astype(BF16)

    for t in range(NC):
        out_copy(t).wait()
    fix1 = pltpu.make_async_copy(fix_buf.at[0:16], out_hbm.at[pl.ds(b1, 16)], sem_out)
    fix2 = pltpu.make_async_copy(fix_buf.at[16:32], out_hbm.at[pl.ds(b2, 16)], sem_out)
    fix1.start()

    @pl.when(b1 != b2)
    def _():
        fix2.start()
        fix2.wait()

    fix1.wait()


@jax.jit
def pallas_adaLN_cond__linear_kernel_hedgehog__moe_arch_mod__prompt_kernel(
    A_x: jax.Array,
    A_wqkv: jax.Array,
    A_w_phi: jax.Array,
    A_wo: jax.Array,
    B_x: jax.Array,
    B_w_r: jax.Array,
    B_w_gate: jax.Array,
    B_w_up: jax.Array,
    B_w_down: jax.Array,
    c: jax.Array,
    w_mod: jax.Array,
):
    hbm = pl.BlockSpec(memory_space=pl.ANY)
    vmem = pltpu.VMEM
    out = pl.pallas_call(
        _kernel,
        out_shape=jax.ShapeDtypeStruct((S, D), BF16),
        in_specs=[hbm] * 10,
        out_specs=hbm,
        scratch_shapes=[
            vmem((S, D), BF16),
            vmem((3, G, D, 128), BF16),
            vmem((H, DH, DH), BF16),
            vmem((D, D), BF16),
            vmem((D,), BF16),
            vmem((D, F), BF16),
            vmem((D, F), BF16),
            vmem((F, D + 128), BF16),
            vmem((1, D), BF16),
            vmem((D, 6 * D + 128), BF16),
            [vmem((7, HT // 2, HD), U32)] * NC,
            [vmem((7, len(SUMMED), HT // 2, QD), U32)] * (NC // 2),
            [vmem((7, 96, HD), U32)] * DEEP,
            [vmem((7, 7, 48, QD), U32)] * 3,
            [vmem((NC, 2, 2, 64, 128), F32)] * 3,
            [vmem((7, HT // 2, HD), U32)] * NC,
            vmem((1, 7, HD // 2, HD), U32),
            vmem((S, D), F32),
            vmem((S, 128), F32),
            vmem((S // 2, 128), F32),
            [vmem((1, T + 16, D), BF16)] * NC,
            vmem((1, 7, 8, D), F32),
            vmem((32, D), BF16),
            pltpu.SemaphoreType.DMA((NC + 5 + HD // SCALE_COLS,)),
        ],
        compiler_params=pltpu.CompilerParams(vmem_limit_bytes=120 * 2**20),
        name="adaln_hedgehog_mod",
    )(A_x.reshape(S, D), A_wqkv, A_w_phi, A_wo, B_w_r, B_w_gate, B_w_up, B_w_down, c, w_mod)
    return out.reshape(1, S, D)
```

```python
import numpy as np

import jax
import jax.numpy as jnp
from jax import lax
import jax.experimental.pallas as pl
import jax.experimental.pallas.tpu as pltpu

S, D, H, DH, F = 2048, 1024, 32, 32, 3584
G = 8
HD, QD = D // 2, D // 4
T = 256
HT = T // 2
NC = S // T

LOG2E = float(np.log2(np.e))
BF16_MAX = 3.3895313892515355e38
F32_TINY = float(np.finfo(np.float32).tiny)
NT = (((1,), (1,)), ((), ()))
NN = (((1,), (0,)), ((), ()))
F32, BF16, U32 = jnp.float32, jnp.bfloat16, jnp.uint32

LEAD_IN = [int(g) for g in "0000010101011111"]
SLOTS = [(g, LEAD_IN[:i].count(g)) for i, g in enumerate(LEAD_IN)] + [(g, c) for g in range(2, G) for c in range(NC)]
SLOT = {gc: s for s, gc in enumerate(SLOTS)}
PRODUCTS = (3, 1, 0, 2, 5, 4, 6)
SHIFT_SLOT, FOLD_SLOT, LATE_SLOT = 7, 10, 23
TILE_SLOT = len(SLOTS) + 4
DEEP = 2
DEEP_SLOTS = range(10, DEEP * NC + 4)
SUMMED = (0, 2, 3, 5, 6)
SCALE_COLS, WO_COLS = 256, 256
SLACK = 3
EPILOGUE_LAG = 9

PLAN_FIRST, PLAN_STREAM = "ppppppwpf", "wpppppppf"
PLAN_SHIFT, PLAN_WAIT = "pppwppppkkqqqqqqrqqf", "pkkqpqpqpwqpqfpqprqpqf"
PLAN_STEADY = "pwkkqpqfpqpqfpqpqfprqpq"
PLAN_DRAIN, PLAN_TILE = "kkqpppprpppp", "pkkpqpqpqpqprp"


def _dot(a, b, dims=NN):
    return lax.dot_general(a, b, dims, preferred_element_type=F32)


def _rnd(x):
    return x.astype(BF16).astype(F32)


def _iota(shape, axis):
    return lax.broadcasted_iota(jnp.int32, shape, axis)


def _pack(even, odd):
    return pltpu.pack_elementwise([even, odd], packed_dtype=BF16)


def _pack_halves(x):
    n = x.shape[0] // 2
    return _pack(x[:n], x[n:])


def _unpack(words):
    return pltpu.bitcast(words, BF16)


def _split(x):
    words = pltpu.bitcast(x, U32)
    return [pltpu.unpack_elementwise(words, index=i, packed_dtype=BF16, unpacked_dtype=F32) for i in range(2)]


def _interleave_halves(x):
    return _unpack(_pack_halves(x)).astype(F32) + _unpack(_pack_halves(x - _rnd(x))).astype(F32)


def _tree(x3, op):
    return op(op(op(x3[0], x3[1]), op(x3[2], x3[3])), op(op(x3[4], x3[5]), op(x3[6], x3[7])))


def _fold_rows(m, op):
    m = op(m, pltpu.roll(m, 2, 0))
    return op(m, pltpu.roll(m, 4, 0))


def _softmax2(p3, sign):
    if sign == 0:
        e = jnp.exp2(p3 - _fold_rows(_tree(p3, jnp.maximum), jnp.maximum)[None])
    else:
        e = jnp.exp2(_fold_rows(_tree(p3, jnp.minimum), jnp.minimum)[None] - p3)
    return e * pl.reciprocal(_fold_rows(_tree(e, jnp.add), jnp.add), full_range=False)[None]


def _row_means(xs):
    return [jnp.mean(x, axis=-1, keepdims=True) for x in xs]


def _row_spread(xs, means):
    lane = _iota((xs[0].shape[0], 128), 1)
    centred, var = [], None
    for i, (x, mean) in enumerate(zip(xs, means)):
        rounded = _rnd(mean)
        d = x - rounded
        v = jnp.mean(d * d, axis=-1, keepdims=True) - (mean - rounded) * (mean - rounded)
        var = jnp.where(lane == i, v, var) if i else jnp.broadcast_to(v, lane.shape)
        centred.append(d)
    return centred, var


def _row_scales(var):
    return 1.0 / _rnd(jnp.sqrt(_rnd(_rnd(var) + _rnd(jnp.full_like(var, 1e-5)))))


def _lhs_term(a, n):
    return (lambda: a(0, 0) + a(1, 1), lambda: a(1, 0) + a(1, 1), lambda: a(0, 0), lambda: a(1, 1),
            lambda: a(0, 0) + a(0, 1), lambda: a(1, 0) - a(0, 0), lambda: a(0, 1) - a(1, 1))[n]()


def _rhs_term(b, n):
    return (lambda: b(0, 0) + b(1, 1), lambda: b(0, 0), lambda: b(0, 1) - b(1, 1), lambda: b(1, 0) - b(0, 0),
            lambda: b(1, 1), lambda: b(0, 0) + b(0, 1), lambda: b(1, 0) + b(1, 1))[n]()


def _quadrant(m, i, j):
    if (i, j) == (0, 0):
        return (m(0) + m(3)) + (m(6) - m(4))
    if (i, j) == (0, 1):
        return m(2) + m(4)
    if (i, j) == (1, 0):
        return m(1) + m(3)
    return (m(0) - m(1)) + (m(2) + m(5))


def _spread(tasks, n):
    return [tasks[i * len(tasks) // n:(i + 1) * len(tasks) // n] for i in range(n)]


def _agenda():
    total, agenda = len(SLOTS), {}

    def key_slot(s):
        lag = 1 if SLOTS[s][0] < DEEP or s == total - 1 else 2
        return max(s + lag, SHIFT_SLOT + 2 + s // 2)

    def ready(g):
        return key_slot(SLOT[g, NC - 1]) + 2

    for s, gc in enumerate(SLOTS):
        agenda.setdefault(("key", key_slot(s)), []).append(gc)
        agenda.setdefault(("sum", key_slot(s) + 1), []).append(gc)
    for u in range(total):
        g, c = divmod(u, NC)
        s = min(max(ready(0) + u * (total + 2 + NC - ready(0)) // total, ready(g)), TILE_SLOT + c - 2)
        assert s >= ready(g)
        agenda.setdefault(("query", s), []).append((g, c))
        agenda.setdefault(("read", s + 1), []).append((g, c))
    return agenda


def _kernel(x_hbm, wqkv_hbm, wphi_hbm, wo_hbm, wr_hbm, wg_hbm, wu_hbm, wd_hbm, c_hbm, wmod_hbm,
            out_hbm,
            x_buf, w_buf, wphi_buf, wo_buf, wr_buf, wg_buf, wu_buf, wd_buf, c_buf, wmod_buf,
            h_terms, h_deep, w_terms, w_deep, pq_bufs, o_terms, wo_terms, x1_buf, mean_buf, scale_buf, out_bufs, coef_buf,
            fix_buf, sem):
    def x_rows(j):
        return [(x_hbm.at[pl.ds(j * T, T)], x_buf.at[pl.ds(j * T, T)])]

    def weights(*groups):
        return [(wqkv_hbm.at[:, pl.ds(i * D + g * 128, 128)], w_buf.at[i, g]) for g in groups for i in range(3)]

    def mod_cols(lo, n):
        return [(wmod_hbm.at[:, pl.ds(lo, n)], wmod_buf.at[:, pl.ds(lo, n)])]

    early = {SLOT[0, c - 1]: x_rows(c) for c in range(1, NC)}
    early[SLOT[1, 0] - 1] = weights(1) + [(wphi_hbm.at[4:H], wphi_buf.at[4:H])] + early[SLOT[1, 0] - 1]
    early[SHIFT_SLOT] = mod_cols(0, D)
    early[FOLD_SLOT] = weights(2, 3)
    batches = {
        "start": [(c_hbm, c_buf), (wphi_hbm.at[0:4], wphi_buf.at[0:4])] + weights(0) + x_rows(0),
        **{("scale", k): mod_cols(D + k, SCALE_COLS) + mod_cols(D + HD + k, SCALE_COLS)
           for k in range(0, HD, SCALE_COLS)},
        **dict(sorted(early.items())),
        LATE_SLOT: weights(*range(4, G)) + [(wr_hbm, wr_buf), (wo_hbm, wo_buf)] + mod_cols(2 * D, 2 * D),
        len(SLOTS) - 1: mod_cols(4 * D, 2 * D) + [(wg_hbm, wg_buf), (wu_hbm, wu_buf), (wd_hbm, wd_buf.at[:, 0:D])],
    }
    batches = {name: [pltpu.make_async_copy(src, dst, sem.at[i]) for src, dst in pairs]
               for i, (name, pairs) in enumerate(batches.items())}
    sem_out = sem.at[len(batches)]
    for copies in batches.values():
        for copy in copies:
            copy.start()

    def arrive(name):
        for copy in batches.pop(name):
            copy.wait()

    def out_copy(t):
        return pltpu.make_async_copy(out_bufs[t].at[0, 0:T], out_hbm.at[pl.ds(t * T, T)], sem_out)

    zero, other_zero = [jnp.min(_iota((8, 128), axis)) for axis in range(2)]
    never = _iota((8, 128), 1) < other_zero
    val, due, holds, recent = {}, {}, {}, []

    def stored(ref):
        return ref.at[zero]

    def after(x, dep, r=0):
        head = jnp.where(never, pltpu.bitcast(dep[0:8, 0:128], x.dtype), x[r:r + 8, 0:128])
        if x.shape[1] > 128:
            head = jnp.concatenate([head, x[r:r + 8, 128:]], axis=1)
        parts = ([x[:r]] if r else []) + [head] + ([x[r + 8:]] if x.shape[0] > r + 8 else [])
        return jnp.concatenate(parts, axis=0)

    def released(x):
        return after(x, val["last product"]) if "last product" in val else x

    def deadline(slot, n, dep, j=0):
        due.setdefault((slot, n, j), []).append(dep)

    def soon(lag, dep, j):
        at = val["position"] + lag
        if at < 7 * len(SLOTS):
            deadline(at // 7, PRODUCTS[at % 7], dep, j)

    def meet(x, slot, n, keys=range(4)):
        cols = [x[:, l:l + 128] for l in range(0, x.shape[1], 128)]
        for l, j in zip(range(len(cols)), keys):
            for i, dep in enumerate(due.pop((slot, n, j), [])):
                cols[l] = after(cols[l], dep, 8 * i % x.shape[0])
        return jnp.concatenate(cols, axis=1)

    same_head = _iota((128, 128), 0) // DH == _iota((128, 128), 1) // DH
    pick_feature = (_iota((128, DH), 0) % DH == _iota((128, DH), 1)).astype(BF16)

    def mix(g):
        wp = wphi_buf[g * 4:g * 4 + 4].reshape(128, DH)
        val["mix", g] = jnp.where(same_head, _dot(pick_feature, wp, NT), 0.0)

    def bias_part(g, i, k):
        left, right = val["folded", g, i, k]
        term = (left.reshape(16, 8, 128) * val["sa"][:, k:k + 128][None]
                + right.reshape(16, 8, 128) * val["sa"][:, HD + k:HD + k + 128][None])
        val["bias", g, i] = term if k == 0 else val["bias", g, i] + term
        if k == HD - 128:
            b = jnp.sum(val["bias", g, i], axis=-1, keepdims=True)
            b = jnp.broadcast_to(b, (16, 8, 128)).reshape(128, 128)
            for p in range(2):
                val["bias", g, i, p] = _interleave_halves(b[64 * p:64 * p + 64])

    def fold_tasks(g):
        def part(i, k):
            def run(slot):
                halves = []
                for lo in (k, HD + k):
                    w = _unpack(released(pltpu.bitcast(w_buf[i, g, lo:lo + 128, :], U32)))
                    halves.append(_dot(val["mix", g].astype(BF16), w, NT) if i < 2 else w.astype(F32).T)
                val["folded", g, i, k] = halves
                if g > 1:
                    bias_part(g, i, k)
                if g >= DEEP:
                    return
                for n in range(7):
                    words = _pack_halves(_lhs_term(lambda p, j: halves[j][64 * p:64 * p + 64], n))
                    w_terms[g][n, 32 * i:32 * i + 32, k:k + 128] = words
                holds["w", g, i, k] = True
                if slot is not None:
                    deadline(slot + SLACK, 1 + k // 128, words)
            return run

        def deep_terms(i, k, r):
            def run(slot):
                folded = [val["folded", g, i, k + j * QD] for j in range(2)]
                for n in PRODUCTS:
                    terms = {(j, q): _lhs_term(lambda p, l: folded[j][l][64 * p + q:64 * p + q + 8], n)
                             for j in range(2) for q in range(r, 64, 16)}
                    for m in range(7):
                        words = _pack(*[_lhs_term(lambda a, j: terms[j, e + 16 * a + r], m) for e in (0, DH)])
                        w_deep[g % 3][n, m, 16 * i + r:16 * i + r + 8, k:k + 128] = words
                    holds["w deep", g % 3, i, k, r, n] = g
                    deadline(slot + SLACK, n, words, 1 + i)
                    if n in (PRODUCTS[3], PRODUCTS[6]):
                        soon(2, words, 1)
            return run

        if g < DEEP:
            return [part(i, k) for i in range(3) for k in range(0, HD, 128)]
        return [task for i in range(3) for k in range(0, QD, 128)
                for task in (part(i, k), part(i, k + QD), deep_terms(i, k, 0), deep_terms(i, k, 8))]

    def wo_tasks():
        def piece(r, l):
            def run(slot):
                quads = {}
                for e in range(2):
                    for i in range(2):
                        lo = r // DH * 128 + r % DH + i * 64 + DH * e
                        for j in range(2):
                            w = wo_buf[lo:lo + 16, j * HD + l:j * HD + l + WO_COLS].astype(F32)
                            quads[e, i, j] = released(w)
                for n in range(7):
                    words = _pack(*[_rhs_term(lambda i, j: quads[e, i, j], n) for e in range(2)])
                    stored(wo_terms)[n, r:r + 16, l:l + WO_COLS] = words
                holds["wo", r, l] = True
                soon(3, wo_terms[0, 6, r:r + 8, l:l + 128], 3)
                deadline(slot + SLACK, (r // 16 + l // 128) % 7, wo_terms[0, 0, r:r + 8, l:l + 128])
            return run
        return [piece(r, l) for r in range(0, HD // 2, 16) for l in range(0, HD, WO_COLS)]

    def norm_means(c, r):
        rows = [slice(c * T + n * HT + r, c * T + n * HT + r + 16) for n in range(2)]
        xs = [x for n in range(2) for x in _split(x_buf[rows[n], :])]
        val["norm", c, r] = xs, _row_means(xs)

    def norm_spread(c, r):
        val["norm", c, r] = _row_spread(*val["norm", c, r])

    def norm_scales(c, r):
        centred, var = val["norm", c, r]
        scales = _row_scales(var)
        val["norm", c, r] = [(d, scales[:, i:i + 1]) for i, d in enumerate(centred)]

    def norm_stats(c, r):
        for stage, lag in ((norm_means, 0), (norm_spread, 16), (norm_scales, 32)):
            if 0 <= r - lag < HT:
                stage(c, r - lag)

    def norm_terms(c, r, k):
        h = {}
        for j in range(2):
            for n in range(2):
                for e in range(2):
                    d, scale = val["norm", c, r][2 * n + e]
                    h[e, j, n] = d[:, j * HD + k:j * HD + k + 128] * scale * val["scale", j * HD + k]
        for n in range(7):
            words = _pack(*[_rhs_term(lambda j, m: h[e, j, m], n) for e in range(2)])
            h_terms[c][n, r // 2:r // 2 + 8, k:k + 128] = words
        holds["h", c, r, k] = True
        return words

    def norm_tasks(c):
        def step(r):
            def run(slot):
                norm_stats(c, r)
                if r >= 32:
                    for k in range(0, HD, 128):
                        words = norm_terms(c, r - 32, k)
                    if slot + 1 < SLOT[0, c]:
                        deadline(slot + 1, PRODUCTS[r // 16 % 4], words)
            return run
        return [step(r) for r in range(0, HT + 32, 16)]

    def deep_tasks(pair):
        def piece(n, k):
            def run(slot):
                assert all(("h", 2 * pair + 1, r, l) in holds for r in range(0, HT, 16) for l in range(0, HD, 128))
                parts = {(j, l): _split(_unpack(released(h_terms[2 * pair + l][n, :, j * QD + k:j * QD + k + 128])))
                         for j in range(2) for l in range(2)}
                for i, m in enumerate(SUMMED):
                    words = _pack(*[_rhs_term(lambda j, l: parts[j, l][e], m) for e in range(2)])
                    h_deep[pair][n, i, :, k:k + 128] = words
                    deadline(slot + SLACK - 1, (n + i) % 7, words[56:64], 2)
                    if i in (1, 4):
                        soon(3, words[56:64], 1)
                holds["h deep", pair, n, k] = True
            return run
        return [piece(n, k) for n in PRODUCTS for k in range(0, QD, 128)]

    arrive("start")
    mix(0)
    for task in fold_tasks(0):
        task(None)
    cv = c_buf[...].astype(F32)
    cond = jnp.broadcast_to(_rnd(cv * _rnd(jax.nn.sigmoid(cv))), (16, D)).astype(BF16)
    for r in range(0, HT + 32, 16):
        norm_stats(0, r)
    cond_rows = jnp.broadcast_to(cond[0:1].astype(F32), (128, D))
    cond_cols = [cond_rows[:, k:k + 128].T for k in range(0, D, 128)]
    for k in range(0, HD, SCALE_COLS):
        arrive(("scale", k))
        for lo in (k, HD + k):
            block = _rnd(1.0 + _rnd(_dot(cond, wmod_buf[:, D + lo:D + lo + SCALE_COLS])[0:8])) * LOG2E
            for l in range(0, SCALE_COLS, 128):
                val["scale", lo + l] = block[:, l:l + 128]
        for r in range(0, HT, 16):
            for l in range(k, k + SCALE_COLS, 128):
                norm_terms(0, r, l)

    kv_mask = _iota((64, 128), 0) % 2 == (_iota((64, 128), 1) // 2) % 2

    def project_tasks(g, c):
        def product(n):
            def run():
                assert all(("w", g, i, k) in holds for i in range(3) for k in range(0, HD, 128))
                assert all(("h", c, r, k) in holds for r in range(0, HT, 16) for k in range(0, HD, 128))
                rhs = meet(h_terms[c][n], SLOT[g, c], n)
                val["last product"] = val["qkv", g, c, n] = _dot(_unpack(w_terms[g][n]), _unpack(rhs), NT)
            return run

        def deep_products(step, inner):
            def run():
                for q, (n, m) in enumerate(inner):
                    assert all(holds["w deep", g % 3, i, k, r, n] == g
                               for i in range(3) for k in range(0, QD, 128) for r in (0, 8))
                    assert all(("h deep", c // 2, n, k) in holds for k in range(0, QD, 128))
                    if m in SUMMED:
                        rhs = h_deep[c // 2][n, SUMMED.index(m)]
                    else:
                        rhs = h_terms[c - c % 2 + m // 4][n, :, m // 4 * QD:m // 4 * QD + QD]
                    rhs = meet(rhs, SLOT[g, c], step, (q, 3 if q == len(inner) - 1 else None))
                    val["inner", m] = _dot(_unpack(w_deep[g % 3][n, m]), _unpack(rhs), NT)
                    recent.append(val["inner", m])
                    val["last product"] = recent[-6:][0]
                    if m == PRODUCTS[-1]:
                        for l in range(2):
                            halves = [_quadrant(lambda k: val["inner", k], a, l) for a in range(2)]
                            val["qkv", g, c - c % 2 + l, n] = jnp.concatenate(
                                [x[32 * i:32 * i + 32] for i in range(3) for x in halves], axis=0)
            return run

        if g < DEEP:
            return [product(n) for n in PRODUCTS]
        steps = _spread([(n, m) for n in PRODUCTS for m in PRODUCTS], 14)[c % 2 * 7:c % 2 * 7 + 7]
        return [deep_products(step, inner) for step, inner in zip(PRODUCTS, steps)]

    def key_tasks(g, c):
        def piece(p, n):
            def run():
                def part(i):
                    y = _quadrant(lambda k: val["qkv", g, c, k][64 * i:64 * i + 64], p, n)
                    return y + val["bias", g, i, p] if i < 2 else y
                pq_bufs[g % 3][c, p, n] = part(0)
                holds["pq", g % 3, c, p, n] = g
                val["v", g, c, p, n] = part(2)
                logits = part(1).reshape(8, 8, 128)
                words = []
                for sign in range(2):
                    phi = _softmax2(logits, sign)
                    words.append(_pack_halves(phi.reshape(64, 128)))
                    val["z", g, p, sign] = val["z", g, p, sign] + phi if ("z", g, p, sign) in val else phi
                val["phi_k", g, c, p, n] = jnp.concatenate(words, axis=0)
                for sign in range(2):
                    soon(1, words[sign][24:32], 2 * sign)
            return run
        return [piece(p, n) for p, n in ((1, 0), (0, 1), (1, 1), (0, 0))]

    def summary_tasks(g, c):
        def piece(p):
            def run():
                v = jnp.concatenate([val["v", g, c, p, n] for n in range(2)], axis=1).astype(BF16)
                phi = _unpack(jnp.concatenate([val["phi_k", g, c, p, n] for n in range(2)], axis=1))
                kv = _dot(v, phi, NT)
                val["kv", g, p] = kv if c == 0 else val["kv", g, p] + kv
                if c == NC - 1:
                    for sign in range(2):
                        z = jnp.sum(val["z", g, p, sign], axis=-1, keepdims=True)
                        val["z total", g, p, sign] = jnp.broadcast_to(z, (8, 8, 128))
                    z_row = jnp.concatenate(
                        [_interleave_halves(val["z total", g, p, sign].reshape(64, 128)) for sign in range(2)],
                        axis=0).T[0:64]
                    val["kv", g, p] = jnp.where(kv_mask, val["kv", g, p] + val["bias", g, 2, p] * z_row, 0.0)
            return run
        return [piece(p) for p in range(2)]

    def query_tasks(g, c):
        def piece(p, n):
            def run():
                assert holds["pq", g % 3, c, p, n] == g
                logits = released(pq_bufs[g % 3][c, p, n]).reshape(8, 8, 128)
                words, den = [], None
                for sign in range(2):
                    phi = _softmax2(logits, sign)
                    words.append(_pack_halves(phi.reshape(64, 128)))
                    w = _tree(phi * val["z total", g, p, sign], jnp.add)
                    den = w if den is None else den + w
                val["1 / den", g, c, p, n] = pl.reciprocal(_fold_rows(den, jnp.add) + 1e-6, full_range=False)
                val["phi_q", g, c, p, n] = jnp.concatenate(words, axis=0)
                for sign in range(2):
                    soon(1, words[sign][24:32], 2 * sign)
            return run
        return [piece(p, n) for n in range(2) for p in range(2)]

    def readout(g, c, slot):
        nums = [_dot(val["kv", g, p].astype(BF16),
                     _unpack(jnp.concatenate([val["phi_q", g, c, p, n] for n in range(2)], axis=1)))
                for p in range(2)]
        for p in range(2):
            for n in range(2):
                num = nums[p][:, n * HT:(n + 1) * HT].reshape(8, 8, 128)
                val["o", g, c, n, p] = (num * val["1 / den", g, c, p, n][None]).reshape(64, 128)
        if g % 2:
            for k in range(7):
                term = _lhs_term(
                    lambda n, p: jnp.concatenate([val["o", g - 1, c, n, p], val["o", g, c, n, p]], axis=0), k)
                words = pltpu.bitcast(term.astype(BF16).T, U32)
                o_terms[c][k, :, 64 * (g - 1):64 * (g + 1)] = words
                deadline(slot + SLACK, k, words[56:64])
            holds["o", c, g] = True
        else:
            for k, (n, p) in enumerate(((0, 0), (0, 1), (1, 0), (1, 1))):
                deadline(slot + SLACK, k, val["o", g, c, n, p][56:64])

    agenda = _agenda()

    def run_slot(s, plan, products, extras=(), wait=None):
        keys = [task for gc in agenda.get(("key", s), []) for task in key_tasks(*gc)]
        queries = [task for gc in agenda.get(("query", s), []) for task in query_tasks(*gc)]
        mixed = sorted([((i + 0.5) / len(keys), 0, i) for i in range(len(keys))]
                       + [((i + 0.5) / len(queries), 1, i) for i in range(len(queries))])
        pieces = _spread([(keys, queries)[kind][i] for _, kind, i in mixed], plan.count("q"))
        sums = _spread([task for gc in agenda.get(("sum", s), []) for task in summary_tasks(*gc)], plan.count("k"))
        products, sides = list(products), _spread(list(extras), plan.count("f"))
        assert plan.count("p") >= len(products) and ("f" in plan or not extras) and ("w" in plan or not wait)
        assert all(step in plan or (kind, s) not in agenda
                   for step, kind in (("q", "key"), ("q", "query"), ("k", "sum"), ("r", "read")))
        val["position"] = 7 * s
        for step in plan:
            val["position"] += step == "p"
            if step == "p" and products:
                products.pop(0)()
            elif step in "qk":
                for task in (pieces if step == "q" else sums).pop(0):
                    task()
            elif step == "r":
                for gc in agenda.get(("read", s), []):
                    readout(*gc, s)
            elif step == "f":
                for task in sides.pop(0):
                    task(s)
            elif step == "w" and wait:
                wait()

    def shift():
        arrive(SHIFT_SLOT)
        val["sa"] = _rnd(_dot(cond, wmod_buf[:, 0:D])[0:8]) * LOG2E

    waits = {s: (lambda s=s: arrive(s)) for s in batches if isinstance(s, int)}
    waits[SHIFT_SLOT] = shift

    def mod_tasks():
        def piece(i, k):
            def run(slot):
                cols = released(cond_cols[k // 128])
                acc = val.get(("mod sum", i))
                for r in range(0, 128, 8):
                    term = (wmod_buf[k + r:k + r + 8, i * HD:(i + 1) * HD].astype(F32)
                            * jnp.concatenate([cols[r:r + 8]] * 4, axis=1))
                    acc = term if acc is None else acc + term
                val["mod sum", i] = acc
                for j in range(4):
                    deadline(slot + SLACK, 0, acc[:, 128 * j:128 * j + 128])
                if k == D - 128:
                    val["mod", i] = jnp.broadcast_to(_rnd(jnp.sum(acc, axis=0, keepdims=True)), (8, HD))
            return run
        return [piece(i, k) for i in range(4, 8) for k in range(0, D, 128)]

    extras = {s: [] for s in range(len(SLOTS))}

    def assign(tasks, slots):
        for s, chunk in zip(slots, _spread(tasks, len(slots))):
            extras[s] += chunk

    assign([lambda s, g=g: mix(g) for g in range(1, G)] + fold_tasks(1), [SLOT[1, 0] - 1])
    for c in range(1, NC):
        assign(norm_tasks(c), range(SLOT[0, c - 1], SLOT[0, c]))
    for g, slots in enumerate(([SHIFT_SLOT], range(SHIFT_SLOT + 1, SHIFT_SLOT + 4))):
        assign([lambda s, g=g, i=i, k=k: bias_part(g, i, k) for i in range(3) for k in range(0, HD, 128)], slots)
    for g in range(2, G):
        tasks, slots = fold_tasks(g), range(max((g - 1) * NC, FOLD_SLOT), g * NC - 1)
        assign(tasks[:len(tasks) * 2 // 3], slots)
        assign(tasks[len(tasks) * 2 // 3:], slots)
    assign([task for pair in range(NC // 2) for task in deep_tasks(pair)], DEEP_SLOTS)
    assign(wo_tasks(), range(LATE_SLOT, len(SLOTS) - 2))
    assign(mod_tasks(), range(LATE_SLOT, len(SLOTS) - 4))

    for s, gc in enumerate(SLOTS):
        plan = (PLAN_FIRST if s == 0 else PLAN_STREAM if s < SHIFT_SLOT else PLAN_SHIFT if s == SHIFT_SLOT
                else PLAN_WAIT if s in waits and s > FOLD_SLOT else PLAN_STEADY)
        run_slot(s, plan, project_tasks(*gc), extras[s], waits.get(s))

    def mod_part(i):
        def run():
            lhs = _unpack(released(pltpu.bitcast(cond, U32)))
            val["mod", i] = _rnd(_dot(lhs, wmod_buf[:, i * HD:(i + 1) * HD])[0:8])
        return run

    def head_start(n):
        def run():
            assert all(("o", 0, g) in holds for g in range(1, G - 2, 2))
            assert all(("wo", r, l) in holds for r in range(0, HD // 2, 16) for l in range(0, HD, WO_COLS))
            lhs = released(o_terms[0][n, :, 0:HD - 128])
            val["head start", 0, n] = _dot(_unpack(lhs), _unpack(wo_terms[0, n, 0:HD // 2 - 64]))
        return run

    fillers = [head_start(n) for n in PRODUCTS[:4]] + [mod_part(i) for i in range(8, 12)]
    for s, tasks in zip(range(len(SLOTS), TILE_SLOT), _spread(fillers, 4)):
        run_slot(s, PLAN_DRAIN, tasks)
    ga, sb, cb, gb = [jnp.concatenate([val["mod", 2 * i], val["mod", 2 * i + 1]], axis=1) for i in range(2, 6)]
    cb1 = _rnd(1.0 + cb)
    wr = jnp.broadcast_to(wr_buf[...].reshape(1, D).astype(F32), (8, D))
    coefs = {"attn": ga * (1.0 / LOG2E), "out mul": gb * cb1, "out add": gb * sb, "score": cb1 * wr,
             "h mul": cb1, "h add": sb, "gate": gb}
    for i, row in enumerate(coefs.values()):
        stored(coef_buf)[i] = row
    score_add = jnp.sum(sb * wr, axis=-1, keepdims=True)
    deadline(TILE_SLOT, PRODUCTS[0], gb)

    def coef(name):
        return coef_buf[0, list(coefs).index(name)]

    lane = _iota((8, 128), 1)
    scores = [jnp.zeros((8, 128), F32)] * 2

    def finish_rows(t, i, r):
        r0 = t * T + i * HT + r
        xs = []
        for e in (0, 8):
            a = jnp.concatenate(
                [_quadrant(lambda k: val["attn", t, k][r + e:r + e + 8], i, j) for j in range(2)], axis=1)
            xs.append(x_buf[r0 + e:r0 + e + 8, :].astype(F32) + coef("attn") * a)
            x1_buf[r0 + e:r0 + e + 8] = xs[-1]
        means = _row_means(xs)
        centred, var = _row_spread(xs, means)
        scales = _row_scales(var)
        scale_buf[r0 // 2:r0 // 2 + 8] = scales
        outs = []
        for k in range(2):
            scale = scales[:, k:k + 1]
            mean_buf[r0 + 8 * k:r0 + 8 * k + 8] = jnp.broadcast_to(_rnd(means[k]), (8, 128))
            outs.append(xs[k] + (centred[k] * scale * coef("out mul") + coef("out add")))
            score = jnp.sum(centred[k] * coef("score"), axis=-1, keepdims=True) * scale
            scores[r0 // 1024] = jnp.where(lane == (r0 // 8 + k) % 128, score, scores[r0 // 1024])
        rows = slice(r0 - t * T, r0 - t * T + 16)
        stored(out_bufs[t])[rows, :] = jnp.concatenate(outs, axis=0).astype(BF16)
        return pltpu.bitcast(out_bufs[t][0, rows, 0:128], U32), scores[r0 // 1024]

    pending = [(7 * t + EPILOGUE_LAG + k * 7 // 16, t, k) for t in range(NC) for k in range(16)]

    def flush(upto, slot=None, n=None):
        while pending and pending[0][0] <= upto:
            _, t, k = pending.pop(0)
            done = finish_rows(t, 1 - k // 8, 16 * (k % 8))
            if slot is not None:
                for dep in done:
                    deadline(slot, n, dep)
            if k == 15:
                out_copy(t).start()
                stored(out_bufs[t])[T:T + 16, 0:128] = jnp.zeros((16, 128), BF16)
                deadline(TILE_SLOT + (upto + 2) // 7, PRODUCTS[(upto + 2) % 7],
                         pltpu.bitcast(out_bufs[t][0, T:T + 16, 0:128], U32), 3)

    def tile_tasks(t):
        def product(j, n):
            def run():
                flush(7 * t + j, TILE_SLOT + t, n)
                assert all(("o", t, g) in holds for g in range(1, G, 2))
                assert all(("wo", r, l) in holds for r in range(0, HD // 2, 16) for l in range(0, HD, WO_COLS))
                lo = HD - 128 if ("head start", t, n) in val else 0
                rhs = meet(wo_terms[0, n, lo // 2:], TILE_SLOT + t, n)
                val["last product"] = val["attn", t, n] = _dot(_unpack(o_terms[t][n, :, lo:]), _unpack(rhs))
                if lo:
                    val["attn", t, n] += val["head start", t, n]
            return run
        return [product(j, n) for j, n in enumerate(PRODUCTS)]

    for t in range(NC):
        run_slot(TILE_SLOT + t, PLAN_TILE, tile_tasks(t))
    flush(pending[-1][0])
    assert not batches

    r = _rnd(jnp.concatenate(scores, axis=0) + jnp.concatenate([score_add] * 2, axis=0))
    r = jnp.clip(jnp.where(r != r, -BF16_MAX, r), -BF16_MAX, BF16_MAX)
    r = jnp.where(jnp.abs(r) < F32_TINY, F32_TINY, r)
    token = (_iota((16, 128), 0) // 8) * 1024 + _iota((16, 128), 1) * 8 + _iota((16, 128), 0) % 8
    keys = pltpu.bitcast(pltpu.bitcast(r, jnp.int32) | jnp.where(r > 0, S - 1 - token, token), F32)
    picks = []
    for _ in range(2):
        top = jnp.max(jnp.max(keys, axis=0, keepdims=True), axis=1, keepdims=True)
        bits = pltpu.bitcast(jnp.broadcast_to(top, (8, 128)), jnp.int32)
        low = bits & (S - 1)
        picks.append((jnp.where(bits > 0, S - 1 - low, low), pltpu.bitcast(bits & -65536, F32)))
        keys = jnp.where(keys == top, -jnp.inf, keys)
    b1, b2 = [pl.multiple_of(jnp.clip(i[0, 0] // 16, 0, S // 16 - 1) * 16, 16) for i, _ in picks]

    def gather(ref):
        return jnp.concatenate([ref[pl.ds(b1, 16)], ref[pl.ds(b2, 16)]], axis=0)

    def wide(x):
        return jnp.concatenate([x] * (D // 128), axis=1)

    x1 = gather(x1_buf)
    stats = [scale_buf[pl.ds(pl.multiple_of(b // 2, 8), 8)] for b in (b1, b2)]
    scale = jnp.concatenate([sv[:, i:i + 1] for sv in stats for i in range(2)], axis=0)
    h2 = (x1 - wide(gather(mean_buf))) * scale * coef("h mul")[0:1] + coef("h add")[0:1]
    hb = h2.astype(BF16)
    u = _dot(hb, wg_buf[...])
    act = u * jax.nn.sigmoid(u) * _dot(hb, wu_buf[...])
    y = _dot(act.astype(BF16), wd_buf[:, 0:D])
    rows = _iota((32, 128), 0)
    rows = jnp.where(rows < 16, rows + b1, rows - 16 + b2)
    update = jnp.zeros((32, D), F32)
    for i, score in picks:
        hit = wide(rows == jnp.concatenate([i] * 4, axis=0))
        update = jnp.where(hit, y * wide(jax.nn.sigmoid(score))[0:1], update)
    fix_buf[...] = (x1 + coef("gate")[0:1] * (h2 + update)).astype(BF16)

    for t in range(NC):
        out_copy(t).wait()
    fix1 = pltpu.make_async_copy(fix_buf.at[0:16], out_hbm.at[pl.ds(b1, 16)], sem_out)
    fix2 = pltpu.make_async_copy(fix_buf.at[16:32], out_hbm.at[pl.ds(b2, 16)], sem_out)
    fix1.start()

    @pl.when(b1 != b2)
    def _():
        fix2.start()
        fix2.wait()

    fix1.wait()


@jax.jit
def pallas_adaLN_cond__linear_kernel_hedgehog__moe_arch_mod__prompt_kernel(
    A_x: jax.Array,
    A_wqkv: jax.Array,
    A_w_phi: jax.Array,
    A_wo: jax.Array,
    B_x: jax.Array,
    B_w_r: jax.Array,
    B_w_gate: jax.Array,
    B_w_up: jax.Array,
    B_w_down: jax.Array,
    c: jax.Array,
    w_mod: jax.Array,
):
    hbm = pl.BlockSpec(memory_space=pl.ANY)
    vmem = pltpu.VMEM
    out = pl.pallas_call(
        _kernel,
        out_shape=jax.ShapeDtypeStruct((S, D), BF16),
        in_specs=[hbm] * 10,
        out_specs=hbm,
        scratch_shapes=[
            vmem((S, D), BF16),
            vmem((3, G, D, 128), BF16),
            vmem((H, DH, DH), BF16),
            vmem((D, D), BF16),
            vmem((D,), BF16),
            vmem((D, F), BF16),
            vmem((D, F), BF16),
            vmem((F, D + 128), BF16),
            vmem((1, D), BF16),
            vmem((D, 6 * D + 128), BF16),
            [vmem((7, HT // 2, HD), U32)] * NC,
            [vmem((7, len(SUMMED), HT // 2, QD), U32)] * (NC // 2),
            [vmem((7, 96, HD), U32)] * DEEP,
            [vmem((7, 7, 48, QD), U32)] * 3,
            [vmem((NC, 2, 2, 64, 128), F32)] * 3,
            [vmem((7, HT // 2, HD), U32)] * NC,
            vmem((1, 7, HD // 2, HD), U32),
            vmem((S, D), F32),
            vmem((S, 128), F32),
            vmem((S // 2, 128), F32),
            [vmem((1, T + 16, D), BF16)] * NC,
            vmem((1, 7, 8, D), F32),
            vmem((32, D), BF16),
            pltpu.SemaphoreType.DMA((NC + 5 + HD // SCALE_COLS,)),
        ],
        compiler_params=pltpu.CompilerParams(vmem_limit_bytes=120 * 2**20),
        name="adaln_hedgehog_mod",
    )(A_x.reshape(S, D), A_wqkv, A_w_phi, A_wo, B_w_r, B_w_gate, B_w_up, B_w_down, c, w_mod)
    return out.reshape(1, S, D)
```
